```python
import jax
import jax.numpy as jnp

def _softmax(x, axis=-1):
    return jax.nn.softmax(x, axis=axis)
def _gelu(x):
    return jax.nn.gelu(x, approximate=True)
def _silu(x):
    return jax.nn.silu(x)
def _sigmoid(x):
    return jax.nn.sigmoid(x)
def _layernorm(x, axis=-1, eps=1e-5):
    m = jnp.mean(x, axis=axis, keepdims=True)
    v = jnp.var(x, axis=axis, keepdims=True)
    return (x - m) / jnp.sqrt(v + eps)
def _scatter_add(tgt, idx, src, axis=0):
    return tgt.at[idx].add(src)
def _segment_sum(src, seg, n):
    return jax.ops.segment_sum(src, seg, n)
class _Rng:
    def __init__(self, key):
        self._k = key
    def _next(self):
        self._k, sub = jax.random.split(self._k)
        return sub
    def normal(self, shape):
        return jax.random.normal(self._next(), shape, dtype=jnp.bfloat16)
    def randint(self, lo, hi, shape):
        return jax.random.randint(self._next(), shape, lo, hi, dtype=jnp.int32)
    def uniform(self, shape, lo=0.0, hi=1.0):
        return jax.random.uniform(self._next(), shape, jnp.bfloat16, lo, hi)
    def permutation(self, n):
        return jax.random.permutation(self._next(), n)


kernel_name = 'recurrent_scan__sliding_local_dilated__geglu_ffn__prompt'

def setup_inputs():
    _rng = _Rng(jax.random.key(int.from_bytes(__import__("os").urandom(4), "little")))
    _w = (lambda a: (lambda t: t.astype(jnp.bfloat16) if jnp.issubdtype(t.dtype, jnp.floating) else t)(jnp.asarray(a)))
    def _A_setup():
        B, S, D = 1, 2048, 1024
        return {
            "x": _w((lambda *s: _rng.normal(s) * 0.05)(B, S, D)),
            "wqkv": _w((lambda *s: _rng.normal(s) * 0.05)(D, 3 * D)),
            "wo": _w((lambda *s: _rng.normal(s) * 0.05)(D, D)),
        }
    _A_in = _A_setup()

    def _B_setup():
        B, S, D, F = 1, 2048, 1024, 3584
        return {
            "x": _w((lambda *s: _rng.normal(s) * 0.05)(B, S, D)),
            "w_gate": _w((lambda *s: _rng.normal(s) * 0.05)(D, F)),
            "w_up": _w((lambda *s: _rng.normal(s) * 0.05)(D, F)),
            "w_down": _w((lambda *s: _rng.normal(s) * 0.05)(F, D)),
        }
    _B_in = _B_setup()

    return {
        "A_x": _A_in["x"],
        "A_wqkv": _A_in["wqkv"],
        "A_wo": _A_in["wo"],
        "B_x": _B_in["x"],
        "B_w_gate": _B_in["w_gate"],
        "B_w_up": _B_in["w_up"],
        "B_w_down": _B_in["w_down"],
    }

def reference(A_x, A_wqkv, A_wo, B_x, B_w_gate, B_w_up, B_w_down):
    def _A_ref(x, wqkv, wo):
        B, S, D = x.shape
        H = 32; Dh = D // H
        W, dil = 8, 2
        qkv = (lambda x, *d: x.transpose(*d))((x @ wqkv).reshape(B, S, 3, H, Dh), 2, 0, 3, 1, 4)
        q, k, v = qkv[0], qkv[1], qkv[2]
        scale = Dh ** -0.5
        pos = jnp.arange(S)
        off = jnp.arange(W) * dil
        idx = pos[:, None] - off[None, :]
        mask = idx >= 0
        idx_c = jnp.where(mask, idx, 0).reshape(-1)
        kg = k[:, :, idx_c, :].reshape(B, H, S, W, Dh)
        vg = v[:, :, idx_c, :].reshape(B, H, S, W, Dh)
        logits = jnp.einsum("bhsd,bhswd->bhsw", q, kg) * scale
        logits = jnp.where(mask[None, None, :, :], logits, -1e9)
        attn = _softmax(logits, axis=-1)
        o = jnp.einsum("bhsw,bhswd->bhsd", attn, vg)
        return (lambda x, *d: x.transpose(*d))(o, 0, 2, 1, 3).reshape(B, S, D) @ wo

    def _B_ref(x, w_gate, w_up, w_down):
        return (_gelu(x @ w_gate) * (x @ w_up)) @ w_down

    x = A_x
    xn = _layernorm(x, axis=-1)
    s = _A_ref(xn, A_wqkv, A_wo)
    g = _silu(_B_ref(xn, B_w_gate, B_w_up, B_w_down))
    return x + s * g
```

```python
import functools
import math

import jax
import jax.numpy as jnp
import numpy as np
from jax import lax
import jax.experimental.pallas as pl
import jax.experimental.pallas.tpu as pltpu

S, D, F = 2048, 1024, 3584
H, DH, W, DIL = 32, 32, 8, 2
PAD = 16
LOG2E = math.log2(math.e)
f32, bf16 = jnp.float32, jnp.bfloat16


def _dot(a, b):
    return jnp.dot(a, b, preferred_element_type=f32)


def _layernorm(x):
    x = x.astype(f32)
    m = jnp.mean(x, axis=-1, keepdims=True)
    xc = x - m
    v = jnp.mean(xc * xc, axis=-1, keepdims=True)
    return xc * lax.rsqrt(v + 1e-5)


def _shuffle(cols):
    lane = lax.broadcasted_iota(jnp.int32, cols[0].shape, 1)
    cols = list(cols)
    for b in range(3):
        sh = 4 << b
        lo = (lane & sh) == 0
        for c in range(8):
            if c & (1 << b):
                continue
            a, bb = cols[c], cols[c | (1 << b)]
            cols[c] = jnp.where(lo, a, pltpu.roll(bb, sh, 1))
            cols[c | (1 << b)] = jnp.where(lo, pltpu.roll(a, 128 - sh, 1), bb)
    return cols


def _shuffle_bf16(cols):
    packed = [pltpu.bitcast(c.astype(bf16), jnp.uint32) for c in cols]
    return [pltpu.bitcast(p, bf16) for p in _shuffle(packed)]


def _geglu2(g, u):
    c0 = math.sqrt(2.0 / math.pi)
    t = jnp.tanh(g * (g * g * (c0 * 0.044715) + c0))
    p = g * u
    return p * t + p


def make(tm1=512, rb1=256, fc=256, rb2=256, tm3=256, ab=16, attn=True):
    n1 = S // tm1
    n2 = F // fc
    n3 = S // tm3
    arows = -(-S // (n2 * ab)) * ab
    WCH = 512
    nw = 3 * D // WCH

    def attention_block(r0, q_s, k_s, v_s, o_s):
        lane = lax.broadcasted_iota(jnp.int32, (ab, 128), 1)
        row = lax.broadcasted_iota(jnp.int32, (ab, 128), 0) + r0
        logits = [None] * W
        for j in range(8):
            q = q_s[j, pl.ds(r0, ab), :]
            for w in range(W):
                t = q * k_s[j, pl.ds(r0 + (PAD - DIL * w), ab), :]
                logits[w] = t if j == 0 else logits[w] + t
        for w in range(W):
            t = logits[w]
            t = t + pltpu.roll(t, 127, 1)
            t = t + pltpu.roll(t, 126, 1)
            t = t * (DH ** -0.5 * LOG2E)
            if w:
                t = jnp.where(row >= DIL * w, t, -1e9 * LOG2E)
            logits[w] = t
        m = functools.reduce(jnp.maximum, logits)
        e = [jnp.exp2(t - m) for t in logits]
        inv = 1.0 / functools.reduce(lambda a, b: a + b, e)
        p = []
        for w in range(W):
            t = e[w] * inv
            t = jnp.where((lane & 1) == 0, t, pltpu.roll(t, 1, 1))
            t = jnp.where((lane & 2) == 0, t, pltpu.roll(t, 2, 1))
            p.append(t)
        outs = []
        for j in range(8):
            acc = None
            for w in range(W):
                t = p[w] * v_s[j, pl.ds(r0 + (PAD - DIL * w), ab), :]
                acc = t if acc is None else acc + t
            outs.append(acc)
        outs = _shuffle_bf16(outs)
        for c in range(8):
            o_s[pl.ds(r0, ab), c * 128:(c + 1) * 128] = outs[c]

    def kern(x_h, wqkv_h, wo_h, wg_h, wu_h, wd_h, out_h,
             x_s, xn_s, xc_s, q_s, k_s, v_s, o_s, y_s, wqkv_s, wo_s, wg_s, wu_s, wd_s,
             sx, sqkv, swo, sg, su, sd, so):
        def x_cp(t):
            r = pl.ds(pl.multiple_of(t * tm1, tm1), tm1)
            return pltpu.make_async_copy(x_h.at[r, :], x_s.at[r, :], sx.at[t])

        def qkv_cp(c):
            return pltpu.make_async_copy(wqkv_h.at[:, pl.ds(c * WCH, WCH)], wqkv_s.at[c], sqkv.at[c])

        def ffn_cps(c):
            r = pl.ds(pl.multiple_of(c * fc, fc), fc)
            return (pltpu.make_async_copy(wg_h.at[:, r], wg_s.at[c], sg.at[c]),
                    pltpu.make_async_copy(wu_h.at[:, r], wu_s.at[c], su.at[c]),
                    pltpu.make_async_copy(wd_h.at[r, :], wd_s.at[c], sd.at[c]))

        wo_cp = pltpu.make_async_copy(wo_h, wo_s, swo.at[0])

        def out_cp(t):
            r = pl.ds(pl.multiple_of(t * tm3, tm3), tm3)
            return pltpu.make_async_copy(x_s.at[r, :], out_h.at[r, :], so.at[t])

        x_cp(0).start()
        qkv_cp(0).start()
        x_cp(0).wait()
        qkv_cp(1).start()
        xn0 = _layernorm(x_s[0:tm1, :]).astype(bf16)
        xn_s[0:tm1, :] = xn0

        def phase1(t, _):
            r0 = pl.multiple_of(t * tm1, tm1)
            xc_s[...] = xn_s[pl.ds(r0, tm1), :]

            @pl.when(t + 1 < n1)
            def _():
                x_cp(t + 1).start()

            @pl.when(t == 1)
            def _():
                for cp in ffn_cps(0):
                    cp.start()

            for part, dst in enumerate((q_s, k_s, v_s)):
                for rb in range(tm1 // rb1):
                    cols = []
                    for hc in range(D // WCH):
                        c = part * (D // WCH) + hc
                        if rb == 0:
                            @pl.when(t == 0)
                            def _():
                                qkv_cp(c).wait()
                                if c + 2 < nw:
                                    qkv_cp(c + 2).start()
                        y = _dot(xc_s[rb * rb1:(rb + 1) * rb1, :], wqkv_s[c])
                        cols += [y[:, i * 128:(i + 1) * 128] for i in range(WCH // 128)]
                    cols = _shuffle_bf16(cols)
                    off = rb * rb1 + (PAD if part else 0)
                    for j in range(8):
                        dst[j, pl.ds(r0 + off, rb1), :] = cols[j].astype(f32)
                if part == 1:
                    @pl.when(t + 1 < n1)
                    def _():
                        x_cp(t + 1).wait()
                    rn = pl.multiple_of(jnp.minimum(t + 1, n1 - 1) * tm1, tm1)
                    xn_s[pl.ds(rn, tm1), :] = _layernorm(x_s[pl.ds(rn, tm1), :]).astype(bf16)

        lax.fori_loop(0, n1, phase1, None)

        for j in range(8):
            k_s[j, 0:PAD, :] = jnp.broadcast_to(k_s[j, PAD:PAD + 1, :], (PAD, 128))
            v_s[j, 0:PAD, :] = jnp.broadcast_to(v_s[j, PAD:PAD + 1, :], (PAD, 128))
        y_s[...] = jnp.zeros_like(y_s)
        wo_cp.start()

        def phase2(c, _):
            for cp in ffn_cps(c):
                cp.wait()

            @pl.when(c + 1 < n2)
            def _():
                for cp in ffn_cps(c + 1):
                    cp.start()

            a0 = jnp.minimum(c * arows, S - arows)
            nb = S // rb2
            na = arows // ab
            hs = [None] * nb
            done = 0
            for rb in range(nb + 1):
                if rb < nb:
                    xn = xn_s[rb * rb2:(rb + 1) * rb2, :]
                    hs[rb] = _geglu2(_dot(xn, wg_s[c]), _dot(xn, wu_s[c])).astype(bf16)
                if rb > 0:
                    r = slice((rb - 1) * rb2, rb * rb2)
                    y_s[r, :] += _dot(hs[rb - 1], wd_s[c])
                if attn:
                    upto = min(na, -(-na * (rb + 1) // nb))
                    for i in range(done, upto):
                        attention_block(pl.multiple_of(a0 + i * ab, ab), q_s, k_s, v_s, o_s)
                    done = upto

        lax.fori_loop(0, n2, phase2, None)
        wo_cp.wait()

        def phase3(t, _):
            r = pl.ds(pl.multiple_of(t * tm3, tm3), tm3)
            s = _dot(o_s[r, :], wo_s[...])
            y = y_s[r, :] * 0.5
            g = y * jax.nn.sigmoid(y)
            x_s[r, :] = (x_s[r, :].astype(f32) + s * g).astype(bf16)
            out_cp(t).start()

        lax.fori_loop(0, n3, phase3, None)
        for t in range(n3):
            out_cp(t).wait()

    def fn(A_x, A_wqkv, A_wo, B_x, B_w_gate, B_w_up, B_w_down):
        any_spec = pl.BlockSpec(memory_space=pl.ANY)
        out = pl.pallas_call(
            kern,
            in_specs=[any_spec] * 6,
            out_specs=any_spec,
            out_shape=jax.ShapeDtypeStruct((S, D), bf16),
            scratch_shapes=[
                pltpu.VMEM((S, D), bf16),
                pltpu.VMEM((S, D), bf16),
                pltpu.VMEM((tm1, D), bf16),
                pltpu.VMEM((8, S, 128), f32),
                pltpu.VMEM((8, S + PAD, 128), f32),
                pltpu.VMEM((8, S + PAD, 128), f32),
                pltpu.VMEM((S, D), bf16),
                pltpu.VMEM((S, D), f32),
                pltpu.VMEM((nw, D, WCH), bf16),
                pltpu.VMEM((D, D), bf16),
                pltpu.VMEM((n2, D, fc), bf16),
                pltpu.VMEM((n2, D, fc), bf16),
                pltpu.VMEM((n2, fc, D), bf16),
                pltpu.SemaphoreType.DMA((n1,)),
                pltpu.SemaphoreType.DMA((nw,)),
                pltpu.SemaphoreType.DMA((1,)),
                pltpu.SemaphoreType.DMA((n2,)),
                pltpu.SemaphoreType.DMA((n2,)),
                pltpu.SemaphoreType.DMA((n2,)),
                pltpu.SemaphoreType.DMA((n3,)),
            ],
            compiler_params=pltpu.CompilerParams(vmem_limit_bytes=110 << 20),
        )(A_x.reshape(S, D), A_wqkv, A_wo, B_w_gate, B_w_up, B_w_down)
        return out.reshape(1, S, D)

    return fn


@jax.jit
def pallas_recurrent_scan__sliding_local_dilated__geglu_ffn__prompt_kernel(
    A_x, A_wqkv, A_wo, B_x, B_w_gate, B_w_up, B_w_down
):
    return make()(A_x, A_wqkv, A_wo, B_x, B_w_gate, B_w_up, B_w_down)
```

```python
import functools
import math

import jax
import jax.numpy as jnp
from jax import lax
import jax.experimental.pallas as pl
import jax.experimental.pallas.tpu as pltpu

S, D, F = 2048, 1024, 3584
H, DH, W, DIL = 32, 32, 8, 2
PAD = 16
LOG2E = math.log2(math.e)
f32, bf16, u32 = jnp.float32, jnp.bfloat16, jnp.uint32


def _dot(a, b):
    return jnp.dot(a, b, preferred_element_type=f32)


def _pack(v):
    return pltpu.bitcast(v.astype(bf16), u32)


def _unpack(v):
    return pltpu.bitcast(v, bf16)


def _put(ref, n, rows, cols, v):
    ref[pl.ds(n, 1), rows, cols] = _pack(v[None])


def _ds(start, size, align):
    if isinstance(start, int):
        return pl.ds(start, size)
    return pl.ds(pl.multiple_of(start, align), size)


def _layernorm(x):
    x = x.astype(f32)
    m = jnp.mean(x, axis=-1, keepdims=True)
    xc = x - m
    v = jnp.mean(xc * xc, axis=-1, keepdims=True)
    return xc * lax.rsqrt(v + 1e-5)


def _swap_level(cols, b):
    sh = 4 << b
    lo = (lax.broadcasted_iota(jnp.int32, cols[0].shape, 1) & sh) == 0
    cols = list(cols)
    for c in range(8):
        if not c & (1 << b):
            x, y = cols[c], cols[c | (1 << b)]
            cols[c] = jnp.where(lo, x, pltpu.roll(y, sh, 1))
            cols[c | (1 << b)] = jnp.where(lo, pltpu.roll(x, 128 - sh, 1), y)
    return cols


def _geglu2(g, u):
    c0 = math.sqrt(2.0 / math.pi)
    t = jnp.tanh(g * (g * g * (c0 * 0.044715) + c0))
    p = g * u
    return p * t + p


def _grid(v, n):
    r, c = v.shape[0] // n, v.shape[1] // n
    return [[v[i * r:(i + 1) * r, j * c:(j + 1) * c] for j in range(n)] for i in range(n)]


def _quad(g):
    h = len(g) // 2
    return ([r[:h] for r in g[:h]], [r[h:] for r in g[:h]],
            [r[:h] for r in g[h:]], [r[h:] for r in g[h:]])


def _add(a, b):
    return [[x + y for x, y in zip(r, s)] for r, s in zip(a, b)]


def _sub(a, b):
    return [[x - y for x, y in zip(r, s)] for r, s in zip(a, b)]


def _lhs_term(q, n):
    a11, a12, a21, a22 = q
    return (lambda: _add(a21(), a22()), lambda: _add(a11(), a12()), a11, a22, lambda: _add(a11(), a22()),
            lambda: _sub(a21(), a11()), lambda: _sub(a12(), a22()))[n]()


def _rhs_term(q, n):
    b11, b12, b21, b22 = q
    return (b11, b22, lambda: _sub(b12(), b22()), lambda: _sub(b21(), b11()), lambda: _add(b11(), b22()),
            lambda: _add(b11(), b12()), lambda: _add(b21(), b22()))[n]()


def _terms(term, g):
    if len(g) == 1:
        return [g[0][0]]
    q = [lambda v=v: v for v in _quad(g)]
    return [x for n in range(7) for x in _terms(term, term(q, n))]


def _outer_terms(term, load, level, n):
    if level == 0:
        return [load(0, 0)]
    h = 2 ** (level - 1)
    q = [lambda a=a, b=b: [[load(a * h + i, b * h + j) for j in range(h)] for i in range(h)]
         for a in range(2) for b in range(2)]
    return _terms(term, term(q, n))


def _merge(m, emit):
    m2 = m(0)
    m5 = m(1)
    m3 = m(2)
    emit(0, 1, _add(m3, m5))
    t22 = _sub(m3, m2)
    m4 = m(3)
    emit(1, 0, _add(m2, m4))
    t11 = _sub(m4, m5)
    m1 = m(4)
    t11 = _add(t11, m1)
    t22 = _add(t22, m1)
    emit(1, 1, _add(t22, m(5)))
    emit(0, 0, _add(t11, m(6)))


def _combine(prod, level, emit=None, base=0):
    g = 2 ** level
    out = [[None] * g for _ in range(g)]

    def put(i, j, v):
        out[i][j] = v
        if emit is not None:
            emit(i, j, v)

    if level == 0:
        put(0, 0, prod(base))
        return out

    def quadrant(a, b, q):
        for i in range(g // 2):
            for j in range(g // 2):
                put(a * g // 2 + i, b * g // 2 + j, q[i][j])

    _merge(lambda i: _combine(prod, level - 1, None, base + i * 7 ** (level - 1)), quadrant)
    return out


class _Tasks:
    def __init__(self):
        self.queues = []

    def add(self, tasks, steps):
        q = [list(tasks), max(steps, 1), 0, 0]
        self.queues.append(q)
        return q

    def step(self):
        for q in self.queues:
            q[2] += 1
            upto = min(len(q[0]), -(-len(q[0]) * q[2] // q[1]))
            while q[3] < upto:
                q[3] += 1
                q[0][q[3] - 1]()

    def finish(self, *qs):
        for q in qs or self.queues:
            while q[3] < len(q[0]):
                q[3] += 1
                q[0][q[3] - 1]()


def make(tm1=512, sb=256, fc=512, th=1024, nsb2=1, tm3=1024, rb3=256, ab=16, l1=1, l2=1, l3=1,
         rb1=256, nt1=256, nt2=256, ntd=512, nt3=512, attn=True, yacc=False, gr=32, rq=True, flags=None,
         bsr=32, only=None, af=0.9, skew=7, lchain=2, lf=0.7):
    n1 = S // tm1
    n2 = F // fc
    nh = S // th
    n3 = S // tm3
    g1, g2, g3 = 2 ** l1, 2 ** l2, 2 ** l3
    ag = 16 * g3
    na = -(-S // (n2 * nh * ag))
    nls = tm1 // sb // 2
    xe = 2
    lnb = 16

    def attention_tasks(g0, qkv_s, st_s, o_s):
        res = {}

        def block(b):
            r0 = (b - 1) * 16
            parts = (0, 1, 2) if b else (1, 2)
            st = {}

            def gather(p, lvl):
                if lvl == 0:
                    st["in", p] = [qkv_s[p, _ds((g0 * ag + b * 16) // 2, 8, 8), j * 128:(j + 1) * 128]
                                   for j in range(8)]
                st["in", p] = _swap_level(st["in", p], lvl)
                if lvl == 2:
                    for j, v in enumerate(st["in", p]):
                        st_s[p, j, b * 16:(b + 1) * 16, :] = _unpack(v).astype(f32)

            def scores(j):
                q = st_s[0, j, pl.ds(r0 + PAD, 16), :]
                for w in range(W):
                    t = q * st_s[1, j, pl.ds(r0 + PAD - DIL * w, 16), :]
                    st[w] = t if j == 0 else st[w] + t

            def reduce(sh):
                for w in range(W):
                    st[w] = st[w] + pltpu.roll(st[w], 128 - sh, 1)

            def softmax():
                row = lax.broadcasted_iota(jnp.int32, (16, 128), 0) + (g0 * ag + r0)
                logits = []
                for w in range(W):
                    t = st[w] * (DH ** -0.5 * LOG2E)
                    if r0 < DIL * w:
                        t = jnp.where(row >= DIL * w, t, -1e9 * LOG2E)
                    logits.append(t)
                m = functools.reduce(jnp.maximum, logits)
                e = [jnp.exp2(t - m) for t in logits]
                inv = 1.0 / functools.reduce(lambda a, b: a + b, e)
                for w in range(W):
                    st[w] = e[w] * inv

            def spread(sh):
                keep = (lax.broadcasted_iota(jnp.int32, (16, 128), 1) & sh) == 0
                for w in range(W):
                    st[w] = jnp.where(keep, st[w], pltpu.roll(st[w], sh, 1))

            def values(j):
                acc = None
                for w in range(W):
                    t = st[w] * st_s[2, j, pl.ds(r0 + PAD - DIL * w, 16), :]
                    acc = t if acc is None else acc + t
                st.setdefault("o", []).append(acc)

            def scatter(lvl):
                st["o"] = _swap_level(st["o"], lvl)

            def store():
                res[b - 1] = jnp.concatenate(st["o"], axis=1)
                if b % g3 == 0:
                    o = jnp.concatenate([res[i] for i in range(b - g3, b)], axis=0)
                    for i, t in enumerate(_terms(_lhs_term, _grid(o, g3))):
                        _put(o_s, i, _ds((g0 + b // g3 - 1) * 8, 8, 8), slice(None), t)

            P = functools.partial
            stages = [[P(gather, p, lvl) for p in parts] for lvl in range(3)]
            if b:
                stages += [[P(scores, j) for j in range(8)] + [P(reduce, 1)], [P(reduce, 2)],
                           [softmax, P(spread, 1)], [P(spread, 2)],
                           [P(values, j) for j in range(8)] + [P(scatter, 0)], [P(scatter, 1)], [P(scatter, 2), store]]
            return stages

        blocks = [block(b) for b in range(na * g3 + 1)]
        order = sorted((b * skew + s, b, s) for b, stages in enumerate(blocks) for s in range(len(stages)))
        return [t for _, b, s in order for t in blocks[b][s]]

    def kern(x_h, wqkv_h, wo_h, wg_h, wu_h, wd_h, out_h,
             x_s, xa_s, xc_s, xd_s, qkv_s, st_s, o_s, y_s, wqkv_s, wo_s, wg_s, wu_s, wd_s,
             bq_s, bo_s, bg_s, bd_s,
             sx, sqkv, swo, sg, su, sd, so, idx_s):
        def x_cp(t):
            r = _ds(t * tm1, tm1, tm1)
            return pltpu.make_async_copy(x_h.at[r, :], x_s.at[r, :], sx.at[t])

        def qkv_cp(c):
            return pltpu.make_async_copy(wqkv_h.at[:, _ds(c * D, D, D)], wqkv_s.at[c], sqkv.at[c])

        def ffn_cps(c):
            r = _ds(c * fc, fc, fc)
            return (pltpu.make_async_copy(wg_h.at[:, r], wg_s.at[c], sg.at[c]),
                    pltpu.make_async_copy(wu_h.at[:, r], wu_s.at[c], su.at[c]),
                    pltpu.make_async_copy(wd_h.at[r, :], wd_s.at[c], sd.at[c]))

        wo_cp = pltpu.make_async_copy(wo_h, wo_s, swo.at[0])

        def out_cp(t):
            r = _ds(t * rb3, rb3, rb3)
            return pltpu.make_async_copy(x_s.at[r, :], out_h.at[r, :], so.at[t])

        def norm_tasks(s, chain=0):
            gm = max(g1, g2)
            tasks = []
            for i in range(sb // gm // lnb):
                rows = []

                def norm(q, i=i, rows=rows):
                    rows.append(_layernorm(x_s[_ds(s * sb + q * (sb // gm) + i * lnb, lnb, lnb), :]))
                    if chain and (i * gm + q + 1) % chain == 0:
                        x_s[_ds(idx_s[0], 16, 16), 0:128] = rows[-1][:, 0:128].astype(bf16)

                def sums(g, ref, e, col, i=i, rows=rows):
                    blocks = [[v[:, j * (D // g) + col:j * (D // g) + col + 128] for j in range(g)]
                              for v in rows[e::gm // g]]
                    off = (s * (sb // g) + e * (sb // gm) + i * lnb) // 2
                    for n, v in enumerate(_terms(_lhs_term, blocks)):
                        _put(ref, n, _ds(off, lnb // 2, 8), pl.ds(col, 128), v)

                tasks += [functools.partial(norm, q) for q in range(gm)]
                for g, ref in [(g2, xa_s)] + ([(g1, xd_s)] if g1 != g2 else []):
                    tasks += [functools.partial(sums, g, ref, e, col)
                              for e in range(gm // g) for col in range(0, D // g, 128)]
            return tasks

        def rhs_tasks(srcs, shape, level, n, dst, flip=()):
            g = 2 ** level
            kb, nb = shape[0] // g, shape[1] // g
            per = 7 ** max(level - 1, 0)
            cw = min(nb, 256)
            br = bsr * 128 // cw

            def task(si, r, col):
                jj = (lambda j: g - 1 - j) if si in flip else (lambda j: j)
                raw = lambda i, j: srcs[si](pl.ds(i * kb + r, br), pl.ds(jj(j) * nb + col, cw))
                if level == 0 or (level == 1 and n < 2):
                    vs = [raw(n, n)]
                elif cw == 128:
                    vs = _outer_terms(_rhs_term, lambda i, j: _unpack(_pack(raw(i, j))).astype(f32), level, n)
                else:
                    vs = _outer_terms(_rhs_term, lambda i, j: raw(i, j).astype(f32), level, n)
                for m, v in enumerate(vs):
                    _put(dst, n * per + m, pl.ds(r // 2, br // 2), pl.ds(si * nb + col, cw), v)

            return [functools.partial(task, si, r, col)
                    for col in range(0, nb, cw) for si in range(len(srcs)) for r in range(0, kb, br)]

        def phase1(it, _):
            t, part = it // 3, it % 3
            pl.when(it < 3)(lambda: qkv_cp(part).wait())
            pl.when((it % xe == 1) & (it < xe * (n1 - 1)))(lambda: x_cp(it // xe + 1).wait())
            pl.when(it == 0)(lambda: qkv_cp(2).start())
            pl.when((it % xe == 0) & (it < xe * (n1 - 1)))(lambda: x_cp(it // xe + 1).start())
            pl.when(it == 2)(lambda: wo_cp.start())
            for cp in ffn_cps(0):
                pl.when(it == 3)(lambda cp=cp: cp.start())
            rows, per, dq = tm1 // g1, 7 ** l1, D // g1
            sub = 7 ** max(l1 - 1, 0)
            bg = _Tasks()
            src = xa_s if g1 == g2 else xd_s

            def copy(n, r):
                xc_s[it % 2, n, r:r + 16, :] = src[n, _ds(t * (rows // 2) + r, 16, 16), :]

            def pre_tasks(m):
                return (rhs_tasks([lambda r, cc: wqkv_s[part, r, cc]], (D, D), l1, m, bq_s)
                        + [functools.partial(copy, n, r)
                           for n in range(m * sub, (m + 1) * sub) for r in range(0, rows // 2, 16)])

            nrb = rows // rb1
            steps = per * (dq // nt1) * nrb
            pending = bg.add(pre_tasks(0), 1)
            for rb in range(nrb):
                for col in range(0, dq, nt1):
                    def prod(n, col=col):
                        nonlocal pending
                        if rb == 0 and col == 0 and n % sub == 0:
                            bg.finish(pending)
                            if n + sub < per:
                                pending = bg.add(pre_tasks(n // sub + 1), sub)
                            else:
                                s0 = jnp.minimum(tm1 // sb - nls + it * nls, S // sb - nls)
                                left = max(int(lf * (steps - per)), 1)
                                bg.add([k for s in range(nls) for k in norm_tasks(s0 + s, lchain)], left)
                        y = _dot(_unpack(xc_s[it & 1, n, rb * rb1 // 2:(rb + 1) * rb1 // 2, :]),
                                 _unpack(bq_s[n, :, col:col + nt1]))
                        bg.step()
                        return y

                    def emit(i, j, v, col=col):
                        q = sb // g1
                        e = min(q, rb1)
                        for r in range(0, rb1, e):
                            rr = rb * rb1 + r
                            off = (rr // q) * sb + i * q + rr % q + PAD
                            _put(qkv_s, part, _ds((t * tm1 + off) // 2, e // 2, 8),
                                 pl.ds(j * dq + col, nt1), v[r:r + e])

                    _combine(prod, l1, emit)
            bg.finish()

        x_cp(0).start()
        qkv_cp(0).start()
        idx_s[0] = S

        def zero(i, _):
            y_s[:, _ds(i * 32, 32, 32), :] = jnp.zeros((y_s.shape[0], 32, y_s.shape[2]), f32)

        lax.fori_loop(0, y_s.shape[1] // 32, zero, None)
        x_cp(0).wait()
        qkv_cp(1).start()

        def norm_block(s, _):
            for task in norm_tasks(s):
                task()

        lax.fori_loop(0, tm1 // sb, norm_block, None)
        if only in (None, 1):
            lax.fori_loop(0, 3 * n1, phase1, None)

        for p in (1, 2):
            first = _unpack(qkv_s[p, PAD // 2:PAD, :]).astype(f32)[0:1]
            qkv_s[p, 0:PAD // 2, :] = _pack(jnp.broadcast_to(first, (PAD, D)))

        def phase2(it, _):
            c, hf = (it // nh, it % nh) if nh > 1 else (it, 0)
            for cp in ffn_cps(c):
                pl.when(hf == 0)(lambda cp=cp: cp.wait())
            for cp in ffn_cps(jnp.minimum(c + 1, n2 - 1)):
                pl.when((hf == 0) & (c + 1 < n2))(lambda cp=cp: cp.start())

            bg = _Tasks()
            rows = nsb2 * sb // g2
            nb = th // (nsb2 * sb)
            per = 7 ** l2
            sub = 7 ** max(l2 - 1, 0)
            fq, dq = fc // g2, D // g2
            w2 = min(nt2, fq)
            wd = min(ntd, dq)
            ngu, ndn = per * (fq // w2) * 2, per * (dq // wd)
            a0 = jnp.minimum(it * na, S // ag - na)
            gu_tasks = lambda n: rhs_tasks(
                [lambda r, cc: wg_s[c, r, cc], lambda r, cc: wu_s[c, r, cc]], (D, fc), l2, n, bg_s, (1,))
            pending = bg.add(gu_tasks(0), 1)
            hs, hq = [None] * nb, [None] * nb
            for rb in range(nb + 1):
                if rb < nb:
                    h = {}
                    for col in range(0, fq, w2):
                        gu = [{}, {}]
                        for si in range(2):
                            def prod(n, si=si, col=col):
                                nonlocal pending
                                if rb == 0 and col == 0 and si == 0 and n % sub == 0:
                                    bg.finish(pending)
                                    if n + sub < per:
                                        pending = bg.add(gu_tasks(n // sub + 1), sub)
                                    else:
                                        pending = bg.add(
                                            [t for m in range(per // sub) for t in rhs_tasks(
                                                [lambda r, cc: wd_s[c, r, cc]], (fc, D), l2, m, bd_s)], ngu)
                                y = _dot(_unpack(xa_s[n, _ds((hf * (th // g2) + rb * rows) // 2, rows // 2, rows // 2), :]),
                                         _unpack(bg_s[n, :, si * fq + col:si * fq + col + w2]))
                                bg.step()
                                return y

                            def emit(i, j, v, si=si, col=col):
                                if si == 0:
                                    gu[0][i, j] = v
                                else:
                                    j = g2 - 1 - j
                                    h[i, j, col] = _geglu2(gu[0][i, j], v)

                            _combine(prod, l2, emit)
                    parts = {}

                    def sums(col, e, r, h=h, parts=parts):
                        blocks = [[h[i, j, col][r:r + 16, e:e + 128] for j in range(g2)] for i in range(g2)]
                        for n, v in enumerate(_terms(_lhs_term, blocks)):
                            parts[n, col + e, r] = v

                    hq[rb] = bg.add([functools.partial(sums, col, e, r) for r in range(0, rows, 16)
                                     for col in range(0, fq, w2) for e in range(0, w2, 128)],
                                    max(ndn * 3 // 4, 1) if rb else ngu // 2)
                    hs[rb] = parts
                if rb == 0 and attn:
                    bg.add(attention_tasks(a0, qkv_s, st_s, o_s),
                           int(af * (nb - 1) * (ngu + ndn)))
                if rb > 0:
                    bg.finish(pending, hq[rb - 1])
                    parts = hs[rb - 1]
                    r = _ds(hf * (th // g2) + (rb - 1) * rows, rows, rows)
                    lhs = [jnp.concatenate([jnp.concatenate([parts[n, e, q] for e in range(0, fq, 128)], axis=1)
                                            for q in range(0, rows, 16)], axis=0).astype(bf16) for n in range(per)]
                    for col in range(0, dq, wd):
                        def prod(n, col=col):
                            y = _dot(lhs[n], _unpack(bd_s[n, :, col:col + wd]))
                            bg.step()
                            return y

                        if yacc:
                            for m in range(7):
                                def emit(i, j, v, m=m, col=col):
                                    y_s[m * g2 // 2 + i, r, j * dq + col:j * dq + col + wd] += v

                                _combine(prod, l2 - 1, emit, m * sub)
                        else:
                            def emit(i, j, v, col=col):
                                y_s[i, r, j * dq + col:j * dq + col + wd] += v

                            _combine(prod, l2, emit)
            bg.finish()

        if only in (None, 2):
            lax.fori_loop(0, n2 * nh, phase2, None)
        wo_cp.wait()

        def phase3(t, _):
            bg = _Tasks()
            rows, per, dq = rb3 // g3, 7 ** l3, D // g3
            wo_tasks = lambda n: rhs_tasks([lambda r, cc: wo_s[r, cc]], (D, D), l3, n, bo_s)
            pending = bg.add(wo_tasks(0), 1)

            def gate(o, c0):
                q = sb // g2
                yq, r = (o % sb) // q, _ds(t * (tm3 // g2) + (o // sb) * q + o % q, 16, 16)
                if yacc:
                    a, i, b, cc = yq // (g2 // 2), yq % (g2 // 2), c0 // (D // 2), c0 % (D // 2)
                    m = lambda n: y_s[n * g2 // 2 + i, r, cc:cc + 128]
                    y = ((lambda: m(3) - m(1) + m(4) + m(6), lambda: m(2) + m(1)),
                         (lambda: m(0) + m(3), lambda: m(2) - m(0) + m(4) + m(5)))[a][b]()
                else:
                    y = y_s[yq, r, c0:c0 + 128]
                y = y * 0.25
                return y * jnp.tanh(y) + y

            for rb in range(tm3 // rb3):
                for col in range(0, dq, nt3):
                    def prod(n, col=col):
                        nonlocal pending
                        if rb == 0 and col == 0:
                            bg.finish(pending)
                            if n + 1 < per:
                                pending = bg.add(wo_tasks(n + 1), 1)
                        y = _dot(_unpack(o_s[n, _ds((t * (tm3 // g3) + rb * rows) // 2, rows // 2, rows // 2), :]),
                                 _unpack(bo_s[n, :, col:col + nt3]))
                        bg.step()
                        return y

                    def emit(i, j, v, col=col):
                        c0 = j * dq + col
                        for e in range(rows // 16):
                            o = rb * rb3 + (e * g3 + i) * 16
                            g = jnp.concatenate([gate(o, c0 + k) for k in range(0, nt3, 128)], axis=1)
                            r = _ds(t * tm3 + o, 16, 16)
                            x_s[r, c0:c0 + nt3] = (
                                x_s[r, c0:c0 + nt3].astype(f32) + v[e * 16:(e + 1) * 16] * g).astype(bf16)

                    _combine(prod, l3, emit)
                out_cp(t * (tm3 // rb3) + rb).start()

        if only in (None, 3):
            lax.fori_loop(0, n3, phase3, None)
        for t in range(S // rb3):
            out_cp(t).wait()

    def fn(A_x, A_wqkv, A_wo, B_x, B_w_gate, B_w_up, B_w_down):
        any_spec = pl.BlockSpec(memory_space=pl.ANY)
        out = pl.pallas_call(
            kern,
            in_specs=[any_spec] * 6,
            out_specs=any_spec,
            out_shape=jax.ShapeDtypeStruct((S, D), bf16),
            scratch_shapes=[
                pltpu.VMEM((S + 16, D), bf16),
                pltpu.VMEM((7 ** l2, S // g2 // 2, D // g2), u32),
                pltpu.VMEM((2, 7 ** l1, tm1 // g1 // 2, D // g1), u32),
                pltpu.VMEM((7 ** l1, S // g1 // 2, D // g1) if g1 != g2 else (8, 128), u32),
                pltpu.VMEM((3, (S + PAD) // 2, D), u32),
                pltpu.VMEM((3, 8, na * ag + PAD, 128), f32),
                pltpu.VMEM((7 ** l3, S // g3 // 2, D // g3), u32),
                pltpu.VMEM((7 * g2 // 2, S // g2, D // 2) if yacc else (g2, S // g2, D), f32),
                pltpu.VMEM((3, D, D), bf16),
                pltpu.VMEM((D, D), bf16),
                pltpu.VMEM((n2, D, fc), bf16),
                pltpu.VMEM((n2, D, fc), bf16),
                pltpu.VMEM((n2, fc, D), bf16),
                pltpu.VMEM((7 ** l1, D // g1 // 2, D // g1), u32),
                pltpu.VMEM((7 ** l3, D // g3 // 2, D // g3), u32),
                pltpu.VMEM((7 ** l2, D // g2 // 2, 2 * fc // g2), u32),
                pltpu.VMEM((7 ** l2, fc // g2 // 2, D // g2), u32),
                pltpu.SemaphoreType.DMA((n1,)),
                pltpu.SemaphoreType.DMA((3,)),
                pltpu.SemaphoreType.DMA((1,)),
                pltpu.SemaphoreType.DMA((n2,)),
                pltpu.SemaphoreType.DMA((n2,)),
                pltpu.SemaphoreType.DMA((n2,)),
                pltpu.SemaphoreType.DMA((S // rb3,)),
                pltpu.SMEM((1,), jnp.int32),
            ],
            compiler_params=pltpu.CompilerParams(vmem_limit_bytes=126 << 20, flags=flags),
        )(A_x.reshape(S, D), A_wqkv, A_wo, B_w_gate, B_w_up, B_w_down)
        return out.reshape(1, S, D)

    return fn


@jax.jit
def pallas_recurrent_scan__sliding_local_dilated__geglu_ffn__prompt_kernel(
    A_x, A_wqkv, A_wo, B_x, B_w_gate, B_w_up, B_w_down
):
    return make(th=2048, tm3=512, lchain=0, skew=4, rb3=512, flags={'XLA_TPU_EVENLY_DISTRIBUTE_CRITICAL_NODES': True})(A_x, A_wqkv, A_wo, B_x, B_w_gate, B_w_up, B_w_down)
```

```python
import functools
import math

import jax
import jax.numpy as jnp
from jax import lax
import jax.experimental.pallas as pl
import jax.experimental.pallas.tpu as pltpu

S, D, F = 2048, 1024, 3584
DH, W, DIL = 32, 8, 2
PAD = 16
NP = 49
NZ = 28
GT = 64
NG = S // GT
CW = 512
NC = F // CW
LOG2E = math.log2(math.e)
C0 = math.sqrt(2.0 / math.pi)
XS = (C0 * 0.044715) ** (1.0 / 3.0)
f32, bf16, u32, i32 = jnp.float32, jnp.bfloat16, jnp.uint32, jnp.int32
P = functools.partial


def _pack(v):
    return pltpu.bitcast(v.astype(bf16), u32)


def _unpack(v):
    return pltpu.bitcast(v, bf16)


def _ds(start, size, align):
    if isinstance(start, int):
        return pl.ds(start, size)
    return pl.ds(pl.multiple_of(start, align), size)


def _tile(v, j):
    return v[:, j * 128:(j + 1) * 128]


def _lane_bit(shape, bit):
    return (lax.broadcasted_iota(i32, shape, 1) & bit) == 0


def _sum(vs):
    return functools.reduce(lambda a, b: a + b, vs)


class _Pace:
    def __init__(self, zero=None, lag=256):
        self.zero, self.lag = zero, lag
        self.tok, self.time, self.tiles, self.due, self.queues = None, 0, 0, [], []

    def add(self, tasks, cycles):
        if tasks:
            steps = (None for fn, _ in tasks for _ in fn())
            self.queues.append([steps, sum(n for _, n in tasks), cycles, 0, 0])

    def finish(self):
        for q in self.queues:
            for _ in q[0]:
                pass
        self.queues = []

    def dot(self, lhs, rhs):
        rows, nk = 2 * lhs.shape[0], lhs.shape[1] // 128
        t0 = self.tiles // 4 * rows
        part = range(rows * (self.tiles % 4) // 4, rows * (self.tiles % 4 + nk) // 4)
        self.tiles += nk
        if self.due and self.due[0][0] < t0 + part.stop:
            col = [lhs[r:r + 8, 0:128] for r in range(0, rows // 2, 8)]
            while self.due and self.due[0][0] < t0 + part.stop:
                t, tok = self.due.pop(0)
                i = max(t - t0, 0) // 16
                col[i] = jnp.where(self.zero == 0, col[i], pltpu.bitcast(tok, u32))
            lhs = jnp.concatenate([jnp.concatenate(col, axis=0)] + [_tile(lhs, j) for j in range(1, nk)], axis=1)
        y = jnp.dot(_unpack(lhs), rhs, preferred_element_type=f32)
        for r in part[::8]:
            self.tok, self.time = y[r:r + 8], t0 + r
            for q in self.queues:
                q[3] += 8
                while q[4] < min(q[1], q[1] * q[3] // q[2]):
                    q[4] += 1
                    next(q[0], None)
        return y

    def const(self, c, rows):
        if self.zero is None or self.tok is None:
            return c
        return jnp.concatenate([jnp.where(self.zero == 0, c, self.tok)] * (rows // 8), axis=0)

    def gate(self, v):
        if self.zero is None or self.tok is None:
            return v
        return jnp.where(self.zero == 0, v, jnp.concatenate([self.tok] * (v.shape[0] // 8), axis=0))

    def open(self, ref):
        if self.zero is not None and self.tok is not None:
            if ref.dtype == bf16:
                ref[self.zero, ref.shape[1] - 16:, 0:128] = pltpu.bitcast(self.tok, bf16)
            else:
                ref[ref.shape[0] - 1 + self.zero, 0:8, 0:128] = pltpu.bitcast(self.tok, ref.dtype)
        return ref

    def done(self, v, extra=0):
        if self.zero is not None:
            self.due.append((self.time + self.lag + extra, v[-8:]))
            self.due.sort(key=lambda d: d[0])
        return v

    def stored(self, ref, n, rows, cols=pl.ds(0, 128), extra=0):
        if self.zero is not None:
            self.done(ref[n + self.zero, rows, cols], extra)


LHS, RHS = (6, 3, 0, 2, 1, 4, 5), (6, 0, 5, 4, 2, 1, 3)


def _basis(scaled, x11, x12, x21, x22):
    h = x21 if scaled else x21 * 0.5
    p = x11 + h
    return [x11 + x22, p, h + x22, (p + x22 + x12) * 0.5 if scaled else (p + x22) * 0.5 + x12]


def _unbasis(half, scaled, z0, z1, z2, z3):
    h = z0 * half
    e = z3 + h
    if scaled:
        return [e + z2, z2 + h + z1, h, e + z1]
    return [e + z2, (z2 + h + z1) * 0.5, z0, e + z1]


def _operands(side, block, pc, ref, rows, col, base=0, scaled=False, src=None):
    def quad(a, b):
        if src is not None:
            pc.open(src)
        return _basis(scaled, *[block(2 * a + n // 2, 2 * b + n % 2) for n in range(4)])

    def put(k, x):
        t, p, q, r = x
        for n, v in zip(side, (t, p, q, r, t - p, q - t, r - t)):
            ref[pl.ds(base + 7 * side[k] + n, 1), rows, pl.ds(col, 128)] = _pack(v[None])
        pc.stored(ref, base + 7 * side[k], rows, pl.ds(col, 128))

    def run():
        h = quad(1, 0) if scaled else [v * 0.5 for v in quad(1, 0)]
        yield
        x11 = quad(0, 0)
        put(1, [a + b for a, b in zip(x11, h)])
        yield
        put(5, [b - a for a, b in zip(x11, h)])
        yield
        x22 = quad(1, 1)
        t = [a + b for a, b in zip(x11, x22)]
        put(0, t)
        yield
        put(2, [a + b for a, b in zip(x22, h)])
        yield
        put(4, [a - b for a, b in zip(x22, h)])
        yield
        r = [(a + b + c) * 0.5 if scaled else (a + b) * 0.5 + c for a, b, c in zip(t, h, quad(0, 1))]
        put(3, r)
        yield
        put(6, [a - b for a, b in zip(r, t)])
        yield

    return run, 8


def _products(prod, emit, odd=0):
    for o in range(7):
        m = lambda i: prod(7 * o + i)
        early = (o + odd) % 2
        t = m(6) if early else None
        a = m(0)
        t = t - a if early else a
        emit(4 * o, a + m(1))
        a = m(2)
        t = t - a if early else t + a
        emit(4 * o + 1, a + m(3))
        a = m(4)
        t = t + a if early else a - t
        emit(4 * o + 2, m(5) - a)
        emit(4 * o + 3, t if early else t + m(6))


def _result(pc, ref, rows, cols, scaled=False):
    x = []
    for k in range(4):
        if k % 2 == 0:
            pc.open(ref)
        m = [ref[4 * o + k, rows, cols] for o in range(7)]
        x.append(_unbasis(0.5, scaled, m[0] + m[1], m[2] + m[3], m[5] - m[4], m[4] + m[6] - m[0] - m[2]))
        if k % 2:
            yield
    half = pc.const(0.5, x[0][0].shape[0])
    x = [_unbasis(half, scaled, *col) for col in zip(*x)]
    yield
    return [[x[2 * (i // 2) + j // 2][2 * (i % 2) + j % 2] for j in range(4)] for i in range(4)]


def _skewed(units, skew=1):
    order = sorted((u * skew + s, u, s) for u, st in enumerate(units) for s in range(len(st)))
    return [t for _, u, s in order for t in units[u][s]]


def _mix(*lists):
    keyed = []
    for i, ts in enumerate(lists):
        total, at = sum(n for _, n in ts), 0
        for t in ts:
            keyed.append(((at + t[1] / 2) / total, i, t))
            at += t[1]
    return [t for _, _, t in sorted(keyed, key=lambda k: k[:2])]


def make(g0=4, g1=8, g2=8, g3=4, n3=4, skew=1, attn=True, only=None, flags=None,
         d0=256, d1=256, d2=256, d3=256, nbn=8, nbd=16, xl=128, qs=4, cuts=((0, 44, 64), (0, 34, 64)),
         aw=(1, 2, 2, 5, 1, 6, 6, 2, 2, 1, 4, 4)):
    NX = NG // g0
    na = -(-NG // NC)
    ALL = slice(None)

    def attention_tasks(a0, qkv_s, san, r_s, o_s, pc):
        def block(b):
            r0 = pl.multiple_of(a0 * GT + b * 16, 16)
            a_s = san[b % len(san)]

            def scores():
                st = [None] * W
                for j in range(8):
                    q = pc.gate(qkv_s[j, pl.ds(r0 + PAD, 16), :])
                    for w in range(W):
                        t = q * qkv_s[8 + j, pl.ds(r0 + (PAD - DIL * w), 16), :]
                        st[w] = t if j == 0 else st[w] + t
                    pc.done(st[W - 1])
                    yield
                for w in range(W):
                    a_s[w] = st[w] + pltpu.roll(st[w], 127, 1)
                pc.stored(a_s, 0, pl.ds(0, 8), extra=xl)

            def reduce():
                pc.open(a_s)
                for w in range(W):
                    a_s[W + w] = a_s[w] + pltpu.roll(a_s[w], 126, 1)
                pc.stored(a_s, W, pl.ds(0, 8), extra=xl)
                yield

            def softmax():
                pc.open(a_s)
                row = lax.broadcasted_iota(i32, (16, 128), 0) + r0
                logits = []
                for w in range(W):
                    t = a_s[W + w] * (DH ** -0.5 * LOG2E / XS ** 2)
                    if b == 0 and w:
                        t = jnp.where(row >= DIL * w, t, -1e9 * LOG2E)
                    logits.append(t)
                m = functools.reduce(jnp.maximum, logits)
                yield
                m = pc.gate(m)
                e = [jnp.exp2(t - m) for t in logits]
                inv = (1.0 / XS) / _sum(e)
                yield
                inv = pc.gate(inv)
                for w in range(W):
                    t = e[w] * inv
                    a_s[2 * W + w] = jnp.where(_lane_bit((16, 128), 1), t, pltpu.roll(t, 1, 1))
                pc.stored(a_s, 2 * W, pl.ds(0, 8), extra=xl)
                yield

            def spread():
                pc.open(a_s)
                for w in range(W):
                    t = a_s[2 * W + w]
                    a_s[3 * W + w] = jnp.where(_lane_bit((16, 128), 2), t, pltpu.roll(t, 2, 1))
                pc.stored(a_s, 3 * W, pl.ds(0, 8), extra=xl)
                yield

            def values():
                for j in range(8):
                    pc.open(a_s)
                    r_s[b % 4 * 8 + j] = pc.done(_sum(
                        [a_s[3 * W + w] * qkv_s[16 + j, pl.ds(r0 + (PAD - DIL * w), 16), :] for w in range(W)]))
                    yield

            store = [_operands(LHS, lambda i, j, e=e: r_s[i * 8 + 2 * j + e], pc, o_s,
                               _ds((a0 + b // 4) * 8, 8, 8), e * 128, src=r_s) for e in range(2)]
            return [[(scores, 8)], [(reduce, 1)], [(softmax, 3)], [(spread, 1)],
                    [(values, 8)] + (store if b % 4 == 3 else [])]

        return _skewed([block(b) for b in range(na * 4)], skew)

    def rhs_task(pc, src, load, dst, rows, col, base=0, flip=0):
        load = functools.cache(load)
        return _operands(RHS, lambda i, j: _tile(load(i, (j ^ flip) // 2), (j ^ flip) % 2), pc, dst, rows, col, base, src=src)

    def stacked(ref, n):
        return jnp.concatenate([ref[n, :, k:k + 128] for k in (0, 128)], axis=0)

    def run(tasks):
        for fn, _ in tasks:
            for _ in fn():
                pass

    def kern(x_h, wqkv_h, wo_h, wg_h, wu_h, wd_h, out_h,
             x_s, xa_s, qkv_s, y_s, wg_s, wu_s, wd_s, wo_s, ba_s, bb_s, bd_s, bo_s, z_s,
             sx, sqkv, swo, sg, su, sd, so, zero_s):
        free = _Pace()
        for i in range(4):
            zero_s[i] = 0
        pace = lambda d: _Pace(zero_s[0], d) if d >= 0 else _Pace()

        def g_cp(c):
            return pltpu.make_async_copy(wg_h.at[:, _ds(c * CW, CW, CW)], wg_s.at[c & 1, pl.ds(0, D)], sg.at[c])

        def u_cp(c):
            return pltpu.make_async_copy(wu_h.at[:, _ds(c * CW, CW, CW)], wu_s.at[c & 1, pl.ds(0, D)], su.at[c])

        def dn_cp(c):
            return pltpu.make_async_copy(wd_h.at[_ds(c * CW, CW, CW), :], wd_s.at[c & 1, pl.ds(0, CW)], sd.at[c])

        wo_cp = pltpu.make_async_copy(wo_h, wo_s.at[0, pl.ds(0, D)], swo.at[0])

        def project(wqkv_s, n_s, sw_s):
            def x_cp(t):
                r = _ds(t * g0 * GT, g0 * GT, g0 * GT)
                return pltpu.make_async_copy(x_h.at[r, :], x_s.at[r, :], sx.at[t])

            def qkv_cp(p):
                return pltpu.make_async_copy(wqkv_h.at[:, pl.ds(p * D, D)], wqkv_s.at[p, pl.ds(0, D)], sqkv.at[p])

            g0_cp = pltpu.make_async_copy(wg_h.at[:, pl.ds(0, D)], wqkv_s.at[3, pl.ds(0, D)], sqkv.at[3])

            def norm_tasks(g, n, pc):
                def group(g, m_s):
                    rows = lambda i: _ds(g * GT + i * 16, 16, 16)
                    mean = lambda v: jnp.broadcast_to(jnp.sum(pc.done(v), axis=1, keepdims=True) * (1.0 / D), v.shape)

                    def center():
                        for i in range(4):
                            x = x_s[rows(i), :].astype(f32)
                            m_s[32 + i] = mean(_sum([_tile(x, j) for j in range(8)]))
                            yield

                    def scale():
                        for i in range(4):
                            x, m = x_s[rows(i), :].astype(f32), pc.open(m_s)[32 + i]
                            x = [_tile(x, j) - m for j in range(8)]
                            for j in range(8):
                                m_s[8 * i + j] = x[j]
                            m_s[36 + i] = lax.rsqrt(mean(_sum([v * v for v in x])) + 1e-5) * XS
                            yield
                            yield

                    return [[(center, 4)], [(scale, 8)],
                            [_operands(LHS, lambda i, j, e=e: m_s[8 * i + 2 * j + e] * m_s[36 + i], pc,
                                       xa_s, _ds(g * 8, 8, 8), e * 128, src=m_s) for e in range(2)]]

                return _skewed([group(g + i, n_s[i % 3]) for i in range(n)])

            def qkv_tasks(pc, p, halves, units, plain=None):
                def unit(k, r, t_s):
                    def swap(lvl):
                        sh = 4 << lvl
                        lo = _lane_bit((8, 128), sh)
                        keep = [lo, ~lo] if plain is None else [lo | plain, ~lo | plain]
                        pc.open(t_s if lvl < 2 else wqkv_s)
                        for i in range(4):
                            if lvl == 2:
                                get = lambda c: _pack(wqkv_s[p, _ds(i * 256 + k * 128 + r, 16, 16), c * 128:(c + 1) * 128])
                            else:
                                get = lambda c: t_s[32 * (lvl + 1) + 8 * i + c]
                            get = functools.cache(get)
                            for h, _ in halves:
                                for c in range(4 * h, 4 * h + 4):
                                    t_s[32 * lvl + 8 * i + c] = jnp.where(
                                        keep[c >> lvl & 1], get(c),
                                        pltpu.roll(get(c ^ (1 << lvl)), 128 - sh if c >> lvl & 1 else sh, 1))
                        pc.stored(t_s, 32 * lvl + 4 * halves[0][0], ALL, extra=xl)
                        yield

                    return [[(P(swap, lvl), 1)] for lvl in (2, 1, 0)] + [[
                        _operands(RHS, lambda i, j, h=h: _unpack(t_s[8 * i + 4 * h + j]).astype(f32), pc,
                                  dst, _ds(r // 2, 8, 8), k * 128, src=t_s) for h, dst in halves]]

                return _skewed([unit(k, r, sw_s[u % 4]) for u, (k, r) in enumerate(units)])

            def chunk(pc, seg, tile0, g, ng, lhs, rhs):
                def emit(n, v):
                    z_s[seg % 2][n, 0:ng * 16, :] = v

                _products(lambda n: pc.dot(lhs(n), _unpack(rhs(n))), emit, seg)

                def put(pc, r):
                    res = yield from _result(pc, z_s[seg % 2], pl.ds(r, 8), ALL)
                    rows = lambda i: _ds((g + r // 16) * GT + i * 16 + r % 16 + PAD, 8, 8)
                    for n in range(16):
                        qkv_s[tile0 + n % 4, rows(n // 4), :] = res[n // 4][n % 4]
                    pc.stored(qkv_s, tile0, rows(0))

                return lambda pc: [(P(put, pc, r), 3) for r in range(0, ng * 16, 8)]

            for t in range(2):
                x_cp(t).start()

            def zero(i, _):
                y_s[0:NZ, _ds(i * 8, 8, 8), :] = jnp.zeros((NZ, 8, D // 4), f32)

            lax.fori_loop(0, S // 4 // 8, zero, None)

            def head(t, _):
                pl.when(t + 2 < NX)(lambda: x_cp(jnp.minimum(t + 2, NX - 1)).start())
                pl.when(t == qs)(lambda: qkv_cp(0).start())
                x_cp(t).wait()
                run(norm_tasks(t * g0, g0, free))

            lax.fori_loop(0, NX, head, None)
            qkv_cp(0).wait()
            qkv_cp(1).start()
            lax.fori_loop(0, 4, lambda r, _: run(qkv_tasks(
                free, 0, [(0, ba_s)], [(k, r * 32 + i) for k in range(2) for i in (0, 16)])), None)

            def phase1(it, _):
                p, hf = it >> 1, it & 1
                pl.when(it == 1)(lambda: qkv_cp(2).start())
                pl.when(it == 3)(lambda: g0_cp.start())
                for cp in (wo_cp, u_cp(0), dn_cp(0), g_cp(1)):
                    pl.when(it == 4)(lambda: cp.start())
                pl.when(it == 1)(lambda: qkv_cp(1).wait())
                pl.when(it == 3)(lambda: qkv_cp(2).wait())
                pl.when(it == 5)(lambda: g0_cp.wait())
                pc = pace(d1)
                z = [zero_s[i] & 1 for i in range(4)]
                nxt = (it + 1) >> 1
                units = [(k, r) for k in range(2) for r in range(0, 128, 16)]
                nb = NG // 2 // g1
                seg = NP * g1 * 8
                prep = [qkv_tasks(pc, p, [(1, bb_s)], units), qkv_tasks(pc, nxt, [(0, ba_s)], units, nxt == 3)]
                puts = lambda pc: []
                for s, b_ref in enumerate((ba_s, bb_s)):
                    for rb in range(nb):
                        i, g = s * nb + rb, hf * (NG // 2) + rb * g1
                        cut = [len(prep[s]) * c // 64 for c in cuts[s]]
                        pc.add(_mix(puts(pc), prep[s][cut[rb]:cut[rb + 1]]), seg - (320 if rb == nb - 1 else 0))
                        puts = chunk(pc, i, 8 * p + 4 * s, g, g1, lambda n: xa_s[n, _ds(g * 8, g1 * 8, g1 * 8), :],
                                     lambda n: stacked(b_ref, n + z[rb]))
                        pc.finish()
                run(puts(free))

            if only in (None, 1):
                lax.fori_loop(0, 6, phase1, None)

        pl.run_scoped(project, pltpu.VMEM((4, D + 16, D), bf16),
                      [pltpu.VMEM((41, 16, 128), f32)] * 3, [pltpu.VMEM((97, 8, 128), u32)] * 4)
        wo_cp.wait()

        for j in range(8, 24):
            qkv_s[j, 0:PAD, :] = jnp.broadcast_to(qkv_s[j, PAD:PAD + 1, :], (PAD, 128))

        def mix(o_s, h_s, ha_s, zz_s, san, r_s):
            def phase2(c, _):
                nxt = jnp.minimum(c + 1, NC - 1)
                pl.when(c + 1 < NC)(lambda: u_cp(nxt).start())
                pl.when(c + 2 < NC)(lambda: g_cp(jnp.minimum(c + 2, NC - 1)).start())
                pl.when(c + 1 < NC)(lambda: dn_cp(nxt).start())
                u_cp(c).wait()
                dn_cp(c).wait()
                pl.when(c + 1 < NC)(lambda: g_cp(nxt).wait())
                pc = pace(d2)
                z = [zero_s[i] & 1 for i in range(4)]
                att = attention_tasks(jnp.minimum(c * na, NG - na), qkv_s, san, r_s, o_s, pc) if attn else []

                def up(rb, si):
                    def emit(n, v):
                        (z_s, zz_s)[rb % 2][si][n] = v

                    _products(lambda n: pc.dot(xa_s[n, rb * g2 * 8:(rb + 1) * g2 * 8, :],
                                               _unpack(stacked((ba_s, bb_s)[si], n + z[rb]))), emit, pc.tiles // 2)

                def down(rb):
                    for e in range(2):
                        def emit(n, v):
                            y_s[n, rb * g2 * 16:(rb + 1) * g2 * 16, e * 128:(e + 1) * 128] += v

                        _products(lambda n: pc.dot(stacked(ha_s[rb % 3], n + z[e + rb // 3 * 2]),
                                                   _unpack(bd_s[n + z[rb], :, e * 128:(e + 1) * 128])), emit, e)

                def act(rb, r):
                    g = yield from _result(pc, (z_s, zz_s)[rb % 2][0], pl.ds(r, 8), ALL, True)
                    u = yield from _result(pc, (z_s, zz_s)[rb % 2][1], pl.ds(r, 8), ALL)
                    for n in range(16):
                        i, j = n // 4, n % 4
                        s = 2.0 ** (j // 2 - i // 2 + j % 2 - i % 2)
                        t = pc.gate(g[i][j])
                        v = t * t if s == 1 else t * t * s ** -3
                        p = t * u[i][j ^ 3]
                        h_s[n, r:r + 8, :] = p * jnp.tanh(t * (v + C0 / XS / s)) + p
                        if j == 3:
                            pc.stored(h_s, n, pl.ds(r, 8))
                            yield

                def prep(w_s, slot, dst, flip):
                    return [rhs_task(pc, w_s, lambda i, h, r=k + r: w_s[slot, pl.ds(i * 256 + r, 16), pl.ds(h * 256, 256)].astype(f32),
                                     dst, pl.ds(r // 2, 8), k, 0, flip) for k in (0, 128) for r in range(0, 128, 16)]

                def out_task(u, e, j0):
                    def load(i, h):
                        lo = lax.broadcasted_iota(i32, (8, 256), 0) < 4
                        v = [wo_s[0, _ds((u & 1) * 512 + (u >> 1) * 32 + k * 128 + i * 8, 8, 8),
                                  pl.ds(e * CW + h * 256, 256)].astype(f32) for k in range(4)]
                        v = [jnp.where(lo, pltpu.roll(a, 4, 0), b) if j0 else jnp.where(lo, a, pltpu.roll(b, 4, 0))
                             for a, b in (v[:2], v[2:])]
                        return jnp.concatenate(v, axis=0)

                    return rhs_task(pc, wo_s, load, bo_s, _ds(j0 * 64 + u * 8, 8, 8), e * 128)

                bd = [rhs_task(pc, wd_s, lambda i, h, e=e, r=r: wd_s[c & 1, pl.ds(i * 128 + r, 16), pl.ds(e * CW + h * 256, 256)].astype(f32),
                               bd_s, pl.ds(r // 2, 8), e * 128) for e in range(2) for r in range(0, 128, 16)]
                bo = [out_task((2 * c + u) & 7, e, j0) for u in range(2) for e in range(2) for j0 in range(2)]
                A = lambda rb: [(P(act, rb, r), 10) for r in range(0, g2 * 16, 8)]
                H = lambda rb: [_operands(LHS, lambda i, j, e=e: h_s[4 * i + j, e * 16:(e + 1) * 16, :], pc, ha_s[rb % 3],
                                          pl.ds(e % (g2 // 2) * 8, 8), e // (g2 // 2) * 128, scaled=True, src=h_s)
                                for e in range(g2)]
                bu, bn = prep(wu_s, c & 1, bb_s, 3), prep(wg_s, nxt & 1, ba_s, 0)
                plan = [(P(up, 0, 0), bu, 1), (P(up, 0, 1), bd[:nbd], 0), (P(up, 1, 0), A(0), 0), (P(up, 1, 1), _mix(H(0), bd[nbd:]), 1),
                        (P(down, 0), A(1), 0), (P(up, 2, 0), H(1), 0), (P(up, 2, 1), bo, 0), (P(up, 3, 0), A(2), 0),
                        (P(up, 3, 1), H(2) + bn[:nbn], 0), (P(down, 1), A(3), 0), (P(down, 2), H(3), 1),
                        (P(down, 3), bn[nbn:], 1)]
                done = 0
                for i, (products, tasks, early) in enumerate(plan):
                    upto = len(att) * sum(aw[:i + 1]) // sum(aw)
                    pc.add(_mix(tasks, att[done:upto]), NP * g2 * 8 - 320 * early)
                    done = upto
                    products()
                    pc.finish()

            if only in (None, 2):
                lax.fori_loop(0, NC, phase2, None)

            def out_cp(t):
                r = _ds(t * g3 * GT, g3 * GT, g3 * GT)
                return pltpu.make_async_copy(x_s.at[r, :], out_h.at[r, :], so.at[t])

            def phase3(t, _):
                pc = pace(d3)
                z = [zero_s[i] & 1 for i in range(4)]
                nb = NG // g3 // n3
                outs = lambda pc: []
                for rb in range(nb):
                    tb = t * nb + rb
                    for e in range(2):
                        def gate(r, e=e, tb=tb):
                            y = yield from _result(pc, y_s, _ds(tb * g3 * 16 + r, 8, 8), pl.ds(e * 128, 128))
                            for n in range(16):
                                h = y[n // 4][n % 4] * pc.const(0.25 / XS ** 2, 8)
                                zz_s[e][n, r:r + 8, :] = h * jnp.tanh(h) + h
                                if n % 8 == 7:
                                    pc.stored(zz_s[e], n, pl.ds(r, 8))
                                    yield

                        def emit(n, v):
                            z_s[e][n, 0:g3 * 16, :] = v

                        pc.add(_mix(outs(pc), [(P(gate, r), 5) for r in range(0, g3 * 16, 8)]), NP * g3 * 8)
                        _products(lambda n: pc.dot(o_s[n + z[e], _ds(tb * g3 * 8, g3 * 8, g3 * 8), :],
                                                   _unpack(bo_s[n + z[rb % 2], :, e * 128:(e + 1) * 128])), emit, e)
                        pc.finish()

                        def out(pc, r, e=e, tb=tb):
                            s = yield from _result(pc, z_s[e], pl.ds(r, 8), ALL)
                            for i in range(4):
                                rows = _ds((tb * g3 + r // 16) * GT + i * 16 + r % 16, 8, 8)
                                if i % 2 == 0:
                                    pc.open(zz_s[e])
                                v = jnp.concatenate([s[i][j] * zz_s[e][4 * i + j, r:r + 8, :] for j in range(4)], axis=1)
                                v = x_s[rows, e * CW:(e + 1) * CW].astype(f32) + v
                                x_s[rows, e * CW:(e + 1) * CW] = v.astype(bf16)
                                pc.done(_tile(v, 3))
                                if i % 2:
                                    yield
                            if e and r + 8 == g3 * 16:
                                out_cp(tb).start()

                        outs = lambda pc, out=out: [(P(out, pc, r), 5) for r in range(0, g3 * 16, 8)]
                run(outs(free))

            if only in (None, 3):
                lax.fori_loop(0, n3, phase3, None)
            for t in range(NG // g3):
                out_cp(t).wait()

        pl.run_scoped(mix, pltpu.VMEM((NP, S // 8, D // 4), u32), pltpu.VMEM((17, g2 * 16, 128), f32),
                      [pltpu.VMEM((NP, g2 * 4, 256), u32)] * 3, [pltpu.VMEM((NZ + 1, g2 * 16, 128), f32)] * 2,
                      [pltpu.VMEM((4 * W + 1, 16, 128), f32)] * 5, pltpu.VMEM((33, 16, 128), f32))

    def fn(A_x, A_wqkv, A_wo, B_x, B_w_gate, B_w_up, B_w_down):
        any_spec = pl.BlockSpec(memory_space=pl.ANY)
        out = pl.pallas_call(
            kern,
            in_specs=[any_spec] * 6,
            out_specs=any_spec,
            out_shape=jax.ShapeDtypeStruct((S, D), bf16),
            scratch_shapes=[
                pltpu.VMEM((S, D), bf16),
                pltpu.VMEM((NP, S // 8, D // 4), u32),
                pltpu.VMEM((24, S + PAD, 128), f32),
                pltpu.VMEM((NZ + 1, S // 4, D // 4), f32),
                pltpu.VMEM((2, D + 16, CW), bf16),
                pltpu.VMEM((2, D + 16, CW), bf16),
                pltpu.VMEM((2, CW + 16, D), bf16),
                pltpu.VMEM((1, D + 16, D), bf16),
                pltpu.VMEM((NP, 64, 256), u32),
                pltpu.VMEM((NP, 64, 256), u32),
                pltpu.VMEM((NP, 64, 256), u32),
                pltpu.VMEM((NP, 128, 256), u32),
                [pltpu.VMEM((NZ + 1, g2 * 16, 128), f32)] * 2,
                pltpu.SemaphoreType.DMA((NX,)),
                pltpu.SemaphoreType.DMA((4,)),
                pltpu.SemaphoreType.DMA((1,)),
                pltpu.SemaphoreType.DMA((NC,)),
                pltpu.SemaphoreType.DMA((NC,)),
                pltpu.SemaphoreType.DMA((NC,)),
                pltpu.SemaphoreType.DMA((NG // g3,)),
                pltpu.SMEM((4,), i32),
            ],
            compiler_params=pltpu.CompilerParams(vmem_limit_bytes=127 << 20, flags=flags),
        )(A_x.reshape(S, D), A_wqkv, A_wo, B_w_gate, B_w_up, B_w_down)
        return out.reshape(1, S, D)

    return fn


@jax.jit
def pallas_recurrent_scan__sliding_local_dilated__geglu_ffn__prompt_kernel(
    A_x, A_wqkv, A_wo, B_x, B_w_gate, B_w_up, B_w_down
):
    return make(d1=384)(A_x, A_wqkv, A_wo, B_x, B_w_gate, B_w_up, B_w_down)
```

```python
import functools
import math

import jax
import jax.numpy as jnp
from jax import lax
import jax.experimental.pallas as pl
import jax.experimental.pallas.tpu as pltpu

S, D, F = 2048, 1024, 3584
DH, W, DIL = 32, 8, 2
PAD = 16
NP = 49
NZ = 28
GT = 64
NG = S // GT
CW = 512
NC = F // CW
LOG2E = math.log2(math.e)
C0 = math.sqrt(2.0 / math.pi)
XS = (C0 * 0.044715) ** (1.0 / 3.0)
f32, bf16, u32, i32 = jnp.float32, jnp.bfloat16, jnp.uint32, jnp.int32
P = functools.partial


def _pack(v):
    return pltpu.bitcast(v.astype(bf16), u32)


def _unpack(v):
    return pltpu.bitcast(v, bf16)


def _ds(start, size, align):
    if isinstance(start, int):
        return pl.ds(start, size)
    return pl.ds(pl.multiple_of(start, align), size)


def _tile(v, j):
    return v[:, j * 128:(j + 1) * 128]


def _lane_bit(shape, bit):
    return (lax.broadcasted_iota(i32, shape, 1) & bit) == 0


def _sum(vs):
    return functools.reduce(lambda a, b: a + b, vs)


class _Pace:
    def __init__(self, zero=None, lag=256):
        self.zero, self.lag = zero, lag
        self.tok, self.time, self.tiles, self.due, self.queues = None, 0, 0, [], []

    def add(self, tasks, cycles):
        if tasks:
            steps = (None for fn, _ in tasks for _ in fn())
            self.queues.append([steps, sum(n for _, n in tasks), cycles, 0, 0])

    def finish(self):
        for q in self.queues:
            for _ in q[0]:
                pass
        self.queues = []

    def dot(self, lhs, rhs):
        rows, nk = 2 * lhs.shape[0], lhs.shape[1] // 128
        t0 = self.tiles // 4 * rows
        part = range(rows * (self.tiles % 4) // 4, rows * (self.tiles % 4 + nk) // 4)
        self.tiles += nk
        if self.due and self.due[0][0] < t0 + part.stop:
            col = [lhs[r:r + 8, 0:128] for r in range(0, rows // 2, 8)]
            while self.due and self.due[0][0] < t0 + part.stop:
                t, tok = self.due.pop(0)
                i = max(t - t0, 0) // 16
                col[i] = jnp.where(self.zero == 0, col[i], pltpu.bitcast(tok, u32))
            lhs = jnp.concatenate([jnp.concatenate(col, axis=0)] + [_tile(lhs, j) for j in range(1, nk)], axis=1)
        y = jnp.dot(_unpack(lhs), rhs, preferred_element_type=f32)
        for r in part[::8]:
            self.tok, self.time = y[r:r + 8], t0 + r
            for q in self.queues:
                q[3] += 8
                while q[4] < min(q[1], q[1] * q[3] // q[2]):
                    q[4] += 1
                    next(q[0], None)
        return y

    def const(self, c, rows):
        if self.zero is None or self.tok is None:
            return c
        return jnp.concatenate([jnp.where(self.zero == 0, c, self.tok)] * (rows // 8), axis=0)

    def gate(self, v):
        if self.zero is None or self.tok is None:
            return v
        return jnp.where(self.zero == 0, v, jnp.concatenate([self.tok] * (v.shape[0] // 8), axis=0))

    def open(self, ref):
        if self.zero is not None and self.tok is not None:
            if ref.dtype == bf16:
                ref[self.zero, ref.shape[1] - 16:, 0:128] = pltpu.bitcast(self.tok, bf16)
            else:
                ref[ref.shape[0] - 1 + self.zero, 0:8, 0:128] = pltpu.bitcast(self.tok, ref.dtype)
        return ref

    def done(self, v, extra=0):
        if self.zero is not None and extra >= 0:
            self.due.append((self.time + self.lag + extra, v[-8:]))
            self.due.sort(key=lambda d: d[0])
        return v

    def stored(self, ref, n, rows, cols=pl.ds(0, 128), extra=0):
        if self.zero is not None and extra >= 0:
            self.done(ref[n + self.zero, rows, cols], extra)


LHS, RHS = (6, 3, 0, 2, 1, 4, 5), (6, 0, 5, 4, 2, 1, 3)


def _basis(scaled, x11, x12, x21, x22):
    h = x21 if scaled else x21 * 0.5
    p = x11 + h
    return [x11 + x22, p, h + x22, (p + x22 + x12) * 0.5 if scaled else (p + x22) * 0.5 + x12]


def _unbasis(half, scaled, z0, z1, z2, z3):
    h = z0 * half
    e = z3 + h
    if scaled:
        return [e + z2, z2 + h + z1, h, e + z1]
    return [e + z2, (z2 + h + z1) * 0.5, z0, e + z1]


def _operands(side, block, pc, ref, rows, col, base=0, scaled=False, src=None):
    def quad(a, b):
        if src is not None:
            pc.open(src)
        return _basis(scaled, *[block(2 * a + n // 2, 2 * b + n % 2) for n in range(4)])

    def put(k, x):
        t, p, q, r = x
        for n, v in zip(side, (t, p, q, r, t - p, q - t, r - t)):
            ref[pl.ds(base + 7 * side[k] + n, 1), rows, pl.ds(col, 128)] = _pack(v[None])
        pc.stored(ref, base + 7 * side[k], rows, pl.ds(col, 128))

    def run():
        h = quad(1, 0) if scaled else [v * 0.5 for v in quad(1, 0)]
        yield
        x11 = quad(0, 0)
        put(1, [a + b for a, b in zip(x11, h)])
        yield
        put(5, [b - a for a, b in zip(x11, h)])
        yield
        x22 = quad(1, 1)
        t = [a + b for a, b in zip(x11, x22)]
        put(0, t)
        yield
        put(2, [a + b for a, b in zip(x22, h)])
        yield
        put(4, [a - b for a, b in zip(x22, h)])
        yield
        r = [(a + b + c) * 0.5 if scaled else (a + b) * 0.5 + c for a, b, c in zip(t, h, quad(0, 1))]
        put(3, r)
        yield
        put(6, [a - b for a, b in zip(r, t)])
        yield

    return run, 8


def _products(prod, emit, odd=0):
    for o in range(7):
        m = lambda i: prod(7 * o + i)
        early = (o + odd) % 2
        t = m(6) if early else None
        a = m(0)
        t = t - a if early else a
        emit(o, a + m(1))
        a = m(2)
        t = t - a if early else t + a
        emit(7 + o, a + m(3))
        a = m(4)
        t = t + a if early else a - t
        emit(14 + o, m(5) - a)
        emit(21 + o, t if early else t + m(6))


def _result(pc, ref, rows, base=0, scaled=False):
    x = []
    for k in range(4):
        if k % 2 == 0:
            pc.open(ref)
        m = [ref[base + 7 * k + o, rows, :] for o in range(7)]
        x.append(_unbasis(0.5, scaled, m[0] + m[1], m[2] + m[3], m[5] - m[4], m[4] + m[6] - m[0] - m[2]))
        if k % 2:
            yield
    half = pc.const(0.5, x[0][0].shape[0])
    x = [_unbasis(half, scaled, *col) for col in zip(*x)]
    yield
    return [[x[2 * (i // 2) + j // 2][2 * (i % 2) + j % 2] for j in range(4)] for i in range(4)]


def _skewed(units, skew=1):
    order = sorted((u * skew + s, u, s) for u, st in enumerate(units) for s in range(len(st)))
    return [t for _, u, s in order for t in units[u][s]]


def _mix(*lists):
    keyed = []
    for i, ts in enumerate(lists):
        total, at = sum(n for _, n in ts), 0
        for t in ts:
            keyed.append(((at + t[1] / 2) / total, i, t))
            at += t[1]
    return [t for _, _, t in sorted(keyed, key=lambda k: k[:2])]


def make(g0=4, g1=8, g2=8, g3=4, n3=4, skew=1, attn=True, only=None, flags=None,
         d0=256, d1=256, d2=256, d3=256, vo=2, nbn=8, nbd=16, xl=128, sk1=1, cutz=(0, 3, 5, 7, 8), xa=2, nq=4, qs=(5, 6, 7, 7), cuts=(0, 22, 44, 64, 64),
         aw=(1, 2, 2, 5, 1, 6, 6, 2, 2, 1, 4, 4)):
    NX = NG // g0
    na = -(-NG // NC)
    ALL = slice(None)

    def attention_tasks(a0, qkv_s, san, r_s, o_s, pc):
        base = pl.multiple_of(a0 * GT, GT)
        win = qkv_s.at[:, pl.ds(base, na * GT + PAD), :]

        def block(b):
            r0 = base + b * 16
            a_s = san[b % len(san)]

            def shifted(j):
                v = {r: win[j, pl.ds(b * 16 + PAD + r, 8), :] for r in range(8, -DIL * W, -DIL)}
                return [jnp.concatenate([v[-DIL * w], v[8 - DIL * w]], axis=0) for w in range(W)]

            def scores():
                st = [None] * W
                for j in range(8):
                    q = pc.gate(win[j, pl.ds(b * 16 + PAD, 16), :])
                    for w, k in enumerate(shifted(8 + j)):
                        st[w] = q * k if j == 0 else st[w] + q * k
                    pc.done(st[W - 1])
                    yield
                for w in range(W):
                    a_s[w] = st[w] + pltpu.roll(st[w], 127, 1)
                pc.stored(a_s, 0, pl.ds(0, 8), extra=xl)

            def reduce():
                pc.open(a_s)
                for w in range(W):
                    a_s[W + w] = a_s[w] + pltpu.roll(a_s[w], 126, 1)
                pc.stored(a_s, W, pl.ds(0, 8), extra=xl)
                yield

            def softmax():
                pc.open(a_s)
                row = lax.broadcasted_iota(i32, (16, 128), 0) + r0
                logits = []
                for w in range(W):
                    t = a_s[W + w] * (DH ** -0.5 * LOG2E / XS ** 2)
                    if b == 0 and w:
                        t = jnp.where(row >= DIL * w, t, -1e9 * LOG2E)
                    logits.append(t)
                m = functools.reduce(jnp.maximum, logits)
                yield
                m = pc.gate(m)
                e = [jnp.exp2(t - m) for t in logits]
                inv = (1.0 / XS) / _sum(e)
                yield
                inv = pc.gate(inv)
                for w in range(W):
                    t = e[w] * inv
                    a_s[2 * W + w] = jnp.where(_lane_bit((16, 128), 1), t, pltpu.roll(t, 1, 1))
                pc.stored(a_s, 2 * W, pl.ds(0, 8), extra=xl)
                yield

            def spread():
                pc.open(a_s)
                for w in range(W):
                    t = a_s[2 * W + w]
                    a_s[3 * W + w] = jnp.where(_lane_bit((16, 128), 2), t, pltpu.roll(t, 2, 1))
                pc.stored(a_s, 3 * W, pl.ds(0, 8), extra=xl)
                yield

            def values():
                for j in range(8):
                    if j % vo == 0:
                        pc.open(a_s)
                        p = [a_s[3 * W + w] for w in range(W)]
                    v = shifted(16 + j)
                    r_s[b % 4 * 8 + j] = pc.done(_sum([p[w] * (v[w] if w else pc.gate(v[w])) for w in range(W)]))
                    yield

            store = [_operands(LHS, lambda i, j, e=e: r_s[i * 8 + 2 * j + e], pc, o_s,
                               _ds((a0 + b // 4) * 8, 8, 8), e * 128, src=r_s) for e in range(2)]
            return [[(scores, 8)], [(reduce, 1)], [(softmax, 3)], [(spread, 1)],
                    [(values, 8)] + (store if b % 4 == 3 else [])]

        return _skewed([block(b) for b in range(na * 4)], skew)

    def rhs_task(pc, src, load, dst, rows, col, base=0, flip=0):
        load = functools.cache(load)
        return _operands(RHS, lambda i, j: _tile(load(i, (j ^ flip) // 2), (j ^ flip) % 2), pc, dst, rows, col, base, src=src)

    def stacked(ref, n):
        return jnp.concatenate([ref[n, 0:ref.shape[1] - 8, k:k + 128] for k in (0, 128)], axis=0)

    def run(tasks):
        for fn, _ in tasks:
            for _ in fn():
                pass

    def kern(x_h, wqkv_h, wo_h, wg_h, wu_h, wd_h, out_h,
             x_s, xa_s, qkv_s, y_s, wg_s, wu_s, wd_s, wo_s, ba_s, bb_s, bd_s, bo_s, z_s, project_s, mix_s,
             sx, sq, sqkv, swo, sg, su, sd, so, zero_s):
        free = _Pace()
        for i in range(4):
            zero_s[i] = 0
        pace = lambda d: _Pace(zero_s[0], d) if d >= 0 else _Pace()

        def g_cp(c):
            return pltpu.make_async_copy(wg_h.at[:, :, _ds(c * CW, CW, CW)], wg_s.at[pl.ds((c & 1) * 4, 4), pl.ds(0, 256)], sg.at[c])

        def u_cp(c):
            return pltpu.make_async_copy(wu_h.at[:, :, _ds(c * CW, CW, CW)], wu_s.at[pl.ds((c & 1) * 4, 4), pl.ds(0, 256)], su.at[c])

        def dn_cp(c):
            return pltpu.make_async_copy(wd_h.at[_ds(c * CW, CW, CW), :], wd_s.at[c & 1, pl.ds(0, CW)], sd.at[c])

        wo_cp = pltpu.make_async_copy(wo_h, wo_s.at[0, pl.ds(0, D)], swo.at[0])

        def project(wqkv_s, sw_s):
            def x_cp(t):
                r = _ds(t * g0 * GT, g0 * GT, g0 * GT)
                return pltpu.make_async_copy(x_h.at[r, :], x_s.at[r, :], sx.at[t])

            def q_cps(t):
                r = _ds(t * (256 // nq), 256 // nq, 16)
                return [pltpu.make_async_copy(wqkv_h.at[:, r, pl.ds(p * CW, CW)], wqkv_s.at[p, :, r, :], sq.at[2 * t + p])
                        for p in range(2)]

            def qkv_cp(p):
                src = wqkv_h.at[:, :, pl.ds(p * CW, CW)] if p < 6 else wg_h.at[:, :, pl.ds(0, CW)]
                return pltpu.make_async_copy(src, wqkv_s.at[p], sqkv.at[p])

            def norm(g):
                mean = lambda vs: jnp.sum(_sum(vs), axis=1, keepdims=True) * (1.0 / D)
                x = [x_s[_ds(g * GT + i * 16, 16, 16), :].astype(f32) for i in range(4)]
                m = [mean([_tile(v, j) for j in range(8)]) for v in x]
                yield
                x = [v - a for v, a in zip(x, m)]
                r = [lax.rsqrt(mean([_tile(v * v, j) for j in range(8)]) + 1e-5) * XS for v in x]
                yield
                run([_operands(LHS, lambda i, j, e=e: _tile(x[i], 2 * j + e) * r[i], free, xa_s, _ds(g * 8, 8, 8), e * 128)
                     for e in range(2)])
                yield

            def qkv_tasks(pc, job, dst, units, plain=False):
                side = job & 1

                def unit(src, row, col, t_s):
                    st = {}

                    def swap(lvl):
                        lo = _lane_bit((8, 128), 4 << lvl)
                        for i in range(4):
                            if lvl == 2:
                                a, b = [_pack(wqkv_s[s, i, _ds(src, 16, 16), :])
                                        for s in (job, jnp.where(plain, job, job ^ 1))]
                                st[i] = [jnp.where((lo ^ (side == 1)) | plain, _tile(a, c),
                                                   pltpu.roll(_tile(b, c), 16 + 96 * side, 1)) for c in range(4)]
                            else:
                                st[i] = [jnp.where((~lo if c >> lvl & 1 else lo) | plain, st[i][c], pltpu.roll(
                                    st[i][c ^ (1 << lvl)], 128 - (4 << lvl) if c >> lvl & 1 else 4 << lvl, 1))
                                    for c in range(4)]
                            if lvl == 0:
                                for c in range(4):
                                    t_s[4 * i + c] = st[i][c]
                        yield

                    return [[(P(swap, lvl), 1)] for lvl in (2, 1, 0)] + [[
                        _operands(RHS, lambda i, j: _unpack(t_s[4 * i + j]).astype(f32), pc,
                                  dst, _ds(row, 8, 8), col, src=t_s)]]

                return _skewed([unit(*u, sw_s[n % 4]) for n, u in enumerate(units)], sk1)

            def put_tasks(pc, job, rb):
                def put(r):
                    res = yield from _result(pc, z_s[rb % 2], pl.ds(r, 8))
                    rows = lambda i: pl.ds((rb * g1 + r // 16) * GT + i * 16 + r % 16 + PAD, 8)
                    for n in range(16):
                        qkv_s[4 * job + n % 4, rows(n // 4), :] = res[n // 4][n % 4]
                    pc.stored(qkv_s, 4 * job, rows(0))

                return [(P(put, r), 3) for r in range(0, g1 * 16, 8)]

            def zero_tasks(pc, job):
                def zero(n):
                    for r in range(0, S // 4, 64):
                        y_s[8 * job + 8 + n, r:r + 64, :] = jnp.broadcast_to(pc.const(0.0, 64), (64, 128))
                        yield

                return [(P(zero, n), 8) for n in range(8)]

            for t in range(xa):
                x_cp(t).start()

            def zero(i, _):
                y_s[0:8, _ds(i * 32, 32, 32), :] = jnp.zeros((8, 32, 128), f32)
                z_s[1][:, _ds(i * 8, 8, 8), :] = jnp.zeros((NZ + 4, 8, 128), f32)

            lax.fori_loop(0, 16, zero, None)

            def head(t, _):
                pl.when(t + xa < NX)(lambda: x_cp(jnp.minimum(t + xa, NX - 1)).start())
                for i in range(nq):
                    for cp in q_cps(i):
                        pl.when(t == qs[i])(lambda: cp.start())
                x_cp(t).wait()
                for step in _skewed([[[gen]] * 3 for gen in [norm(t * g0 + i) for i in range(g0)]]):
                    next(step)

            jax.named_call(lambda: lax.fori_loop(0, NX, head, None), name='head')()

            def first(t, _):
                for cp in q_cps(t):
                    cp.wait()
                n = 256 // nq
                run(qkv_tasks(free, 0, ba_s, [(t * n + r, ((t * n) & 127) // 2 + r // 2, pl.multiple_of((t * n) & 128, 128))
                                              for r in range(0, n, 16)]))

            jax.named_call(lambda: lax.fori_loop(0, nq, first, None), name='first')()

            def phase1(job, _):
                for p in range(2, 7):
                    pl.when(job == p // 2 * 2 - 2)(lambda: qkv_cp(p).start())
                for cp in (wo_cp, u_cp(0), dn_cp(0), g_cp(1)):
                    pl.when(job == 4)(lambda: cp.start())
                for p in range(2, 7):
                    pl.when(job == p // 2 * 2 - 1)(lambda: qkv_cp(p).wait())
                pc = pace(d1)
                z = [zero_s[i] & 1 for i in range(4)]
                prep = qkv_tasks(pc, job + 1, bb_s, [(k + r, r // 2, k) for k in (0, 128) for r in range(0, 128, 16)],
                                 job == 5)
                cut = [len(prep) * c // 64 for c in cuts]
                nb = NG // g1
                for rb in range(nb):
                    def prod(n):
                        y = pc.dot(xa_s[n, rb * g1 * 8:(rb + 1) * g1 * 8, :],
                                   _unpack(stacked(ba_s, n + z[rb] if rb + 1 < nb else n)))
                        if rb + 1 == nb:
                            ba_s[n, 0:64, :] = pc.open(bb_s)[n, 0:64, :]
                        return y

                    def emit(n, v):
                        z_s[rb % 2][n, 0:g1 * 16, :] = v

                    puts = put_tasks(pc, job, rb - 1) if rb else put_tasks(pc, jnp.maximum(job - 1, 0), nb - 1)
                    pc.add(_mix(puts, prep[cut[rb]:cut[rb + 1]]), NP * g1 * 8 - (256 if rb == nb - 1 else 0))
                    pc.add(zero_tasks(pc, job)[cutz[rb]:cutz[rb + 1]], NP * g1 * 8)
                    _products(prod, emit, rb)
                    pc.finish()

            if only in (None, 1):
                jax.named_call(lambda: lax.fori_loop(0, 6, phase1, None), name='p1')()
            run(put_tasks(free, 5, NG // g1 - 1))

        project(*project_s)
        wo_cp.wait()

        for j in range(8, 24):
            qkv_s[j, 0:PAD, :] = jnp.broadcast_to(qkv_s[j, PAD:PAD + 1, :], (PAD, 128))

        def mix(o_s, h_s, ha_s, zz_s, san, r_s):
            def phase2(c, _):
                nxt = jnp.minimum(c + 1, NC - 1)
                pl.when(c + 1 < NC)(lambda: u_cp(nxt).start())
                pl.when(c + 2 < NC)(lambda: g_cp(jnp.minimum(c + 2, NC - 1)).start())
                pl.when(c + 1 < NC)(lambda: dn_cp(nxt).start())
                u_cp(c).wait()
                dn_cp(c).wait()
                pl.when(c + 1 < NC)(lambda: g_cp(nxt).wait())
                pc = pace(d2)
                z = [zero_s[i] & 1 for i in range(4)]
                att = attention_tasks(jnp.minimum(c * na, NG - na), qkv_s, san, r_s, o_s, pc) if attn else []

                def up(rb, si):
                    def emit(n, v):
                        (z_s, zz_s)[rb % 2][si][n, 0:g2 * 16, :] = v

                    _products(lambda n: pc.dot(xa_s[n, rb * g2 * 8:(rb + 1) * g2 * 8, :],
                                               _unpack(stacked((ba_s, bb_s)[si], n + z[rb]))), emit, pc.tiles // 2)

                def down(rb):
                    for e in range(2):
                        def emit(n, v):
                            y_s[e * NZ + n, rb * g2 * 16:(rb + 1) * g2 * 16, :] += v

                        _products(lambda n: pc.dot(stacked(ha_s[rb % 3], n + z[e + rb // 3 * 2]),
                                                   _unpack(bd_s[n + z[rb], 0:64, e * 128:(e + 1) * 128])), emit, e)

                def act(rb, r):
                    g = yield from _result(pc, (z_s, zz_s)[rb % 2][0], pl.ds(r, 8), 0, True)
                    u = yield from _result(pc, (z_s, zz_s)[rb % 2][1], pl.ds(r, 8))
                    for n in range(16):
                        i, j = n // 4, n % 4
                        s = 2.0 ** (j // 2 - i // 2 + j % 2 - i % 2)
                        t = pc.gate(g[i][j])
                        v = t * t if s == 1 else t * t * s ** -3
                        p = t * u[i][j ^ 3]
                        h_s[n, r:r + 8, :] = p * jnp.tanh(t * (v + C0 / XS / s)) + p
                        if j == 3:
                            pc.stored(h_s, n, pl.ds(r, 8))
                            yield

                def prep(w_s, slot, dst, flip):
                    return [rhs_task(pc, w_s, lambda i, h, r=k + r: w_s[4 * slot + i, pl.ds(r, 16), pl.ds(h * 256, 256)].astype(f32),
                                     dst, pl.ds(r // 2, 8), k, 0, flip) for k in (0, 128) for r in range(0, 128, 16)]

                def out_task(u, e, j0):
                    def load(i, h):
                        lo = lax.broadcasted_iota(i32, (8, 256), 0) < 4
                        v = [wo_s[0, _ds((u & 1) * 512 + (u >> 1) * 32 + k * 128 + i * 8, 8, 8),
                                  pl.ds(e * CW + h * 256, 256)].astype(f32) for k in range(4)]
                        v = [jnp.where(lo, pltpu.roll(a, 4, 0), b) if j0 else jnp.where(lo, a, pltpu.roll(b, 4, 0))
                             for a, b in (v[:2], v[2:])]
                        return jnp.concatenate(v, axis=0)

                    return rhs_task(pc, wo_s, load, bo_s, _ds(j0 * 64 + u * 8, 8, 8), e * 128)

                bd = [rhs_task(pc, wd_s, lambda i, h, e=e, r=r: wd_s[c & 1, pl.ds(i * 128 + r, 16), pl.ds(e * CW + h * 256, 256)].astype(f32),
                               bd_s, pl.ds(r // 2, 8), e * 128) for e in range(2) for r in range(0, 128, 16)]
                bo = [out_task((2 * c + u) & 7, e, j0) for u in range(2) for e in range(2) for j0 in range(2)]
                A = lambda rb: [(P(act, rb, r), 10) for r in range(0, g2 * 16, 8)]
                H = lambda rb: [_operands(LHS, lambda i, j, e=e: h_s[4 * i + j, e * 16:(e + 1) * 16, :], pc, ha_s[rb % 3],
                                          pl.ds(e % (g2 // 2) * 8, 8), e // (g2 // 2) * 128, scaled=True, src=h_s)
                                for e in range(g2)]
                bu, bn = prep(wu_s, c & 1, bb_s, 3), prep(wg_s, nxt & 1, ba_s, 0)
                plan = [(P(up, 0, 0), bu, 1), (P(up, 0, 1), bd[:nbd], 0), (P(up, 1, 0), A(0), 0), (P(up, 1, 1), _mix(H(0), bd[nbd:]), 1),
                        (P(down, 0), A(1), 0), (P(up, 2, 0), H(1), 0), (P(up, 2, 1), bo, 0), (P(up, 3, 0), A(2), 0),
                        (P(up, 3, 1), H(2) + bn[:nbn], 0), (P(down, 1), A(3), 0), (P(down, 2), H(3), 1),
                        (P(down, 3), bn[nbn:], 1)]
                done = 0
                for i, (products, tasks, early) in enumerate(plan):
                    upto = len(att) * sum(aw[:i + 1]) // sum(aw)
                    pc.add(_mix(tasks, att[done:upto]), NP * g2 * 8 - 320 * early)
                    done = upto
                    products()
                    pc.finish()

            if only in (None, 2):
                jax.named_call(lambda: lax.fori_loop(0, NC, phase2, None), name='p2')()

            def out_cp(t):
                r = _ds(t * g3 * GT, g3 * GT, g3 * GT)
                return pltpu.make_async_copy(x_s.at[r, :], out_h.at[r, :], so.at[t])

            def out_tasks(pc, dst, e):
                def out(r):
                    s = yield from _result(pc, z_s[e], pl.ds(r, 8))
                    for i in range(4):
                        rows = pl.ds(r // 16 * GT + i * 16 + r % 16, 8)
                        if i % 2 == 0:
                            pc.open(zz_s[e])
                        v = jnp.concatenate([s[i][j] * zz_s[e][4 * i + j, r:r + 8, :] for j in range(4)], axis=1)
                        v = dst[rows, e * CW:(e + 1) * CW].astype(f32) + v
                        dst[rows, e * CW:(e + 1) * CW] = v.astype(bf16)
                        pc.done(_tile(v, 3))
                        if i % 2:
                            yield

                return [(P(out, r), 5) for r in range(0, g3 * 16, 8)]

            def phase3(t, _):
                pc = pace(d3)
                z = [zero_s[i] & 1 for i in range(4)]
                nb = NG // g3 // n3
                y0 = pl.multiple_of(t * (nb * g3 * 16), nb * g3 * 16)
                rows = lambda tb: x_s.at[_ds(tb * g3 * GT, g3 * GT, g3 * GT), :]
                for rb in range(nb):
                    tb = t * nb + rb
                    for e in range(2):
                        def gate(r):
                            y = yield from _result(pc, y_s, pl.ds(y0 + rb * g3 * 16 + r, 8), e * NZ)
                            for n in range(16):
                                h = y[n // 4][n % 4] * pc.const(0.25 / XS ** 2, 8)
                                zz_s[e][n, r:r + 8, :] = h * jnp.tanh(h) + h
                                if n % 8 == 7:
                                    pc.stored(zz_s[e], n, pl.ds(r, 8))
                                    yield

                        def emit(n, v):
                            z_s[e][n, 0:g3 * 16, :] = v

                        outs = out_tasks(pc, rows(tb if e else jnp.where(tb > 0, tb - 1, NG // g3)), 1 - e)
                        pc.add(_mix(outs, [(P(gate, r), 5) for r in range(0, g3 * 16, 8)]), NP * g3 * 8)
                        _products(lambda n: pc.dot(o_s[n + z[e], _ds(tb * g3 * 8, g3 * 8, g3 * 8), :],
                                                   _unpack(bo_s[n + z[rb], 0:128, e * 128:(e + 1) * 128])), emit, e)
                        pc.finish()
                        if e == 0:
                            pl.when(tb > 0)(lambda: out_cp(jnp.maximum(tb - 1, 0)).start())

            x_s[S:, :] = jnp.zeros((g3 * GT, D), bf16)
            if only in (None, 3):
                jax.named_call(lambda: lax.fori_loop(0, n3, phase3, None), name='p3')()
            run(out_tasks(free, x_s.at[S - g3 * GT:S, :], 1))
            out_cp(NG // g3 - 1).start()
            for t in range(NG // g3):
                out_cp(t).wait()

        mix(*mix_s)

    def fn(A_x, A_wqkv, A_wo, B_x, B_w_gate, B_w_up, B_w_down):
        any_spec = pl.BlockSpec(memory_space=pl.ANY)
        out = pl.pallas_call(
            kern,
            in_specs=[any_spec] * 6,
            out_specs=any_spec,
            out_shape=jax.ShapeDtypeStruct((S, D), bf16),
            scratch_shapes=[
                pltpu.VMEM((S + g3 * GT, D), bf16),
                pltpu.VMEM((NP + 1, S // 8 + 8, D // 4), u32),
                pltpu.VMEM((24, S + PAD, 128), f32),
                pltpu.VMEM((2 * NZ + 4, S // 4 + 8, 128), f32),
                pltpu.VMEM((8, D // 4 + 16, CW), bf16),
                pltpu.VMEM((8, D // 4 + 16, CW), bf16),
                pltpu.VMEM((2, CW + 16, D), bf16),
                pltpu.VMEM((1, D + 16, D), bf16),
                pltpu.VMEM((NP + 1, 72, 256), u32),
                pltpu.VMEM((NP + 1, 72, 256), u32),
                pltpu.VMEM((NP + 1, 72, 256), u32),
                pltpu.VMEM((NP + 1, 136, 256), u32),
                [pltpu.VMEM((NZ + 4, g2 * 16 + 8, 128), f32)] * 2,
                [pltpu.VMEM((7, 4, D // 4, CW), bf16), [pltpu.VMEM((20, 8, 128), u32)] * 4],
                [pltpu.VMEM((NP + 1, S // 8 + 8, D // 4), u32), pltpu.VMEM((18, g2 * 16 + 16, 128), f32),
                      [pltpu.VMEM((NP + 1, g2 * 4 + 8, 256), u32)] * 3, [pltpu.VMEM((NZ + 4, g2 * 16 + 8, 128), f32)] * 2,
                      [pltpu.VMEM((4 * W + 2, 16, 128), f32)] * 5, pltpu.VMEM((34, 16, 128), f32)],
                pltpu.SemaphoreType.DMA((NX,)),
                pltpu.SemaphoreType.DMA((2 * nq,)),
                pltpu.SemaphoreType.DMA((7,)),
                pltpu.SemaphoreType.DMA((1,)),
                pltpu.SemaphoreType.DMA((NC,)),
                pltpu.SemaphoreType.DMA((NC,)),
                pltpu.SemaphoreType.DMA((NC,)),
                pltpu.SemaphoreType.DMA((NG // g3,)),
                pltpu.SMEM((4,), i32),
            ],
            compiler_params=pltpu.CompilerParams(vmem_limit_bytes=127 << 20, flags=flags),
        )(A_x.reshape(S, D), A_wqkv.reshape(4, D // 4, 3 * D), A_wo, B_w_gate.reshape(4, D // 4, F),
          B_w_up.reshape(4, D // 4, F), B_w_down)
        return out.reshape(1, S, D)

    return fn


@jax.jit
def pallas_recurrent_scan__sliding_local_dilated__geglu_ffn__prompt_kernel(
    A_x, A_wqkv, A_wo, B_x, B_w_gate, B_w_up, B_w_down
):
    return make()(A_x, A_wqkv, A_wo, B_x, B_w_gate, B_w_up, B_w_down)
```

```python
import functools
import math

import jax
import jax.numpy as jnp
from jax import lax
import jax.experimental.pallas as pl
import jax.experimental.pallas.tpu as pltpu

S, D, F = 2048, 1024, 3584
DH, W, DIL = 32, 8, 2
PAD = 16
NP = 49
NZ = 28
GT = 64
NG = S // GT
CW = 512
NC = F // CW
LOG2E = math.log2(math.e)
C0 = math.sqrt(2.0 / math.pi)
XS = (C0 * 0.044715) ** (1.0 / 3.0)
f32, bf16, u32, i32 = jnp.float32, jnp.bfloat16, jnp.uint32, jnp.int32
P = functools.partial


def _pack(v):
    return pltpu.bitcast(v.astype(bf16), u32)


def _unpack(v):
    return pltpu.bitcast(v, bf16)


def _ds(start, size, align):
    if isinstance(start, int):
        return pl.ds(start, size)
    return pl.ds(pl.multiple_of(start, align), size)


def _tile(v, j):
    return v[:, j * 128:(j + 1) * 128]


def _lane_bit(shape, bit):
    return (lax.broadcasted_iota(i32, shape, 1) & bit) == 0


def _sum(vs):
    return functools.reduce(lambda a, b: a + b, vs)


class _Pace:
    def __init__(self, zero=None, lag=256):
        self.zero, self.lag = zero, lag
        self.tok, self.time, self.tiles, self.due, self.queues = None, 0, 0, [], []

    def add(self, tasks, cycles):
        if tasks:
            steps = (None for fn, _ in tasks for _ in fn())
            self.queues.append([steps, sum(n for _, n in tasks), cycles, 0, 0])

    def finish(self):
        for q in self.queues:
            for _ in q[0]:
                pass
        self.queues = []

    def dot(self, lhs, rhs):
        rows, nk = 2 * lhs.shape[0], lhs.shape[1] // 128
        t0 = self.tiles // 4 * rows
        part = range(rows * (self.tiles % 4) // 4, rows * (self.tiles % 4 + nk) // 4)
        self.tiles += nk
        if self.due and self.due[0][0] < t0 + part.stop:
            col = [lhs[r:r + 8, 0:128] for r in range(0, rows // 2, 8)]
            while self.due and self.due[0][0] < t0 + part.stop:
                t, tok = self.due.pop(0)
                i = max(t - t0, 0) // 16
                col[i] = jnp.where(self.zero == 0, col[i], pltpu.bitcast(tok, u32))
            lhs = jnp.concatenate([jnp.concatenate(col, axis=0)] + [_tile(lhs, j) for j in range(1, nk)], axis=1)
        y = jnp.dot(_unpack(lhs), rhs, preferred_element_type=f32)
        for r in part[::8]:
            self.tok, self.time = y[r:r + 8], t0 + r
            for q in self.queues:
                q[3] += 8
                while q[4] < min(q[1], q[1] * q[3] // q[2]):
                    q[4] += 1
                    next(q[0], None)
        return y

    def const(self, c, rows):
        if self.zero is None or self.tok is None:
            return c
        return jnp.concatenate([jnp.where(self.zero == 0, c, self.tok)] * (rows // 8), axis=0)

    def gate(self, v):
        if self.zero is None or self.tok is None:
            return v
        return jnp.where(self.zero == 0, v, jnp.concatenate([self.tok] * (v.shape[0] // 8), axis=0))

    def open(self, ref):
        if self.zero is not None and self.tok is not None:
            if ref.dtype == bf16:
                ref[self.zero, ref.shape[1] - 16:, 0:128] = pltpu.bitcast(self.tok, bf16)
            else:
                ref[ref.shape[0] - 1 + self.zero, 0:8, 0:128] = pltpu.bitcast(self.tok, ref.dtype)
        return ref

    def done(self, v, extra=0):
        if self.zero is not None and extra >= 0:
            self.due.append((self.time + self.lag + extra, v[-8:]))
            self.due.sort(key=lambda d: d[0])
        return v

    def stored(self, ref, extra=0):
        if self.zero is not None and extra >= 0:
            self.done(ref[ref.shape[0] - 1 + self.zero, ref.shape[1] - 8:, 0:128], extra)


LHS, RHS = (6, 3, 0, 2, 1, 4, 5), (6, 0, 5, 4, 2, 1, 3)


def _basis(scaled, x11, x12, x21, x22):
    h = x21 if scaled else x21 * 0.5
    p = x11 + h
    return [x11 + x22, p, h + x22, (p + x22 + x12) * 0.5 if scaled else (p + x22) * 0.5 + x12]


def _unbasis(half, scaled, z0, z1, z2, z3):
    h = z0 * half
    e = z3 + h
    if scaled:
        return [e + z2, z2 + h + z1, h, e + z1]
    return [e + z2, (z2 + h + z1) * 0.5, z0, e + z1]


def _operands(side, block, pc, ref, rows, col, base=0, scaled=False, src=None):
    def quad(a, b):
        if src is not None:
            pc.open(src)
        return _basis(scaled, *[block(2 * a + n // 2, 2 * b + n % 2) for n in range(4)])

    def put(k, x):
        t, p, q, r = x
        for n, v in zip(side, (t, p, q, r, t - p, q - t, r - t)):
            ref[pl.ds(base + 7 * side[k] + n, 1), rows, pl.ds(col, 128)] = _pack(v[None])
        pc.stored(ref)

    def run():
        h = quad(1, 0) if scaled else [v * 0.5 for v in quad(1, 0)]
        yield
        x11 = quad(0, 0)
        put(1, [a + b for a, b in zip(x11, h)])
        yield
        put(5, [b - a for a, b in zip(x11, h)])
        yield
        x22 = quad(1, 1)
        t = [a + b for a, b in zip(x11, x22)]
        put(0, t)
        yield
        put(2, [a + b for a, b in zip(x22, h)])
        yield
        put(4, [a - b for a, b in zip(x22, h)])
        yield
        r = [(a + b + c) * 0.5 if scaled else (a + b) * 0.5 + c for a, b, c in zip(t, h, quad(0, 1))]
        put(3, r)
        yield
        put(6, [a - b for a, b in zip(r, t)])
        yield

    return run, 8


def _products(prod, emit, odd=0):
    for o in range(7):
        m = lambda i: prod(7 * o + i)
        early = (o + odd) % 2
        t = m(6) if early else None
        a = m(0)
        t = t - a if early else a
        emit(o, a + m(1))
        a = m(2)
        t = t - a if early else t + a
        emit(7 + o, a + m(3))
        a = m(4)
        t = t + a if early else a - t
        emit(14 + o, m(5) - a)
        emit(21 + o, t if early else t + m(6))


def _result(pc, ref, rows, base=0, scaled=False):
    x = []
    for k in range(4):
        if k % 2 == 0:
            pc.open(ref)
        m = [ref[base + 7 * k + o, rows, :] for o in range(7)]
        x.append(_unbasis(0.5, scaled, m[0] + m[1], m[2] + m[3], m[5] - m[4], m[4] + m[6] - m[0] - m[2]))
        if k % 2:
            yield
    half = pc.const(0.5, x[0][0].shape[0])
    x = [_unbasis(half, scaled, *col) for col in zip(*x)]
    yield
    return [[x[2 * (i // 2) + j // 2][2 * (i % 2) + j % 2] for j in range(4)] for i in range(4)]


def _skewed(units, skew=1):
    order = sorted((u * skew + s, u, s) for u, st in enumerate(units) for s in range(len(st)))
    return [t for _, u, s in order for t in units[u][s]]


def _mix(*lists):
    keyed = []
    for i, ts in enumerate(lists):
        total, at = sum(n for _, n in ts), 0
        for t in ts:
            keyed.append(((at + t[1] / 2) / total, i, t))
            at += t[1]
    return [t for _, _, t in sorted(keyed, key=lambda k: k[:2])]


def make(g0=2, g1=8, g2=8, g3=4, n3=4, skew=1, attn=True, only=None, flags=None,
         d0=256, d1=256, d2=256, d3=256, vo=2, nbn=8, nbd=16, xl=128, sk1=1, nbc=True, cutz=(0, 3, 5, 7, 8), xa=16, nq=4, qs=(5, 6, 7, 7), cuts=(0, 22, 44, 64, 64),
         aw=(1, 2, 2, 5, 1, 6, 6, 2, 2, 1, 4, 4)):
    NX = NG // g0
    na = -(-NG // NC)
    ALL = slice(None)

    def attention_tasks(a0, qkv_s, san, r_s, o_s, pc):
        base = pl.multiple_of(a0 * GT, GT)
        win = qkv_s.at[:, pl.ds(base, na * GT + PAD), :]

        def block(b):
            r0 = base + b * 16
            a_s = san[b % len(san)]

            def shifted(j):
                v = {r: win[j, pl.ds(b * 16 + PAD + r, 8), :] for r in range(8, -DIL * W, -DIL)}
                return [jnp.concatenate([v[-DIL * w], v[8 - DIL * w]], axis=0) for w in range(W)]

            def scores():
                st = [None] * W
                for j in range(8):
                    q = pc.gate(win[j, pl.ds(b * 16 + PAD, 16), :])
                    for w, k in enumerate(shifted(8 + j)):
                        st[w] = q * k if j == 0 else st[w] + q * k
                    pc.done(st[W - 1])
                    yield
                for w in range(W):
                    a_s[w] = st[w] + pltpu.roll(st[w], 127, 1)
                pc.stored(a_s, xl)

            def reduce():
                pc.open(a_s)
                for w in range(W):
                    a_s[W + w] = a_s[w] + pltpu.roll(a_s[w], 126, 1)
                pc.stored(a_s, xl)
                yield

            def softmax():
                pc.open(a_s)
                row = lax.broadcasted_iota(i32, (16, 128), 0) + r0
                logits = []
                for w in range(W):
                    t = a_s[W + w] * (DH ** -0.5 * LOG2E / XS ** 2)
                    if b == 0 and w:
                        t = jnp.where(row >= DIL * w, t, -1e9 * LOG2E)
                    logits.append(t)
                m = functools.reduce(jnp.maximum, logits)
                yield
                m = pc.gate(m)
                e = [jnp.exp2(t - m) for t in logits]
                inv = (1.0 / XS) / _sum(e)
                yield
                inv = pc.gate(inv)
                for w in range(W):
                    t = e[w] * inv
                    a_s[2 * W + w] = jnp.where(_lane_bit((16, 128), 1), t, pltpu.roll(t, 1, 1))
                pc.stored(a_s, xl)
                yield

            def spread():
                pc.open(a_s)
                for w in range(W):
                    t = a_s[2 * W + w]
                    a_s[3 * W + w] = jnp.where(_lane_bit((16, 128), 2), t, pltpu.roll(t, 2, 1))
                pc.stored(a_s, xl)
                yield

            def values():
                for j in range(8):
                    if j % vo == 0:
                        pc.open(a_s)
                        p = [a_s[3 * W + w] for w in range(W)]
                    v = shifted(16 + j)
                    r_s[b % 4 * 8 + j] = pc.done(_sum([p[w] * (v[w] if w else pc.gate(v[w])) for w in range(W)]))
                    yield

            store = [_operands(LHS, lambda i, j, e=e: r_s[i * 8 + 2 * j + e], pc, o_s,
                               _ds((a0 + b // 4) * 8, 8, 8), e * 128, src=r_s) for e in range(2)]
            return [[(scores, 8)], [(reduce, 1)], [(softmax, 3)], [(spread, 1)],
                    [(values, 8)] + (store if b % 4 == 3 else [])]

        return _skewed([block(b) for b in range(na * 4)], skew)

    def rhs_task(pc, src, load, dst, rows, col, base=0, flip=0):
        load = functools.cache(load)
        return _operands(RHS, lambda i, j: _tile(load(i, (j ^ flip) // 2), (j ^ flip) % 2), pc, dst, rows, col, base, src=src)

    def stacked(ref, n):
        return jnp.concatenate([ref[n, 0:ref.shape[1] - 8, k:k + 128] for k in (0, 128)], axis=0)

    def run(tasks):
        for fn, _ in tasks:
            for _ in fn():
                pass

    def kern(x_h, wqkv_h, wo_h, wg_h, wu_h, wd_h, out_h,
             x_s, xa_s, qkv_s, y_s, wg_s, wu_s, wd_s, wo_s, ba_s, bb_s, bd_s, bo_s, z_s, project_s, mix_s,
             sx, sq, sqkv, swo, sg, su, sd, so, zero_s):
        free = _Pace()
        for i in range(4):
            zero_s[i] = 0
        for ref in [xa_s, ba_s, bb_s, bd_s, bo_s, mix_s[0]] + mix_s[2] + mix_s[4]:
            ref[ref.shape[0] - 1, ref.shape[1] - 8:, 0:128] = jnp.zeros((8, 128), ref.dtype)
        pace = lambda d: _Pace(zero_s[0], d) if d >= 0 else _Pace()

        def g_cp(c):
            return pltpu.make_async_copy(wg_h.at[:, :, _ds(c * CW, CW, CW)], wg_s.at[pl.ds((c & 1) * 4, 4), pl.ds(0, 256)], sg.at[c])

        def u_cp(c):
            return pltpu.make_async_copy(wu_h.at[:, :, _ds(c * CW, CW, CW)], wu_s.at[pl.ds((c & 1) * 4, 4), pl.ds(0, 256)], su.at[c])

        def dn_cp(c):
            return pltpu.make_async_copy(wd_h.at[_ds(c * CW, CW, CW), :], wd_s.at[c & 1, pl.ds(0, CW)], sd.at[c])

        wo_cp = pltpu.make_async_copy(wo_h, wo_s.at[0, pl.ds(0, D)], swo.at[0])

        def project(wqkv_s, sw_s):
            def x_cp(t):
                r = _ds(t * g0 * GT, g0 * GT, g0 * GT)
                return pltpu.make_async_copy(x_h.at[r, :], x_s.at[r, :], sx.at[t])

            def q_cps(t):
                r = _ds(t * (256 // NX), 256 // NX, 16)
                return [pltpu.make_async_copy(wqkv_h.at[:, r, pl.ds(p * CW, CW)], wqkv_s.at[p, :, r, :], sq.at[2 * t + p])
                        for p in range(2)]

            def qkv_cp(p):
                src = wqkv_h.at[:, :, pl.ds(p * CW, CW)] if p < 6 else wg_h.at[:, :, pl.ds(0, CW)]
                return pltpu.make_async_copy(src, wqkv_s.at[p], sqkv.at[p])

            def norm_center(g):
                x = x_s[_ds(g * GT, GT, GT), :].astype(f32)
                m = jnp.sum(_sum([_tile(x, j) for j in range(8)]), axis=1, keepdims=True) * (1.0 / D)
                qkv_s[8, _ds(g * GT, GT, GT), :] = jnp.broadcast_to(m, (GT, 128))

            def norm_scale(g):
                win, xw = qkv_s.at[:, _ds(g * GT, GT, GT), :], x_s.at[_ds(g * GT, GT, GT), :]
                for r in range(0, GT, 8):
                    x, m = xw[r:r + 8, :].astype(f32), win[8, r:r + 8, :]
                    x = [_tile(x, j) - m for j in range(8)]
                    for j in range(8):
                        win[j, r:r + 8, :] = x[j]
                    v = jnp.sum(_sum([v * v for v in x]), axis=1, keepdims=True) * (1.0 / D)
                    win[9, r:r + 8, :] = jnp.broadcast_to(lax.rsqrt(v + 1e-5) * XS, (8, 128))

            def norm_operands(g):
                win = qkv_s.at[:, _ds(g * GT, GT, GT), :]
                run([_operands(LHS, lambda i, j, e=e: win[2 * j + e, i * 16:(i + 1) * 16, :] * win[9, i * 16:(i + 1) * 16, :],
                               free, xa_s, _ds(g * 8, 8, 8), e * 128) for e in range(2)])

            def swap_outer(job, i, rows, plain=False):
                side = job & 1
                a, b = [_pack(wqkv_s[s, i, rows, :]) for s in (job, jnp.where(plain, job, job ^ 1))]
                keep = (_lane_bit((8, 128), 16) ^ (side == 1)) | plain
                return [jnp.where(keep, _tile(a, c), pltpu.roll(_tile(b, c), 16 + 96 * side, 1)) for c in range(4)]

            def swap_inner(v, lvl, plain=False):
                lo = _lane_bit((8, 128), 4 << lvl)
                return [jnp.where((~lo if c >> lvl & 1 else lo) | plain, v[c],
                                  pltpu.roll(v[c ^ (1 << lvl)], 128 - (4 << lvl) if c >> lvl & 1 else 4 << lvl, 1))
                        for c in range(4)]

            def qkv_tasks(pc, job, dst, units, plain=False):
                def unit(src, row, col, t_s):
                    st = {}

                    def swap(lvl):
                        for i in range(4):
                            st[i] = swap_outer(job, i, pl.ds(src, 16), plain) if lvl == 2 else swap_inner(st[i], lvl, plain)
                            if lvl == 0:
                                for c in range(4):
                                    t_s[4 * i + c] = st[i][c]
                        yield

                    return [[(P(swap, lvl), 1)] for lvl in (2, 1, 0)] + [[
                        _operands(RHS, lambda i, j: _unpack(t_s[4 * i + j]).astype(f32), pc,
                                  dst, _ds(row, 8, 8), col, src=t_s)]]

                return _skewed([unit(*u, sw_s[n % 4]) for n, u in enumerate(units)], sk1)

            def put_tasks(pc, job, rb):
                def put(r):
                    res = yield from _result(pc, z_s[rb % 2], pl.ds(r, 8))
                    rows = lambda i: pl.ds((rb * g1 + r // 16) * GT + i * 16 + r % 16 + PAD, 8)
                    for n in range(16):
                        qkv_s[4 * job + n % 4, rows(n // 4), :] = res[n // 4][n % 4]
                    pc.done(res[0][3])

                return [(P(put, r), 3) for r in range(0, g1 * 16, 8)]

            def zero_tasks(pc, job):
                def zero(n):
                    for r in range(0, S // 4, 64):
                        y_s[8 * job + 8 + n, r:r + 64, :] = jnp.broadcast_to(pc.const(0.0, 64), (64, 128))
                        yield

                return [(P(zero, n), 8) for n in range(8)]

            def first_cps(t):
                return [x_cp(t)] + q_cps(t)

            for t in range(xa):
                for cp in first_cps(t):
                    cp.start()

            def zero(i, _):
                y_s[0:8, _ds(i * 32, 32, 32), :] = jnp.zeros((8, 32, 128), f32)
                z_s[1][:, _ds(i * 8, 8, 8), :] = jnp.zeros((NZ + 4, 8, 128), f32)
                qkv_s[0:10, _ds(i * 8, 8, 8), :] = jnp.zeros((10, 8, 128), f32)

            lax.fori_loop(0, 16, zero, None)
            for ref in (bb_s, bd_s, bo_s):
                ref[0, 0:64, :] = jnp.zeros((64, 256), u32)

            def head(it, _):
                sh = (16 // NX).bit_length() - 1
                t, new = it >> sh, (it & (16 // NX - 1)) == 0
                if xa < NX:
                    for cp in first_cps(jnp.minimum(t + xa, NX - 1)):
                        pl.when(new & (t + xa < NX))(lambda: cp.start())
                for cp in first_cps(jnp.minimum(t, NX - 1)):
                    pl.when(new & (t < NX))(lambda: cp.wait())
                u = [jnp.clip(it - s, 0, 15) for s in range(4)]
                at = lambda s, i, c: (u[s], pl.ds(16 * i + c // 2 * 8, 8), pl.ds(c % 2 * 128, 128))
                run([_operands(RHS, lambda i, j: _unpack(bo_s[at(3, i, j)]).astype(f32), free,
                               ba_s, _ds((u[3] & 7) * 8, 8, 8), pl.multiple_of((u[3] >> 3) * 128, 128))])
                for s, src, dst in ((2, bd_s, bo_s), (1, bb_s, bd_s), (0, None, bb_s)):
                    for i in range(4):
                        v = swap_inner([src[at(s, i, c)] for c in range(4)], 2 - s) if s else swap_outer(
                            0, i, _ds(u[0] * 16, 16, 16))
                        for c in range(4):
                            dst[at(s, i, c)] = v[c]
                for s, stage in ((2, norm_operands), (1, norm_scale), (0, norm_center)):
                    for g in range(2):
                        stage(2 * u[s] + g)

            jax.named_call(lambda: lax.fori_loop(0, 19, head, None), name='head')()

            def phase1(job, _):
                for p in range(2, 7):
                    pl.when(job == p // 2 * 2 - 2)(lambda: qkv_cp(p).start())
                for cp in (wo_cp, u_cp(0), dn_cp(0), g_cp(1)):
                    pl.when(job == 4)(lambda: cp.start())
                for p in range(2, 7):
                    pl.when(job == p // 2 * 2 - 1)(lambda: qkv_cp(p).wait())
                pc = pace(d1)
                z = [zero_s[i] & 1 for i in range(4)]
                prep = qkv_tasks(pc, job + 1, bb_s, [(k + r, r // 2, k) for k in (0, 128) for r in range(0, 128, 16)],
                                 job == 5)
                cut = [len(prep) * c // 64 for c in cuts]
                nb = NG // g1
                for rb in range(nb):
                    def prod(n):
                        y = pc.dot(xa_s[n, rb * g1 * 8:(rb + 1) * g1 * 8, :],
                                   _unpack(stacked(ba_s, n + z[rb] if rb + 1 < nb else n)))
                        if rb + 1 == nb:
                            ba_s[n, 0:64, :] = pc.open(bb_s)[n, 0:64, :]
                        return y

                    def emit(n, v):
                        z_s[rb % 2][n, 0:g1 * 16, :] = v

                    puts = put_tasks(pc, job, rb - 1) if rb else put_tasks(pc, jnp.maximum(job - 1, 0), nb - 1)
                    pc.add(_mix(puts, prep[cut[rb]:cut[rb + 1]]), NP * g1 * 8 - (256 if rb == nb - 1 else 0))
                    pc.add(zero_tasks(pc, job)[cutz[rb]:cutz[rb + 1]], NP * g1 * 8)
                    _products(prod, emit, rb)
                    pc.finish()

            if only in (None, 1):
                jax.named_call(lambda: lax.fori_loop(0, 6, phase1, None), name='p1')()
            run(put_tasks(free, 5, NG // g1 - 1))

        project(*project_s)
        wo_cp.wait()

        for j in range(8, 24):
            qkv_s[j, 0:PAD, :] = jnp.broadcast_to(qkv_s[j, PAD:PAD + 1, :], (PAD, 128))

        def mix(o_s, h_s, ha_s, zz_s, san, r_s):
            def phase2(c, _):
                nxt = jnp.minimum(c + 1, NC - 1)
                pl.when(c + 1 < NC)(lambda: u_cp(nxt).start())
                pl.when(c + 2 < NC)(lambda: g_cp(jnp.minimum(c + 2, NC - 1)).start())
                pl.when(c + 1 < NC)(lambda: dn_cp(nxt).start())
                u_cp(c).wait()
                dn_cp(c).wait()
                pl.when(c + 1 < NC)(lambda: g_cp(nxt).wait())
                pc = pace(d2)
                z = [zero_s[i] & 1 for i in range(4)]
                att = attention_tasks(jnp.minimum(c * na, NG - na), qkv_s, san, r_s, o_s, pc) if attn else []

                def up(rb, si):
                    def emit(n, v):
                        (z_s, zz_s)[rb % 2][si][n, 0:g2 * 16, :] = v

                    _products(lambda n: pc.dot(xa_s[n, rb * g2 * 8:(rb + 1) * g2 * 8, :],
                                               _unpack(stacked((ba_s, bb_s)[si], n + z[rb]))), emit, pc.tiles // 2)

                def down(rb):
                    for e in range(2):
                        def emit(n, v):
                            y_s[e * NZ + n, rb * g2 * 16:(rb + 1) * g2 * 16, :] += v

                        _products(lambda n: pc.dot(stacked(ha_s[rb % 3], n + z[e + rb // 3 * 2]),
                                                   _unpack(bd_s[n + z[rb], 0:64, e * 128:(e + 1) * 128])), emit, e)

                def act(rb, r):
                    g = yield from _result(pc, (z_s, zz_s)[rb % 2][0], pl.ds(r, 8), 0, True)
                    u = yield from _result(pc, (z_s, zz_s)[rb % 2][1], pl.ds(r, 8))
                    for n in range(16):
                        i, j = n // 4, n % 4
                        s = 2.0 ** (j // 2 - i // 2 + j % 2 - i % 2)
                        t = pc.gate(g[i][j])
                        v = t * t if s == 1 else t * t * s ** -3
                        p = t * u[i][j ^ 3]
                        h_s[n, r:r + 8, :] = v = p * jnp.tanh(t * (v + C0 / XS / s)) + p
                        if j == 3:
                            pc.done(v)
                            yield

                def prep(w_s, slot, dst, flip):
                    return [rhs_task(pc, w_s, lambda i, h, r=k + r: w_s[4 * slot + i, pl.ds(r, 16), pl.ds(h * 256, 256)].astype(f32),
                                     dst, pl.ds(r // 2, 8), k, 0, flip) for k in (0, 128) for r in range(0, 128, 16)]

                def out_task(u, e, j0):
                    def load(i, h):
                        lo = lax.broadcasted_iota(i32, (8, 256), 0) < 4
                        v = [wo_s[0, _ds((u & 1) * 512 + (u >> 1) * 32 + k * 128 + i * 8, 8, 8),
                                  pl.ds(e * CW + h * 256, 256)].astype(f32) for k in range(4)]
                        v = [jnp.where(lo, pltpu.roll(a, 4, 0), b) if j0 else jnp.where(lo, a, pltpu.roll(b, 4, 0))
                             for a, b in (v[:2], v[2:])]
                        return jnp.concatenate(v, axis=0)

                    return rhs_task(pc, wo_s, load, bo_s, _ds(j0 * 64 + u * 8, 8, 8), e * 128)

                bd = [rhs_task(pc, wd_s, lambda i, h, e=e, r=r: wd_s[c & 1, pl.ds(i * 128 + r, 16), pl.ds(e * CW + h * 256, 256)].astype(f32),
                               bd_s, pl.ds(r // 2, 8), e * 128) for e in range(2) for r in range(0, 128, 16)]
                bo = [out_task((2 * c + u) & 7, e, j0) for u in range(2) for e in range(2) for j0 in range(2)]
                A = lambda rb: [(P(act, rb, r), 10) for r in range(0, g2 * 16, 8)]
                H = lambda rb: [_operands(LHS, lambda i, j, e=e: h_s[4 * i + j, e * 16:(e + 1) * 16, :], pc, ha_s[rb % 3],
                                          pl.ds(e % (g2 // 2) * 8, 8), e // (g2 // 2) * 128, scaled=True, src=h_s)
                                for e in range(g2)]
                bu, bn = prep(wu_s, c & 1, bb_s, 3), prep(wg_s, nxt & 1, ba_s, 0)
                plan = [(P(up, 0, 0), bu, 1), (P(up, 0, 1), bd[:nbd], 0), (P(up, 1, 0), A(0), 0), (P(up, 1, 1), _mix(H(0), bd[nbd:]), 1),
                        (P(down, 0), A(1), 0), (P(up, 2, 0), H(1), 0), (P(up, 2, 1), bo, 0), (P(up, 3, 0), A(2), 0),
                        (P(up, 3, 1), H(2) + bn[:nbn], 0), (P(down, 1), A(3), 0), (P(down, 2), H(3), 1),
                        (P(down, 3), bn[nbn:], 1)]
                done = 0
                for i, (products, tasks, early) in enumerate(plan):
                    upto = len(att) * sum(aw[:i + 1]) // sum(aw)
                    pc.add(_mix(tasks, att[done:upto]), NP * g2 * 8 - 320 * early)
                    done = upto
                    products()
                    pc.finish()

            if only in (None, 2):
                jax.named_call(lambda: lax.fori_loop(0, NC, phase2, None), name='p2')()

            def out_cp(t):
                r = _ds(t * g3 * GT, g3 * GT, g3 * GT)
                return pltpu.make_async_copy(x_s.at[r, :], out_h.at[r, :], so.at[t])

            def out_tasks(pc, dst, e):
                def out(r):
                    s = yield from _result(pc, z_s[e], pl.ds(r, 8))
                    for i in range(4):
                        rows = pl.ds(r // 16 * GT + i * 16 + r % 16, 8)
                        if i % 2 == 0:
                            pc.open(zz_s[e])
                        v = jnp.concatenate([s[i][j] * zz_s[e][4 * i + j, r:r + 8, :] for j in range(4)], axis=1)
                        v = dst[rows, e * CW:(e + 1) * CW].astype(f32) + v
                        dst[rows, e * CW:(e + 1) * CW] = v.astype(bf16)
                        pc.done(_tile(v, 3))
                        if i % 2:
                            yield

                return [(P(out, r), 5) for r in range(0, g3 * 16, 8)]

            def phase3(t, _):
                pc = pace(d3)
                z = [zero_s[i] & 1 for i in range(4)]
                nb = NG // g3 // n3
                y0 = pl.multiple_of(t * (nb * g3 * 16), nb * g3 * 16)
                rows = lambda tb: x_s.at[_ds(tb * g3 * GT, g3 * GT, g3 * GT), :]
                for rb in range(nb):
                    tb = t * nb + rb
                    for e in range(2):
                        def gate(r):
                            y = yield from _result(pc, y_s, pl.ds(y0 + rb * g3 * 16 + r, 8), e * NZ)
                            for n in range(16):
                                h = y[n // 4][n % 4] * pc.const(0.25 / XS ** 2, 8)
                                zz_s[e][n, r:r + 8, :] = h = h * jnp.tanh(h) + h
                                if n % 8 == 7:
                                    pc.done(h)
                                    yield

                        def emit(n, v):
                            z_s[e][n, 0:g3 * 16, :] = v

                        outs = out_tasks(pc, rows(tb if e else jnp.where(tb > 0, tb - 1, NG // g3)), 1 - e)
                        pc.add(_mix(outs, [(P(gate, r), 5) for r in range(0, g3 * 16, 8)]), NP * g3 * 8)
                        _products(lambda n: pc.dot(o_s[n + z[e], _ds(tb * g3 * 8, g3 * 8, g3 * 8), :],
                                                   _unpack(bo_s[n + z[rb], 0:128, e * 128:(e + 1) * 128])), emit, e)
                        pc.finish()
                        if e == 0:
                            pl.when(tb > 0)(lambda: out_cp(jnp.maximum(tb - 1, 0)).start())

            x_s[S:, :] = jnp.zeros((g3 * GT, D), bf16)
            if only in (None, 3):
                jax.named_call(lambda: lax.fori_loop(0, n3, phase3, None), name='p3')()
            run(out_tasks(free, x_s.at[S - g3 * GT:S, :], 1))
            out_cp(NG // g3 - 1).start()
            for t in range(NG // g3):
                out_cp(t).wait()

        mix(*mix_s)

    def fn(A_x, A_wqkv, A_wo, B_x, B_w_gate, B_w_up, B_w_down):
        any_spec = pl.BlockSpec(memory_space=pl.ANY)
        out = pl.pallas_call(
            kern,
            in_specs=[any_spec] * 6,
            out_specs=any_spec,
            out_shape=jax.ShapeDtypeStruct((S, D), bf16),
            scratch_shapes=[
                pltpu.VMEM((S + g3 * GT, D), bf16),
                pltpu.VMEM((NP + 1, S // 8 + 8, D // 4), u32),
                pltpu.VMEM((24, S + PAD, 128), f32),
                pltpu.VMEM((2 * NZ + 4, S // 4 + 8, 128), f32),
                pltpu.VMEM((8, D // 4 + 16, CW), bf16),
                pltpu.VMEM((8, D // 4 + 16, CW), bf16),
                pltpu.VMEM((2, CW + 16, D), bf16),
                pltpu.VMEM((1, D + 16, D), bf16),
                pltpu.VMEM((NP + 1, 72, 256), u32),
                pltpu.VMEM((NP + 1, 72, 256), u32),
                pltpu.VMEM((NP + 1, 72, 256), u32),
                pltpu.VMEM((NP + 1, 136, 256), u32),
                [pltpu.VMEM((NZ + 4, g2 * 16 + 8, 128), f32)] * 2,
                [pltpu.VMEM((7, 4, D // 4, CW), bf16), [pltpu.VMEM((20, 8, 128), u32)] * 4],
                [pltpu.VMEM((NP + 1, S // 8 + 8, D // 4), u32), pltpu.VMEM((18, g2 * 16 + 16, 128), f32),
                      [pltpu.VMEM((NP + 1, g2 * 4 + 8, 256), u32)] * 3, [pltpu.VMEM((NZ + 4, g2 * 16 + 8, 128), f32)] * 2,
                      [pltpu.VMEM((4 * W + 2, 16, 128), f32)] * 5, pltpu.VMEM((34, 16, 128), f32)],
                pltpu.SemaphoreType.DMA((NX,)),
                pltpu.SemaphoreType.DMA((2 * NX,)),
                pltpu.SemaphoreType.DMA((7,)),
                pltpu.SemaphoreType.DMA((1,)),
                pltpu.SemaphoreType.DMA((NC,)),
                pltpu.SemaphoreType.DMA((NC,)),
                pltpu.SemaphoreType.DMA((NC,)),
                pltpu.SemaphoreType.DMA((NG // g3,)),
                pltpu.SMEM((4,), i32),
            ],
            compiler_params=pltpu.CompilerParams(vmem_limit_bytes=127 << 20, flags=flags, disable_bounds_checks=nbc),
        )(A_x.reshape(S, D), A_wqkv.reshape(4, D // 4, 3 * D), A_wo, B_w_gate.reshape(4, D // 4, F),
          B_w_up.reshape(4, D // 4, F), B_w_down)
        return out.reshape(1, S, D)

    return fn


@jax.jit
def pallas_recurrent_scan__sliding_local_dilated__geglu_ffn__prompt_kernel(
    A_x, A_wqkv, A_wo, B_x, B_w_gate, B_w_up, B_w_down
):
    return make()(A_x, A_wqkv, A_wo, B_x, B_w_gate, B_w_up, B_w_down)
```

```python
import functools
import math

import jax
import jax.numpy as jnp
from jax import lax
import jax.experimental.pallas as pl
import jax.experimental.pallas.tpu as pltpu

S, D, F = 2048, 1024, 3584
DH, W, DIL = 32, 8, 2
PAD = 16
NP = 49
NZ = 28
GT = 64
NG = S // GT
CW = 512
NC = F // CW
NA = -(-NG // NC)
LOG2E = math.log2(math.e)
C0 = math.sqrt(2.0 / math.pi)
XS = (C0 * 0.044715) ** (1.0 / 3.0)
f32, bf16, u32, i32 = jnp.float32, jnp.bfloat16, jnp.uint32, jnp.int32
P = functools.partial


def _pack(v):
    return pltpu.bitcast(v.astype(bf16), u32)


def _unpack(v):
    return pltpu.bitcast(v, bf16)


def _ds(start, size, align):
    if isinstance(start, int):
        return pl.ds(start, size)
    return pl.ds(pl.multiple_of(start, align), size)


def _tile(v, j):
    return v[:, j * 128:(j + 1) * 128]


def _stacked(ref, n, rows):
    return jnp.concatenate([ref[n, 0:rows, k:k + 128] for k in (0, 128)], axis=0)


def _lane_bit(shape, bit):
    return (lax.broadcasted_iota(i32, shape, 1) & bit) == 0


def _sum(vs):
    return functools.reduce(lambda a, b: a + b, vs)


class _Pace:
    def __init__(self, zero=None, lag=256):
        self.zero, self.lag = zero, lag
        self.always = None if zero is None else zero == 0
        self.tok, self.time, self.tiles, self.due, self.queues = None, 0, 0, [], []

    def add(self, tasks, cycles):
        if tasks:
            steps = (None for fn, _ in tasks for _ in fn())
            self.queues.append([steps, sum(n for _, n in tasks), cycles, 0, 0])

    def finish(self):
        for q in self.queues:
            for _ in q[0]:
                pass
        self.queues = []

    def dot(self, lhs, rhs):
        rows, nk = 2 * lhs.shape[0], lhs.shape[1] // 128
        t0 = self.tiles // 4 * rows
        part = range(rows * (self.tiles % 4) // 4, rows * (self.tiles % 4 + nk) // 4)
        self.tiles += nk
        if self.due and self.due[0][0] < t0 + part.stop:
            col = [lhs[r:r + 8, 0:128] for r in range(0, rows // 2, 8)]
            toks = {}
            while self.due and self.due[0][0] < t0 + part.stop:
                t, tok = self.due.pop(0)
                toks.setdefault(max(t - t0, 0) // 16, []).append(pltpu.bitcast(tok, u32))
            for i, ts in toks.items():
                col[i] = jnp.where(self.always, col[i], functools.reduce(lambda a, b: a | b, ts))
            lhs = jnp.concatenate(
                [jnp.concatenate(col, axis=0)] + [_tile(lhs, j) for j in range(1, nk)], axis=1)
        y = jnp.dot(_unpack(lhs), _unpack(rhs), preferred_element_type=f32)
        for r in part[::8]:
            self.tok, self.time = functools.cache(lambda r=r: y[r:r + 8]), t0 + r
            for q in self.queues:
                q[3] += 8
                while q[4] < min(q[1], q[1] * q[3] // q[2]):
                    q[4] += 1
                    next(q[0], None)
        return y

    def const(self, c, rows):
        if self.zero is None or self.tok is None:
            return c
        return jnp.concatenate([jnp.where(self.always, c, self.tok())] * (rows // 8), axis=0)

    def gate(self, v):
        if self.zero is None or self.tok is None:
            return v
        return jnp.where(self.always, v, jnp.concatenate([self.tok()] * (v.shape[0] // 8), axis=0))

    def open(self, ref):
        if self.zero is not None and self.tok is not None:
            if ref.dtype == bf16:
                ref[self.zero, ref.shape[1] - 16:, 0:128] = pltpu.bitcast(self.tok(), bf16)
            else:
                ref[ref.shape[0] - 1 + self.zero, 0:8, 0:128] = pltpu.bitcast(self.tok(), ref.dtype)
        return ref

    def done(self, v, extra=0):
        if self.zero is not None:
            self.due.append((self.time + self.lag + extra, v[-8:]))
            self.due.sort(key=lambda d: d[0])
        return v

    def stored(self, ref, extra=0):
        if self.zero is not None:
            self.done(ref[ref.shape[0] - 1 + self.zero, ref.shape[1] - 8:, 0:128], extra)


def _run(tasks):
    for fn, _ in tasks:
        for _ in fn():
            pass


def _skewed(units):
    order = sorted((u + s, u, s) for u, st in enumerate(units) for s in range(len(st)))
    return [t for _, u, s in order for t in units[u][s]]


def _mix(*lists):
    keyed = []
    for i, ts in enumerate(lists):
        total, at = sum(n for _, n in ts), 0
        for t in ts:
            keyed.append(((at + t[1] / 2) / total, i, t))
            at += t[1]
    return [t for _, _, t in sorted(keyed, key=lambda k: k[:2])]


LHS, RHS = (6, 3, 0, 2, 1, 4, 5), (6, 0, 5, 4, 2, 1, 3)


def _basis(scaled, x11, x12, x21, x22):
    h = x21 if scaled else x21 * 0.5
    p = x11 + h
    return [x11 + x22, p, h + x22, (p + x22 + x12) * 0.5 if scaled else (p + x22) * 0.5 + x12]


def _unbasis(half, scaled, z0, z1, z2, z3):
    h = z0 * half
    e = z3 + h
    if scaled:
        return [e + z2, z2 + h + z1, h, e + z1]
    return [e + z2, (z2 + h + z1) * 0.5, z0, e + z1]


def _operands(side, block, pc, src, ref, rows, col, scaled=False):
    def quad(a, b):
        pc.open(src)
        return _basis(scaled, *[block(2 * a + n // 2, 2 * b + n % 2) for n in range(4)])

    def put(k, x):
        t, p, q, r = x
        for n, v in zip(side, (t, p, q, r, t - p, q - t, r - t)):
            ref[pl.ds(7 * side[k] + n, 1), rows, pl.ds(col, 128)] = _pack(v[None])
        pc.stored(ref)

    def steps():
        h = quad(1, 0) if scaled else [v * 0.5 for v in quad(1, 0)]
        yield
        x11 = quad(0, 0)
        put(1, [a + b for a, b in zip(x11, h)])
        yield
        put(5, [b - a for a, b in zip(x11, h)])
        yield
        x22 = quad(1, 1)
        t = [a + b for a, b in zip(x11, x22)]
        put(0, t)
        yield
        put(2, [a + b for a, b in zip(x22, h)])
        yield
        put(4, [a - b for a, b in zip(x22, h)])
        yield
        r = [(a + b + c) * 0.5 if scaled else (a + b) * 0.5 + c for a, b, c in zip(t, h, quad(0, 1))]
        put(3, r)
        yield
        put(6, [a - b for a, b in zip(r, t)])
        yield

    return steps, 8


def _weight_operands(pc, src, load, ref, rows, col, flip=0):
    load = functools.cache(load)
    return _operands(RHS, lambda i, j: _tile(load(i, (j ^ flip) // 2), (j ^ flip) % 2),
                     pc, src, ref, rows, col)


def _products(prod, emit, odd=0):
    for o in range(7):
        m = lambda i: prod(7 * o + i)
        early = (o + odd) % 2
        t = m(6) if early else None
        a = m(0)
        t = t - a if early else a
        emit(o, a + m(1))
        a = m(2)
        t = t - a if early else t + a
        emit(7 + o, a + m(3))
        a = m(4)
        t = t + a if early else a - t
        emit(14 + o, m(5) - a)
        emit(21 + o, t if early else t + m(6))


def _result(pc, ref, rows, base=0, scaled=False):
    x = []
    for k in range(4):
        if k % 2 == 0:
            pc.open(ref)
        m = [ref[base + 7 * k + o, rows, :] for o in range(7)]
        x.append(_unbasis(0.5, scaled, m[0] + m[1], m[2] + m[3], m[5] - m[4], m[4] + m[6] - m[0] - m[2]))
        if k % 2:
            yield
    half = pc.const(0.5, 8)
    x = [_unbasis(half, scaled, *col) for col in zip(*x)]
    yield
    return [[x[2 * (i // 2) + j // 2][2 * (i % 2) + j % 2] for j in range(4)] for i in range(4)]


def _swap(mine, other, lvl, upper, plain=False):
    keep = (_lane_bit(mine.shape, 4 << lvl) ^ (upper == 1)) | plain
    return jnp.where(keep, mine, pltpu.roll(other, (4 << lvl) + upper * (128 - (8 << lvl)), 1))


def _attention_tasks(pc, a0, qkv_s, att_s, r_s, o_s, vo, xl):
    base = pl.multiple_of(a0 * GT, GT)
    win = qkv_s.at[:, pl.ds(base, NA * GT + PAD), :]

    def block(b):
        a_s = att_s[b % len(att_s)]

        def shifted(j):
            v = {r: win[j, pl.ds(b * 16 + PAD + r, 8), :] for r in range(8, -DIL * W, -DIL)}
            return [jnp.concatenate([v[-DIL * w], v[8 - DIL * w]], axis=0) for w in range(W)]

        def scores():
            st = [None] * W
            for j in range(8):
                q = pc.gate(win[j, pl.ds(b * 16 + PAD, 16), :])
                for w, k in enumerate(shifted(8 + j)):
                    st[w] = q * k if j == 0 else st[w] + q * k
                pc.done(st[W - 1])
                yield
            for w in range(W):
                a_s[w] = st[w] + pltpu.roll(st[w], 127, 1)
            pc.stored(a_s, xl)

        def reduce():
            pc.open(a_s)
            for w in range(W):
                t = a_s[w]
                a_s[W + w] = t + pltpu.roll(t, 126, 1)
            pc.stored(a_s, xl)
            yield

        def softmax():
            pc.open(a_s)
            logits = []
            for w in range(W):
                t = a_s[W + w] * (DH ** -0.5 * LOG2E / XS ** 2)
                if b == 0 and w:
                    row = lax.broadcasted_iota(i32, (16, 128), 0) + base
                    t = jnp.where(row >= DIL * w, t, -1e9 * LOG2E)
                logits.append(t)
            m = functools.reduce(jnp.maximum, logits)
            yield
            m = pc.gate(m)
            e = [jnp.exp2(t - m) for t in logits]
            inv = (1.0 / XS) / _sum(e)
            yield
            inv = pc.gate(inv)
            for w in range(W):
                t = e[w] * inv
                a_s[2 * W + w] = jnp.where(_lane_bit((16, 128), 1), t, pltpu.roll(t, 1, 1))
            pc.stored(a_s, xl)
            yield

        def spread():
            pc.open(a_s)
            for w in range(W):
                t = a_s[2 * W + w]
                a_s[3 * W + w] = jnp.where(_lane_bit((16, 128), 2), t, pltpu.roll(t, 2, 1))
            pc.stored(a_s, xl)
            yield

        def values():
            for j in range(8):
                if j % vo == 0:
                    pc.open(a_s)
                    p = [a_s[3 * W + w] for w in range(W)]
                v = shifted(16 + j)
                r_s[b % 4 * 8 + j] = pc.done(_sum([p[w] * (v[w] if w else pc.gate(v[w])) for w in range(W)]))
                yield

        tail = [_operands(LHS, lambda i, j, e=e: r_s[i * 8 + 2 * j + e], pc, r_s, o_s,
                          _ds((a0 + b // 4) * 8, 8, 8), e * 128) for e in range(2) if b % 4 == 3]
        return [[(scores, 8)], [(reduce, 1)], [(softmax, 3)], [(spread, 1)], [(values, 8)] + tail]

    return _skewed([block(b) for b in range(NA * 4)])


def make(only=None, flags=None, scopes=False, nsc=False,
         d0=192, d1=256, d2=224, d3=256, vo=2, nbn=8, nbd=12, xl=128, hc=12, sb=4, early=320,
         cutz=(0, 4, 7, 10, 12), cuts=(0, 22, 44, 64, 64), aw=(1, 2, 2, 5, 1, 6, 6, 2, 2, 1, 4, 4)):
    def loop(i, lo, hi, body):
        if only is None or i in only:
            fn = lambda: lax.fori_loop(lo, hi, body, None)
            (jax.named_call(fn, name=f"p{i}") if scopes else fn)()

    def kern(x_h, wqkv_h, wo_h, wg_h, wu_h, wd_h, out_h,
             x_s, wqkv_s, wo_s, wg_s, wu_s, wd_s, xa_s, o_s, ha_s, ba_s, bb_s, bd_s, bo_s,
             qkv_s, y_s, z_s, h_s, att_s, r_s, sw_s, sx, sq, sw, so, zero_s):
        free = _Pace()

        def x_cp(t):
            r = _ds(t * 4 * GT, 4 * GT, 4 * GT)
            return pltpu.make_async_copy(x_h.at[r, :], x_s.at[r, :], sx.at[t])

        def q_cps(t):
            r = _ds(t * 32, 32, 32)
            return [pltpu.make_async_copy(wqkv_h.at[:, r, pl.ds(p * CW, CW)], wqkv_s.at[p, :, r, :], sq.at[t])
                    for p in range(2)]

        def qkv_cp(p):
            src = wqkv_h.at[:, :, pl.ds(p * CW, CW)] if p < 6 else wg_h.at[:, :, pl.ds(0, CW)]
            return pltpu.make_async_copy(src, wqkv_s.at[p], sq.at[p])

        def up_cp(si, c):
            dst = (wg_s, wu_s)[si].at[pl.ds((c & 1) * 4, 4), pl.ds(0, D // 4)]
            return pltpu.make_async_copy((wg_h, wu_h)[si].at[:, :, _ds(c * CW, CW, CW)], dst, sw.at[2 * si + (c & 1)])

        def down_cp(c):
            return pltpu.make_async_copy(
                wd_h.at[_ds(c * CW, CW, CW), :], wd_s.at[c & 1, pl.ds(0, CW)], sw.at[4 + (c & 1)])

        def out_cp(row, rows, e):
            r = _ds(row, rows, GT)
            return pltpu.make_async_copy(x_s.at[r, pl.ds(e * CW, CW)], out_h.at[r, pl.ds(e * CW, CW)], so.at[0])

        wo_cp = pltpu.make_async_copy(wo_h, wo_s.at[0, pl.ds(0, D)], sq.at[7])

        def start_if(cond, *cps):
            for cp in cps:
                pl.when(cond)(lambda: cp.start())

        def wait_if(cond, *cps):
            for cp in cps:
                pl.when(cond)(lambda: cp.wait())

        def zeros():
            return [zero_s[i] & 1 for i in range(4)]

        def center_task(pc, t, b):
            def steps():
                v = x_s[_ds(t * 256 + b * 16, 16, 16), :].astype(f32)
                v = pc.done(_sum([pc.gate(_tile(v, 0))] + [_tile(v, j) for j in range(1, 8)]))
                att_s[0][b] = jnp.broadcast_to(jnp.sum(v, axis=1, keepdims=True) * (1.0 / D), (16, 128))
                yield

            return steps, 1

        def scale_task(pc, t, b, z=0):
            def steps():
                v, m = x_s[_ds((t + z) * 256 + b * 16, 16, 16), :].astype(f32), pc.gate(att_s[0][b + z])
                v = [_tile(v, j) - m for j in range(8)]
                v = jnp.sum(pc.done(_sum([a * a for a in v])), axis=1, keepdims=True) * (1.0 / D)
                att_s[1][b] = jnp.broadcast_to(lax.rsqrt(v + 1e-5) * XS, (16, 128))
                yield
                yield

            return steps, 2

        def norm_task(pc, t, g, e, z=0):
            def block(i, j):
                v = x_s[_ds((t + z) * 256 + g * GT + i * 16, 16, 16), _ds((2 * j + e) * 128, 128, 128)]
                return (v.astype(f32) - att_s[0][4 * g + i]) * att_s[1][4 * g + i + z]

            return _operands(LHS, block, pc, att_s[0], xa_s, _ds(t * 32 + g * 8, 8, 8), _ds(e * 128, 128, 128).start)

        def qkv_tasks(pc, job, ref, units, plain=False):
            def unit(u, t_s):
                st = {}

                def swap(lvl):
                    for i in range(4):
                        if lvl == 2:
                            a, b = [_pack(wqkv_s[s, i, _ds(u * 16, 16, 16), :])
                                    for s in (job, jnp.where(plain, job, job ^ 1))]
                            st[i] = [_swap(_tile(a, c), _tile(b, c), 2, job & 1, plain) for c in range(4)]
                        else:
                            st[i] = [_swap(st[i][c], st[i][c ^ (1 << lvl)], lvl, c >> lvl & 1, plain)
                                     for c in range(4)]
                        if lvl == 0:
                            for c in range(4):
                                t_s[4 * i + c] = st[i][c]
                    yield

                return [[(P(swap, lvl), 1)] for lvl in (2, 1, 0)] + [[
                    _operands(RHS, lambda i, j: _unpack(t_s[4 * i + j]).astype(f32), pc, t_s, ref,
                              _ds((u & 7) * 8, 8, 8), _ds((u >> 3) * 128, 128, 128).start)]]

            return _skewed([unit(u, sw_s[n % 4]) for n, u in enumerate(units)])

        def put_tasks(pc, src, job, g, ng):
            def put(r):
                res = yield from _result(pc, src, pl.ds(r, 8))
                for j in range(4):
                    for i in range(4):
                        qkv_s[4 * job + j, _ds((g + r // 16) * GT + i * 16 + r % 16 + PAD, 8, 8), :] = res[i][j]
                pc.done(res[0][3])

            return [(P(put, r), 3) for r in range(0, ng * 16, 8)]

        def keep(ref, rows):
            def emit(n, v):
                ref[n, 0:rows, :] = v

            return emit

        for cp in [x_cp(0)] + [cp for t in range(8) for cp in q_cps(t)] + [x_cp(1)]:
            cp.start()
        for i in range(4):
            zero_s[i] = 0
        for ref in [xa_s, o_s, ba_s, bb_s, bd_s, bo_s] + ha_s + att_s:
            ref[ref.shape[0] - 1, ref.shape[1] - 8:, 0:128] = jnp.zeros((8, 128), ref.dtype)

        def clear(i, _):
            y_s[0:8, _ds(i * 32, 32, 32), :] = jnp.zeros((8, 32, 128), f32)
            z_s[1][0:NZ, _ds(i * 8, 8, 8), :] = jnp.zeros((NZ, 8, 128), f32)
            for ref in att_s[:2]:
                ref[i] = jnp.zeros((16, 128), f32)
            h_s[0:8, _ds(i * 8, 8, 8), :] = jnp.zeros((8, 8, 128), f32)
            x_s[_ds(S + i * 16, 16, 16), :] = jnp.zeros((16, D), bf16)

        lax.fori_loop(0, 16, clear, None)
        turn = (lax.broadcasted_iota(i32, (128, 128), 0) - lax.broadcasted_iota(i32, (128, 128), 1)) & 127
        for c in range(8):
            bb_s[c, 0:64, 0:128] = jnp.zeros((64, 128), u32)
            bb_s[c:c + 1, 0:64, 128:256] = _pack(jnp.where(turn == 4 * c, 1.0, 0.0)[None])

        def startup(it, _):
            wait_if(it < 8, *q_cps(jnp.minimum(it, 7)))
            u = [jnp.clip(it - s, 0, 7) for s in range(3)]
            _run([_operands(RHS, lambda i, j, r=r, p=p: h_s[4 * p + j, pl.ds(i * 32 + r * 16, 16), :], free, None,
                            ref, _ds((u[2] & 3) * 16 + r * 8, 8, 8), pl.multiple_of((u[2] >> 2) * 128, 128))
                  for r in range(2) for p, ref in enumerate((bd_s, bo_s))])
            for c in range(8):
                h_s[c, 0:128, :] = free.dot(bb_s[c, 0:64, 0:128], bb_s[c, 0:64, 128:256])
            _run([norm_task(free, 0, u[2] >> 1, u[2] & 1)] + [center_task(free, 0, 2 * u[0] + b) for b in range(2)])
            for i in range(8):
                v = [_pack(wqkv_s[p, i // 2, _ds(u[0] * 32 + i % 2 * 16, 16, 16), :]) for p in range(2)]
                v = [pltpu.roll(_tile(v[c // 4], c % 4), 4 * c, 1) if c else _tile(v[0], 0) for c in range(8)]
                v = [v[-c] for c in range(8)]
                for b in (1, 2, 4):
                    v = [jnp.where(_lane_bit((8, 128), 4 * b), v[c], v[c - b]) for c in range(8)]
                for c in range(8):
                    bb_s[c, i * 8:(i + 1) * 8, 0:128] = v[c]
                if i == 3:
                    _run([scale_task(free, 0, 2 * u[0] + b) for b in range(2)])
            start_if(it == 7, x_cp(2), qkv_cp(2), qkv_cp(3), x_cp(3))

        x_cp(0).wait()
        loop(0, 0, 10, startup)

        def phase_q(t, _):
            wait_if(t < 7, x_cp(jnp.minimum(t + 1, 7)))
            wait_if(t == 2, qkv_cp(2), qkv_cp(3))
            pc = _Pace(zero_s[0], d0)
            z = zeros()
            nxt = jnp.minimum(t + 1, 7)
            prep = qkv_tasks(pc, jnp.where(t < 2, 0, 2), ba_s, [jnp.clip(3 * t - 6, 0, 13) + i for i in range(3)])

            def first(n):
                ha_s[0][n, 0:32, :] = v = xa_s[n, _ds(t * 32, 32, 32), :]
                return v

            pc.add(_mix(put_tasks(pc, z_s[1], 1, jnp.maximum(t - 1, 0) * 4, 4), prep[:hc],
                        [center_task(pc, nxt, b) for b in range(16)] + [scale_task(pc, nxt, b, z[0]) for b in range(16)]), NP * 32)
            _products(lambda n: pc.dot(first(n), _stacked(bd_s, n, 64)), keep(z_s[0], 64))
            pc.finish()
            pc.add(_mix(put_tasks(pc, z_s[0], 0, t * 4, 4), prep[hc:], [norm_task(pc, nxt, g, e, z[1]) for g in range(4) for e in range(2)]), NP * 32)
            _products(lambda n: pc.dot(ha_s[0][n + z[0], 0:32, :], _stacked(bo_s, n, 64)), keep(z_s[1], 64), 1)
            pc.finish()
            start_if(t == 1, *[x_cp(i) for i in range(4, 8)])

        loop(1, 0, 8, phase_q)
        for cp in (qkv_cp(4), qkv_cp(5), qkv_cp(6), wo_cp, up_cp(1, 0), down_cp(0), up_cp(0, 1),
                   up_cp(1, 1), down_cp(1), up_cp(0, 2)):
            cp.start()
        _run(put_tasks(free, z_s[1], 1, NG - 4, 4))

        def phase_kv(job, _):
            wait_if(job == 3, qkv_cp(4), qkv_cp(5))
            wait_if(job == 5, qkv_cp(6), wo_cp)
            pc = _Pace(zero_s[0], d1)
            z = zeros()
            prep = qkv_tasks(pc, job + 1, bb_s, range(16), job == 5)

            def clear_y(n):
                for r in range(0, S // 4, 64):
                    y_s[12 * job - 16 + n, r:r + 64, :] = pc.const(0.0, 64)
                    yield

            for rb in range(4):
                def prod(n):
                    y = pc.dot(xa_s[n, rb * 64:(rb + 1) * 64, :], _stacked(ba_s, n + z[rb] if rb < 3 else n, 64))
                    if rb == 3:
                        ba_s[n, 0:64, :] = pc.open(bb_s)[n, 0:64, :]
                    return y

                puts = put_tasks(pc, z_s[1 - rb % 2], job if rb else jnp.maximum(job - 1, 2), (rb - 1) % 4 * 8, 8)
                pc.add(_mix(puts, prep[cuts[rb]:cuts[rb + 1]]), NP * 64 - (256 if rb == 3 else 0))
                pc.add([(P(clear_y, n), 8) for n in range(cutz[rb], cutz[rb + 1])], NP * 64)
                _products(prod, keep(z_s[rb % 2], 128), rb)
                pc.finish()

        loop(2, 2, 6, phase_kv)
        _run(put_tasks(free, z_s[1], 5, NG - 8, 8))
        for j in range(8, 24):
            qkv_s[j, 0:PAD, :] = jnp.broadcast_to(qkv_s[j, PAD:PAD + 1, :], (PAD, 128))

        def phase_ffn(c, _):
            nxt = jnp.minimum(c + 1, NC - 1)
            up_cp(1, c).wait()
            down_cp(c).wait()
            wait_if(c + 1 < NC, up_cp(0, nxt))
            pc = _Pace(zero_s[0], d2)
            z = zeros()

            def up(rb, si):
                _products(lambda n: pc.dot(xa_s[n, rb * 64:(rb + 1) * 64, :], _stacked((ba_s, bb_s)[si], n + z[rb], 64)),
                          keep(z_s[rb % 2 * 2 + si], 128), pc.tiles // 2)

            def down(rb):
                for e in range(2):
                    def emit(n, v):
                        y_s[e * NZ + n, rb * 128:(rb + 1) * 128, :] += v

                    _products(lambda n: pc.dot(_stacked(ha_s[rb % 3], n + z[e + rb // 3 * 2], 32),
                                               bd_s[n + z[rb], 0:64, e * 128:(e + 1) * 128]), emit, e)

            def act(rb, r):
                g = yield from _result(pc, z_s[rb % 2 * 2], pl.ds(r, 8), scaled=True)
                u = yield from _result(pc, z_s[rb % 2 * 2 + 1], pl.ds(r, 8))
                for n in range(16):
                    i, j = n // 4, n % 4
                    s = 2.0 ** (j // 2 - i // 2 + j % 2 - i % 2)
                    t = pc.gate(g[i][j])
                    v = t * t if s == 1 else t * t * s ** -3
                    p = t * u[i][j ^ 3]
                    h_s[n, r:r + 8, :] = v = p * jnp.tanh(t * (v + C0 / XS / s)) + p
                    if j == 3:
                        pc.done(v)
                        yield

            def up_operands(w_s, slot, ref, flip):
                return [_weight_operands(
                    pc, w_s, lambda i, h, r=k + r: w_s[4 * slot + i, pl.ds(r, 16), pl.ds(h * 256, 256)].astype(f32),
                    ref, pl.ds(r // 2, 8), k, flip) for k in (0, 128) for r in range(0, 128, 16)]

            def out_operands(u, e, j0):
                def load(i, h):
                    lo = lax.broadcasted_iota(i32, (8, 256), 0) < 4
                    v = [wo_s[0, _ds((u & 1) * 512 + (u >> 1) * 32 + k * 128 + i * 8, 8, 8),
                              pl.ds(e * CW + h * 256, 256)].astype(f32) for k in range(4)]
                    return jnp.concatenate([
                        jnp.where(lo, pltpu.roll(a, 4, 0), b) if j0 else jnp.where(lo, a, pltpu.roll(b, 4, 0))
                        for a, b in (v[:2], v[2:])], axis=0)

                return _weight_operands(pc, wo_s, load, bo_s, _ds(j0 * 64 + u * 8, 8, 8), e * 128, 3)

            bu, bn = up_operands(wu_s, c & 1, bb_s, 3), up_operands(wg_s, nxt & 1, ba_s, 0)
            bd = [_weight_operands(
                pc, wd_s, lambda i, h, e=e, r=r: wd_s[c & 1, pl.ds(i * 128 + r, 16), pl.ds(e * CW + h * 256, 256)].astype(f32),
                bd_s, pl.ds(r // 2, 8), e * 128) for e in range(2) for r in range(0, 128, 16)]
            bo = [out_operands((2 * c + u) & 7, e, j0) for u in range(2) for e in range(2) for j0 in range(2)]
            acts = lambda rb: [(P(act, rb, r), 10) for r in range(0, 128, 8)]
            sums = lambda rb: [_operands(LHS, lambda i, j, e=e: h_s[4 * i + j, e * 16:(e + 1) * 16, :], pc, h_s,
                                         ha_s[rb % 3], pl.ds(e % 4 * 8, 8), e // 4 * 128, True) for e in range(8)]
            att = _attention_tasks(pc, jnp.minimum(c * NA, NG - NA), qkv_s, att_s, r_s, o_s, vo, xl)
            plan = [(P(up, 0, 0), bu, early), (P(up, 0, 1), bd[:nbd], 0),
                    (P(up, 1, 0), acts(0), 0), (P(up, 1, 1), _mix(sums(0), bd[nbd:]), early),
                    (P(down, 0), acts(1), 0), (P(up, 2, 0), sums(1), 0), (P(up, 2, 1), bo, 0),
                    (P(up, 3, 0), acts(2), 0), (P(up, 3, 1), sums(2) + bn[:nbn], 0),
                    (P(down, 1), acts(3), 0), (P(down, 2), sums(3), early), (P(down, 3), bn[nbn:], early)]
            for i, (products, tasks, slack) in enumerate(plan):
                lo, hi = [len(att) * sum(aw[:k]) // sum(aw) for k in (i, i + 1)]
                pc.add(_mix(tasks, att[lo:hi]), NP * 64 - slack)
                products()
                pc.finish()
            start_if(c + 2 < NC, up_cp(1, jnp.minimum(c + 2, NC - 1)), down_cp(jnp.minimum(c + 2, NC - 1)))
            start_if(c + 3 < NC, up_cp(0, jnp.minimum(c + 3, NC - 1)))

        loop(3, 0, NC, phase_ffn)

        def out_tasks(pc, dst, e):
            def out(r):
                s = yield from _result(pc, z_s[e], pl.ds(r, 8))
                for i in range(4):
                    rows = pl.ds(r // 16 * GT + i * 16 + r % 16, 8)
                    if i % 2 == 0:
                        pc.open(z_s[2 + e])
                    v = jnp.concatenate([s[i][j ^ 3] * z_s[2 + e][4 * i + j, r:r + 8, :] for j in range(4)], axis=1)
                    v = dst[rows, e * CW:(e + 1) * CW].astype(f32) + v
                    dst[rows, e * CW:(e + 1) * CW] = v.astype(bf16)
                    pc.done(_tile(v, 0))
                    if i % 2:
                        yield

            return [(P(out, r), 5) for r in range(0, 64, 8)]

        def phase_out(t, _):
            pc = _Pace(zero_s[0], d3)
            z = zeros()
            y0 = pl.multiple_of(t * 128, 128)
            for rb in range(2):
                tb = 2 * t + rb
                for e in range(2):
                    def gate(r):
                        y = yield from _result(pc, y_s, pl.ds(y0 + rb * 64 + r, 8), e * NZ)
                        for n in range(16):
                            if n % 8 == 0:
                                scale = pc.const(0.25 / XS ** 2, 8)
                            h = y[n // 4][n % 4] * scale
                            z_s[2 + e][n, r:r + 8, :] = h = h * jnp.tanh(h) + h
                            if n % 8 == 7:
                                pc.done(h)
                                yield

                    prev = tb if e else jnp.where(tb > 0, tb - 1, NG // 4)
                    outs = out_tasks(pc, x_s.at[_ds(prev * 4 * GT, 4 * GT, 4 * GT), :], 1 - e)
                    pc.add(_mix(outs, [(P(gate, r), 5) for r in range(0, 64, 8)]), NP * 32)
                    _products(lambda n: pc.dot(o_s[n + z[e], _ds(tb * 32, 32, 32), :],
                                               bo_s[n + z[rb], 0:128, e * 128:(e + 1) * 128]), keep(z_s[e], 64), e)
                    pc.finish()
                    start_if(prev < NG // 4, out_cp(jnp.minimum(prev, NG // 4 - 1) * 4 * GT, 4 * GT, 1 - e))

        loop(4, 0, 4, phase_out)
        last = out_tasks(free, x_s.at[S - 4 * GT:S, :], 1)
        for g in range(4):
            _run(last[2 * g:2 * g + 2])
            out_cp(S - (4 - g) * GT, GT, 1).start()
        pltpu.make_async_copy(x_s.at[pl.ds(0, S), :], out_h, so.at[0]).wait()

    def fn(A_x, A_wqkv, A_wo, B_x, B_w_gate, B_w_up, B_w_down):
        any_spec = pl.BlockSpec(memory_space=pl.ANY)
        out = pl.pallas_call(
            kern,
            in_specs=[any_spec] * 6,
            out_specs=any_spec,
            out_shape=jax.ShapeDtypeStruct((S, D), bf16),
            scratch_shapes=[
                pltpu.VMEM((S + 4 * GT, D), bf16),
                pltpu.VMEM((7, 4, D // 4, CW), bf16),
                pltpu.VMEM((1, D + 16, D), bf16),
                pltpu.VMEM((8, D // 4 + 16, CW), bf16),
                pltpu.VMEM((8, D // 4 + 16, CW), bf16),
                pltpu.VMEM((2, CW + 16, D), bf16),
                pltpu.VMEM((NP + 1, S // 8 + 8, 256), u32),
                pltpu.VMEM((NP + 1, S // 8 + 8, 256), u32),
                [pltpu.VMEM((NP + 1, 40, 256), u32)] * 3,
                pltpu.VMEM((NP + 1, 72, 256), u32),
                pltpu.VMEM((NP + 1, 72, 256), u32),
                pltpu.VMEM((NP + 1, 72, 256), u32),
                pltpu.VMEM((NP + 1, 136, 256), u32),
                pltpu.VMEM((24, S + PAD, 128), f32),
                pltpu.VMEM((2 * NZ + 4, S // 4 + 8, 128), f32),
                [pltpu.VMEM((NZ + 4, 136, 128), f32)] * 4,
                pltpu.VMEM((18, 144, 128), f32),
                [pltpu.VMEM((4 * W + 2, 16, 128), f32)] * 5,
                pltpu.VMEM((34, 16, 128), f32),
                [pltpu.VMEM((20, 8, 128), u32)] * 4,
                pltpu.SemaphoreType.DMA((8,)),
                pltpu.SemaphoreType.DMA((8,)),
                pltpu.SemaphoreType.DMA((6,)),
                pltpu.SemaphoreType.DMA((1,)),
                pltpu.SMEM((4,), i32),
            ],
            compiler_params=pltpu.CompilerParams(vmem_limit_bytes=127 << 20, flags=flags, disable_bounds_checks=nsc),
        )(A_x.reshape(S, D), A_wqkv.reshape(4, D // 4, 3 * D), A_wo,
          B_w_gate.reshape(4, D // 4, F), B_w_up.reshape(4, D // 4, F), B_w_down)
        return out.reshape(1, S, D)

    return fn


@jax.jit
def pallas_recurrent_scan__sliding_local_dilated__geglu_ffn__prompt_kernel(
    A_x, A_wqkv, A_wo, B_x, B_w_gate, B_w_up, B_w_down
):
    return make()(A_x, A_wqkv, A_wo, B_x, B_w_gate, B_w_up, B_w_down)
```

```python
import functools
import math

import jax
import jax.numpy as jnp
from jax import lax
import jax.experimental.pallas as pl
import jax.experimental.pallas.tpu as pltpu

S, D, F = 2048, 1024, 3584
DH, W, DIL = 32, 8, 2
PAD = 16
NP = 49
NZ = 28
GT = 64
NG = S // GT
CW = 512
NC = F // CW
NA = -(-NG // NC)
LOG2E = math.log2(math.e)
C0 = math.sqrt(2.0 / math.pi)
XS = (C0 * 0.044715) ** (1.0 / 3.0)
f32, bf16, u32, i32 = jnp.float32, jnp.bfloat16, jnp.uint32, jnp.int32
P = functools.partial


def _pack(v):
    return pltpu.bitcast(v.astype(bf16), u32)


def _unpack(v):
    return pltpu.bitcast(v, bf16)


def _ds(start, size, align):
    if isinstance(start, int):
        return pl.ds(start, size)
    return pl.ds(pl.multiple_of(start, align), size)


def _tile(v, j):
    return v[:, j * 128:(j + 1) * 128]


def _stacked(ref, n, rows):
    return jnp.concatenate([ref[n, 0:rows, k:k + 128] for k in (0, 128)], axis=0)


def _lane_bit(shape, bit):
    return (lax.broadcasted_iota(i32, shape, 1) & bit) == 0


def _sum(vs):
    return functools.reduce(lambda a, b: a + b, vs)


class _Pace:
    def __init__(self, zero=None, lag=256):
        self.zero, self.lag = zero, lag
        self.always = None if zero is None else zero == 0
        self.tok, self.time, self.tiles, self.due, self.queues = None, 0, 0, [], []

    def add(self, tasks, cycles):
        if tasks:
            steps = (None for fn, _ in tasks for _ in fn())
            self.queues.append([steps, sum(n for _, n in tasks), cycles, 0, 0])

    def finish(self):
        for q in self.queues:
            for _ in q[0]:
                pass
        self.queues = []

    def dot(self, lhs, rhs):
        rows, nk = 2 * lhs.shape[0], lhs.shape[1] // 128
        t0 = self.tiles // 4 * rows
        part = range(rows * (self.tiles % 4) // 4, rows * (self.tiles % 4 + nk) // 4)
        self.tiles += nk
        if self.due and self.due[0][0] < t0 + part.stop:
            col = [lhs[r:r + 8, 0:128] for r in range(0, rows // 2, 8)]
            toks = {}
            while self.due and self.due[0][0] < t0 + part.stop:
                t, tok = self.due.pop(0)
                toks.setdefault(max(t - t0, 0) // 16, []).append(pltpu.bitcast(tok, u32))
            for i, ts in toks.items():
                col[i] = jnp.where(self.always, col[i], functools.reduce(lambda a, b: a | b, ts))
            lhs = jnp.concatenate(
                [jnp.concatenate(col, axis=0)] + [_tile(lhs, j) for j in range(1, nk)], axis=1)
        y = jnp.dot(_unpack(lhs), _unpack(rhs), preferred_element_type=f32)
        for r in part[::8]:
            self.tok, self.time = functools.cache(lambda r=r: y[r:r + 8]), t0 + r
            for q in self.queues:
                q[3] += 8
                while q[4] < min(q[1], q[1] * q[3] // q[2]):
                    q[4] += 1
                    next(q[0], None)
        return y

    def const(self, c, rows):
        if self.zero is None or self.tok is None:
            return c
        return jnp.concatenate([jnp.where(self.always, c, self.tok())] * (rows // 8), axis=0)

    def gate(self, v):
        if self.zero is None or self.tok is None:
            return v
        return jnp.where(self.always, v, jnp.concatenate([self.tok()] * (v.shape[0] // 8), axis=0))

    def open(self, ref):
        if self.zero is not None and self.tok is not None:
            if ref.dtype == bf16:
                ref[self.zero, ref.shape[1] - 16:, 0:128] = pltpu.bitcast(self.tok(), bf16)
            else:
                ref[ref.shape[0] - 1 + self.zero, 0:8, 0:128] = pltpu.bitcast(self.tok(), ref.dtype)
        return ref

    def done(self, v, extra=0):
        if self.zero is not None:
            self.due.append((self.time + self.lag + extra, v[-8:]))
            self.due.sort(key=lambda d: d[0])
        return v

    def stored(self, ref, extra=0):
        if self.zero is not None:
            self.done(ref[ref.shape[0] - 1 + self.zero, ref.shape[1] - 8:, 0:128], extra)


def _run(tasks):
    for fn, _ in tasks:
        for _ in fn():
            pass


def _skewed(units):
    order = sorted((u + s, u, s) for u, st in enumerate(units) for s in range(len(st)))
    return [t for _, u, s in order for t in units[u][s]]


def _mix(*lists):
    keyed = []
    for i, ts in enumerate(lists):
        total, at = sum(n for _, n in ts), 0
        for t in ts:
            keyed.append(((at + t[1] / 2) / total, i, t))
            at += t[1]
    return [t for _, _, t in sorted(keyed, key=lambda k: k[:2])]


LHS, RHS = (6, 3, 0, 2, 1, 4, 5), (6, 0, 5, 4, 2, 1, 3)


def _basis(scaled, x11, x12, x21, x22):
    h = x21 if scaled else x21 * 0.5
    p = x11 + h
    return [x11 + x22, p, h + x22, (p + x22 + x12) * 0.5 if scaled else (p + x22) * 0.5 + x12]


def _unbasis(half, scaled, z0, z1, z2, z3):
    h = z0 * half
    e = z3 + h
    if scaled:
        return [e + z2, z2 + h + z1, h, e + z1]
    return [e + z2, (z2 + h + z1) * 0.5, z0, e + z1]


def _operands(side, block, pc, src, ref, rows, col, scaled=False):
    def quad(a, b):
        pc.open(src)
        return _basis(scaled, *[block(2 * a + n // 2, 2 * b + n % 2) for n in range(4)])

    def put(k, x):
        t, p, q, r = x
        for n, v in zip(side, (t, p, q, r, t - p, q - t, r - t)):
            ref[pl.ds(7 * side[k] + n, 1), rows, pl.ds(col, 128)] = _pack(v[None])
        pc.stored(ref)

    def steps():
        h = quad(1, 0) if scaled else [v * 0.5 for v in quad(1, 0)]
        yield
        x11 = quad(0, 0)
        put(1, [a + b for a, b in zip(x11, h)])
        yield
        put(5, [b - a for a, b in zip(x11, h)])
        yield
        x22 = quad(1, 1)
        t = [a + b for a, b in zip(x11, x22)]
        put(0, t)
        yield
        put(2, [a + b for a, b in zip(x22, h)])
        yield
        put(4, [a - b for a, b in zip(x22, h)])
        yield
        r = [(a + b + c) * 0.5 if scaled else (a + b) * 0.5 + c for a, b, c in zip(t, h, quad(0, 1))]
        put(3, r)
        yield
        put(6, [a - b for a, b in zip(r, t)])
        yield

    return steps, 8


def _weight_operands(pc, src, load, ref, rows, col, flip=0):
    load = functools.cache(load)
    return _operands(RHS, lambda i, j: _tile(load(i, (j ^ flip) // 2), (j ^ flip) % 2),
                     pc, src, ref, rows, col)


def _products(prod, emit, odd=0):
    for o in range(7):
        m = lambda i: prod(7 * o + i)
        early = (o + odd) % 2
        t = m(6) if early else None
        a = m(0)
        t = t - a if early else a
        emit(o, a + m(1))
        a = m(2)
        t = t - a if early else t + a
        emit(7 + o, a + m(3))
        a = m(4)
        t = t + a if early else a - t
        emit(14 + o, m(5) - a)
        emit(21 + o, t if early else t + m(6))


def _result(pc, ref, rows, base=0, scaled=False):
    x = []
    for k in range(4):
        if k % 2 == 0:
            pc.open(ref)
        m = [ref[base + 7 * k + o, rows, :] for o in range(7)]
        x.append(_unbasis(0.5, scaled, m[0] + m[1], m[2] + m[3], m[5] - m[4], m[4] + m[6] - m[0] - m[2]))
        if k % 2:
            yield
    half = pc.const(0.5, 8)
    x = [_unbasis(half, scaled, *col) for col in zip(*x)]
    yield
    return [[x[2 * (i // 2) + j // 2][2 * (i % 2) + j % 2] for j in range(4)] for i in range(4)]


def _swap(mine, other, lvl, upper, plain=False):
    keep = (_lane_bit(mine.shape, 4 << lvl) ^ (upper == 1)) | plain
    return jnp.where(keep, mine, pltpu.roll(other, (4 << lvl) + upper * (128 - (8 << lvl)), 1))


def _attention_tasks(pc, a0, qkv_s, att_s, r_s, o_s, vo, xl):
    base = pl.multiple_of(a0 * GT, GT)
    win = qkv_s.at[:, pl.ds(base, NA * GT + PAD), :]

    def block(b):
        a_s = att_s[b % len(att_s)]

        def shifted(j):
            v = {r: win[j, pl.ds(b * 16 + PAD + r, 8), :] for r in range(8, -DIL * W, -DIL)}
            return [jnp.concatenate([v[-DIL * w], v[8 - DIL * w]], axis=0) for w in range(W)]

        def scores():
            st = [None] * W
            for j in range(8):
                q = pc.gate(win[j, pl.ds(b * 16 + PAD, 16), :])
                for w, k in enumerate(shifted(8 + j)):
                    st[w] = q * k if j == 0 else st[w] + q * k
                pc.done(st[W - 1])
                yield
            for w in range(W):
                a_s[w] = st[w] + pltpu.roll(st[w], 127, 1)
            pc.stored(a_s, xl)

        def reduce():
            pc.open(a_s)
            for w in range(W):
                t = a_s[w]
                a_s[W + w] = t + pltpu.roll(t, 126, 1)
            pc.stored(a_s, xl)
            yield

        def softmax():
            pc.open(a_s)
            logits = []
            for w in range(W):
                t = a_s[W + w] * (DH ** -0.5 * LOG2E / XS ** 2)
                if b == 0 and w:
                    row = lax.broadcasted_iota(i32, (16, 128), 0) + base
                    t = jnp.where(row >= DIL * w, t, -1e9 * LOG2E)
                logits.append(t)
            m = functools.reduce(jnp.maximum, logits)
            yield
            m = pc.gate(m)
            e = [jnp.exp2(t - m) for t in logits]
            inv = (1.0 / XS) / _sum(e)
            yield
            inv = pc.gate(inv)
            for w in range(W):
                t = e[w] * inv
                a_s[2 * W + w] = jnp.where(_lane_bit((16, 128), 1), t, pltpu.roll(t, 1, 1))
            pc.stored(a_s, xl)
            yield

        def spread():
            pc.open(a_s)
            for w in range(W):
                t = a_s[2 * W + w]
                a_s[3 * W + w] = jnp.where(_lane_bit((16, 128), 2), t, pltpu.roll(t, 2, 1))
            pc.stored(a_s, xl)
            yield

        def values():
            for j in range(8):
                if j % vo == 0:
                    pc.open(a_s)
                    p = [a_s[3 * W + w] for w in range(W)]
                v = shifted(16 + j)
                r_s[b % 4 * 8 + j] = pc.done(_sum([p[w] * (v[w] if w else pc.gate(v[w])) for w in range(W)]))
                yield

        tail = [_operands(LHS, lambda i, j, e=e: r_s[i * 8 + 2 * j + e], pc, r_s, o_s,
                          _ds((a0 + b // 4) * 8, 8, 8), e * 128) for e in range(2) if b % 4 == 3]
        return [[(scores, 8)], [(reduce, 1)], [(softmax, 3)], [(spread, 1)], [(values, 8)] + tail]

    return _skewed([block(b) for b in range(NA * 4)])


def make(only=None, flags=None, scopes=False, nsc=False,
         d0=192, d1=256, d2=224, d3=256, vo=2, nbn=8, nbd=12, xl=128, hc=12, early=320,
         cutz=(0, 4, 7, 10, 12), cuts=(0, 22, 44, 64, 64), aw=(1, 2, 2, 5, 1, 6, 6, 2, 2, 1, 4, 4)):
    def loop(i, lo, hi, body):
        if only is None or i in only:
            fn = lambda: lax.fori_loop(lo, hi, body, None)
            (jax.named_call(fn, name=f"p{i}") if scopes else fn)()

    def kern(x_h, wqkv_h, wo_h, wg_h, wu_h, wd_h, out_h,
             x_s, wqkv_s, wo_s, wg_s, wu_s, wd_s, xa_s, o_s, ha_s, ba_s, bb_s, bd_s, bo_s,
             qkv_s, y_s, z_s, h_s, att_s, r_s, sw_s, sx, sq, sw, so, zero_s):
        free = _Pace()

        def x_cp(t):
            r = _ds(t * 4 * GT, 4 * GT, 4 * GT)
            return pltpu.make_async_copy(x_h.at[r, :], x_s.at[r, :], sx.at[t])

        def q_cps(t):
            r = _ds(t * 32, 32, 32)
            return [pltpu.make_async_copy(wqkv_h.at[:, r, pl.ds(p * CW, CW)], wqkv_s.at[p, :, r, :], sq.at[t])
                    for p in range(2)]

        def qkv_cp(p):
            src = wqkv_h.at[:, :, pl.ds(p * CW, CW)] if p < 6 else wg_h.at[:, :, pl.ds(0, CW)]
            return pltpu.make_async_copy(src, wqkv_s.at[p], sq.at[p])

        def up_cp(si, c):
            dst = (wg_s, wu_s)[si].at[pl.ds((c & 1) * 4, 4), pl.ds(0, D // 4)]
            return pltpu.make_async_copy((wg_h, wu_h)[si].at[:, :, _ds(c * CW, CW, CW)], dst, sw.at[2 * si + (c & 1)])

        def down_cp(c):
            return pltpu.make_async_copy(
                wd_h.at[_ds(c * CW, CW, CW), :], wd_s.at[c & 1, pl.ds(0, CW)], sw.at[4 + (c & 1)])

        def out_cp(row, rows, e):
            r = _ds(row, rows, GT)
            return pltpu.make_async_copy(x_s.at[r, pl.ds(e * CW, CW)], out_h.at[r, pl.ds(e * CW, CW)], so.at[0])

        wo_cp = pltpu.make_async_copy(wo_h, wo_s.at[0, pl.ds(0, D)], sq.at[7])

        def start_if(cond, *cps):
            for cp in cps:
                pl.when(cond)(lambda: cp.start())

        def wait_if(cond, *cps):
            for cp in cps:
                pl.when(cond)(lambda: cp.wait())

        def zeros():
            return [zero_s[i] & 1 for i in range(4)]

        def center_task(pc, t, b):
            def steps():
                v = x_s[_ds(t * 256 + b * 16, 16, 16), :].astype(f32)
                v = pc.done(_sum([pc.gate(_tile(v, 0))] + [_tile(v, j) for j in range(1, 8)]))
                att_s[0][b] = jnp.broadcast_to(jnp.sum(v, axis=1, keepdims=True) * (1.0 / D), (16, 128))
                yield

            return steps, 1

        def scale_task(pc, t, b, z=0):
            def steps():
                v, m = x_s[_ds((t + z) * 256 + b * 16, 16, 16), :].astype(f32), pc.gate(att_s[0][b + z])
                v = [_tile(v, j) - m for j in range(8)]
                v = jnp.sum(pc.done(_sum([a * a for a in v])), axis=1, keepdims=True) * (1.0 / D)
                att_s[1][b] = jnp.broadcast_to(lax.rsqrt(v + 1e-5) * XS, (16, 128))
                yield
                yield

            return steps, 2

        def norm_task(pc, t, g, e, z=0):
            def block(i, j):
                v = x_s[_ds((t + z) * 256 + g * GT + i * 16, 16, 16), _ds((2 * j + e) * 128, 128, 128)]
                return (v.astype(f32) - att_s[0][4 * g + i]) * att_s[1][4 * g + i + z]

            return _operands(LHS, block, pc, att_s[0], xa_s, _ds(t * 32 + g * 8, 8, 8), _ds(e * 128, 128, 128).start)

        def qkv_tasks(pc, job, ref, units, plain=False):
            def unit(u, t_s):
                st = {}

                def swap(lvl):
                    for i in range(4):
                        if lvl == 2:
                            a, b = [_pack(wqkv_s[s, i, _ds(u * 16, 16, 16), :])
                                    for s in (job, jnp.where(plain, job, job ^ 1))]
                            st[i] = [_swap(_tile(a, c), _tile(b, c), 2, job & 1, plain) for c in range(4)]
                        else:
                            st[i] = [_swap(st[i][c], st[i][c ^ (1 << lvl)], lvl, c >> lvl & 1, plain)
                                     for c in range(4)]
                        if lvl == 0:
                            for c in range(4):
                                t_s[4 * i + c] = st[i][c]
                    yield

                return [[(P(swap, lvl), 1)] for lvl in (2, 1, 0)] + [[
                    _operands(RHS, lambda i, j: _unpack(t_s[4 * i + j]).astype(f32), pc, t_s, ref,
                              _ds((u & 7) * 8, 8, 8), _ds((u >> 3) * 128, 128, 128).start)]]

            return _skewed([unit(u, sw_s[n % 4]) for n, u in enumerate(units)])

        def put_tasks(pc, src, job, g, ng):
            def put(r):
                res = yield from _result(pc, src, pl.ds(r, 8))
                for j in range(4):
                    for i in range(4):
                        qkv_s[4 * job + j, _ds((g + r // 16) * GT + i * 16 + r % 16 + PAD, 8, 8), :] = res[i][j]
                pc.done(res[0][3])

            return [(P(put, r), 3) for r in range(0, ng * 16, 8)]

        def keep(ref, rows):
            def emit(n, v):
                ref[n, 0:rows, :] = v

            return emit

        for cp in [x_cp(0)] + [cp for t in range(8) for cp in q_cps(t)] + [x_cp(1)]:
            cp.start()
        for i in range(4):
            zero_s[i] = 0
        for ref in [xa_s, o_s, ba_s, bb_s, bd_s, bo_s] + ha_s + att_s:
            ref[ref.shape[0] - 1, ref.shape[1] - 8:, 0:128] = jnp.zeros((8, 128), ref.dtype)

        def clear(i, _):
            y_s[0:8, _ds(i * 32, 32, 32), :] = jnp.zeros((8, 32, 128), f32)
            z_s[1][0:NZ, _ds(i * 8, 8, 8), :] = jnp.zeros((NZ, 8, 128), f32)
            for ref in att_s[:2]:
                ref[i] = jnp.zeros((16, 128), f32)
            x_s[_ds(S + i * 16, 16, 16), :] = jnp.zeros((16, D), bf16)

        lax.fori_loop(0, 16, clear, None)
        turn = (lax.broadcasted_iota(i32, (128, 128), 0) - lax.broadcasted_iota(i32, (128, 128), 1)) & 127
        for c in range(8):
            bb_s[c, 0:64, 0:128] = jnp.zeros((64, 128), u32)
            bb_s[c:c + 1, 0:64, 128:256] = _pack(jnp.where(turn == 4 * c, 1.0, 0.0)[None])

        def startup(it, _):
            wait_if(it < 8, *q_cps(jnp.minimum(it, 7)))
            u = [jnp.clip(it - s, 0, 7) for s in range(2)]
            blocks = [jnp.minimum(it, 3) * 4 + b for b in range(4)]
            for p, ref in enumerate((bd_s, bo_s)):
                v = [free.dot(bb_s[c, 0:64, 0:128], bb_s[c, 0:64, 128:256]) for c in range(4 * p, 4 * p + 4)]
                _run([_operands(RHS, lambda i, j, r=r: v[j][r * 64 + i * 16:r * 64 + i * 16 + 16], free, None, ref,
                                _ds((u[1] & 3) * 16 + r * 8, 8, 8), pl.multiple_of((u[1] >> 2) * 128, 128))
                      for r in range(2)])
            _run([norm_task(free, 0, u[1] >> 1, u[1] & 1)] + [center_task(free, 0, b) for b in blocks])
            for i in range(8):
                v = [_pack(wqkv_s[p, i % 4, _ds(u[0] * 32 + i // 4 * 16, 16, 16), :]) for p in range(2)]
                v = [pltpu.roll(_tile(v[c // 4], c % 4), 4 * c, 1) if c else _tile(v[0], 0) for c in range(8)]
                v = [v[-c] for c in range(8)]
                for b in (1, 2, 4):
                    v = [jnp.where(_lane_bit((8, 128), 4 * b), v[c], v[c - b]) for c in range(8)]
                for c in range(8):
                    bb_s[c, i * 8:(i + 1) * 8, 0:128] = v[c]
                if i == 3:
                    _run([scale_task(free, 0, b, zero_s[0]) for b in blocks])
            start_if(it == 7, x_cp(2), qkv_cp(2), qkv_cp(3), x_cp(3))

        x_cp(0).wait()
        loop(0, 0, 9, startup)

        def phase_q(t, _):
            wait_if(t < 7, x_cp(jnp.minimum(t + 1, 7)))
            wait_if(t == 2, qkv_cp(2), qkv_cp(3))
            pc = _Pace(zero_s[0], d0)
            z = zeros()
            nxt = jnp.minimum(t + 1, 7)
            prep = qkv_tasks(pc, jnp.where(t < 2, 0, 2), ba_s, [jnp.clip(3 * t - 6, 0, 13) + i for i in range(3)])

            def first(n):
                ha_s[0][n, 0:32, :] = v = xa_s[n, _ds(t * 32, 32, 32), :]
                return v

            pc.add(_mix(put_tasks(pc, z_s[1], 1, jnp.maximum(t - 1, 0) * 4, 4), prep[:hc],
                        [center_task(pc, nxt, b) for b in range(16)] + [scale_task(pc, nxt, b, z[0]) for b in range(16)]), NP * 32)
            _products(lambda n: pc.dot(first(n), _stacked(bd_s, n, 64)), keep(z_s[0], 64))
            pc.finish()
            pc.add(_mix(put_tasks(pc, z_s[0], 0, t * 4, 4), prep[hc:], [norm_task(pc, nxt, g, e, z[1]) for g in range(4) for e in range(2)]), NP * 32)
            _products(lambda n: pc.dot(ha_s[0][n + z[0], 0:32, :], _stacked(bo_s, n, 64)), keep(z_s[1], 64), 1)
            pc.finish()
            start_if(t == 1, *[x_cp(i) for i in range(4, 8)])

        loop(1, 0, 8, phase_q)
        for cp in (qkv_cp(4), qkv_cp(5), qkv_cp(6), wo_cp, up_cp(1, 0), down_cp(0), up_cp(0, 1),
                   up_cp(1, 1), down_cp(1), up_cp(0, 2)):
            cp.start()
        _run(put_tasks(free, z_s[1], 1, NG - 4, 4))

        def phase_kv(job, _):
            wait_if(job == 3, qkv_cp(4), qkv_cp(5))
            wait_if(job == 5, qkv_cp(6), wo_cp)
            pc = _Pace(zero_s[0], d1)
            z = zeros()
            prep = qkv_tasks(pc, job + 1, bb_s, range(16), job == 5)

            def clear_y(n):
                for r in range(0, S // 4, 64):
                    y_s[12 * job - 16 + n, r:r + 64, :] = pc.const(0.0, 64)
                    yield

            for rb in range(4):
                def prod(n):
                    y = pc.dot(xa_s[n, rb * 64:(rb + 1) * 64, :], _stacked(ba_s, n + z[rb] if rb < 3 else n, 64))
                    if rb == 3:
                        ba_s[n, 0:64, :] = pc.open(bb_s)[n, 0:64, :]
                    return y

                puts = put_tasks(pc, z_s[1 - rb % 2], job if rb else jnp.maximum(job - 1, 2), (rb - 1) % 4 * 8, 8)
                pc.add(_mix(puts, prep[cuts[rb]:cuts[rb + 1]]), NP * 64 - (256 if rb == 3 else 0))
                pc.add([(P(clear_y, n), 8) for n in range(cutz[rb], cutz[rb + 1])], NP * 64)
                _products(prod, keep(z_s[rb % 2], 128), rb)
                pc.finish()

        loop(2, 2, 6, phase_kv)
        _run(put_tasks(free, z_s[1], 5, NG - 8, 8))
        for j in range(8, 24):
            qkv_s[j, 0:PAD, :] = jnp.broadcast_to(qkv_s[j, PAD:PAD + 1, :], (PAD, 128))

        def phase_ffn(c, _):
            nxt = jnp.minimum(c + 1, NC - 1)
            up_cp(1, c).wait()
            down_cp(c).wait()
            wait_if(c + 1 < NC, up_cp(0, nxt))
            pc = _Pace(zero_s[0], d2)
            z = zeros()

            def up(rb, si):
                _products(lambda n: pc.dot(xa_s[n, rb * 64:(rb + 1) * 64, :], _stacked((ba_s, bb_s)[si], n + z[rb], 64)),
                          keep(z_s[rb % 2 * 2 + si], 128), pc.tiles // 2)

            def down(rb):
                for e in range(2):
                    def emit(n, v):
                        y_s[e * NZ + n, rb * 128:(rb + 1) * 128, :] += v

                    _products(lambda n: pc.dot(_stacked(ha_s[rb % 3], n + z[e + rb // 3 * 2], 32),
                                               bd_s[n + z[rb], 0:64, e * 128:(e + 1) * 128]), emit, e)

            def act(rb, r):
                g = yield from _result(pc, z_s[rb % 2 * 2], pl.ds(r, 8), scaled=True)
                u = yield from _result(pc, z_s[rb % 2 * 2 + 1], pl.ds(r, 8))
                for n in range(16):
                    i, j = n // 4, n % 4
                    s = 2.0 ** (j // 2 - i // 2 + j % 2 - i % 2)
                    t = pc.gate(g[i][j])
                    v = t * t if s == 1 else t * t * s ** -3
                    p = t * u[i][j ^ 3]
                    h_s[n, r:r + 8, :] = v = p * jnp.tanh(t * (v + C0 / XS / s)) + p
                    if j == 3:
                        pc.done(v)
                        yield

            def up_operands(w_s, slot, ref, flip):
                return [_weight_operands(
                    pc, w_s, lambda i, h, r=k + r: w_s[4 * slot + i, pl.ds(r, 16), pl.ds(h * 256, 256)].astype(f32),
                    ref, pl.ds(r // 2, 8), k, flip) for k in (0, 128) for r in range(0, 128, 16)]

            def out_operands(u, e, j0):
                def load(i, h):
                    lo = lax.broadcasted_iota(i32, (8, 256), 0) < 4
                    v = [wo_s[0, _ds((u & 1) * 512 + (u >> 1) * 32 + k * 128 + i * 8, 8, 8),
                              pl.ds(e * CW + h * 256, 256)].astype(f32) for k in range(4)]
                    return jnp.concatenate([
                        jnp.where(lo, pltpu.roll(a, 4, 0), b) if j0 else jnp.where(lo, a, pltpu.roll(b, 4, 0))
                        for a, b in (v[:2], v[2:])], axis=0)

                return _weight_operands(pc, wo_s, load, bo_s, _ds(j0 * 64 + u * 8, 8, 8), e * 128, 3)

            bu, bn = up_operands(wu_s, c & 1, bb_s, 3), up_operands(wg_s, nxt & 1, ba_s, 0)
            bd = [_weight_operands(
                pc, wd_s, lambda i, h, e=e, r=r: wd_s[c & 1, pl.ds(i * 128 + r, 16), pl.ds(e * CW + h * 256, 256)].astype(f32),
                bd_s, pl.ds(r // 2, 8), e * 128) for e in range(2) for r in range(0, 128, 16)]
            bo = [out_operands((2 * c + u) & 7, e, j0) for u in range(2) for e in range(2) for j0 in range(2)]
            acts = lambda rb: [(P(act, rb, r), 10) for r in range(0, 128, 8)]
            sums = lambda rb: [_operands(LHS, lambda i, j, e=e: h_s[4 * i + j, e * 16:(e + 1) * 16, :], pc, h_s,
                                         ha_s[rb % 3], pl.ds(e % 4 * 8, 8), e // 4 * 128, True) for e in range(8)]
            att = _attention_tasks(pc, jnp.minimum(c * NA, NG - NA), qkv_s, att_s, r_s, o_s, vo, xl)
            plan = [(P(up, 0, 0), bu, early), (P(up, 0, 1), bd[:nbd], 0),
                    (P(up, 1, 0), acts(0), 0), (P(up, 1, 1), _mix(sums(0), bd[nbd:]), early),
                    (P(down, 0), acts(1), 0), (P(up, 2, 0), sums(1), 0), (P(up, 2, 1), bo, 0),
                    (P(up, 3, 0), acts(2), 0), (P(up, 3, 1), sums(2) + bn[:nbn], 0),
                    (P(down, 1), acts(3), 0), (P(down, 2), sums(3), early), (P(down, 3), bn[nbn:], early)]
            for i, (products, tasks, slack) in enumerate(plan):
                lo, hi = [len(att) * sum(aw[:k]) // sum(aw) for k in (i, i + 1)]
                pc.add(_mix(tasks, att[lo:hi]), NP * 64 - slack)
                products()
                pc.finish()
            start_if(c + 2 < NC, up_cp(1, jnp.minimum(c + 2, NC - 1)), down_cp(jnp.minimum(c + 2, NC - 1)))
            start_if(c + 3 < NC, up_cp(0, jnp.minimum(c + 3, NC - 1)))

        loop(3, 0, NC, phase_ffn)

        def out_tasks(pc, dst, e):
            def out(r):
                s = yield from _result(pc, z_s[e], pl.ds(r, 8))
                for i in range(4):
                    rows = pl.ds(r // 16 * GT + i * 16 + r % 16, 8)
                    if i % 2 == 0:
                        pc.open(z_s[2 + e])
                    v = jnp.concatenate([s[i][j ^ 3] * z_s[2 + e][4 * i + j, r:r + 8, :] for j in range(4)], axis=1)
                    v = dst[rows, e * CW:(e + 1) * CW].astype(f32) + v
                    dst[rows, e * CW:(e + 1) * CW] = v.astype(bf16)
                    pc.done(_tile(v, 0))
                    if i % 2:
                        yield

            return [(P(out, r), 5) for r in range(0, 64, 8)]

        def phase_out(t, _):
            pc = _Pace(zero_s[0], d3)
            z = zeros()
            y0 = pl.multiple_of(t * 128, 128)
            for rb in range(2):
                tb = 2 * t + rb
                for e in range(2):
                    def gate(r):
                        y = yield from _result(pc, y_s, pl.ds(y0 + rb * 64 + r, 8), e * NZ)
                        for n in range(16):
                            if n % 8 == 0:
                                scale = pc.const(0.25 / XS ** 2, 8)
                            h = y[n // 4][n % 4] * scale
                            z_s[2 + e][n, r:r + 8, :] = h = h * jnp.tanh(h) + h
                            if n % 8 == 7:
                                pc.done(h)
                                yield

                    prev = tb if e else jnp.where(tb > 0, tb - 1, NG // 4)
                    outs = out_tasks(pc, x_s.at[_ds(prev * 4 * GT, 4 * GT, 4 * GT), :], 1 - e)
                    pc.add(_mix(outs, [(P(gate, r), 5) for r in range(0, 64, 8)]), NP * 32)
                    _products(lambda n: pc.dot(o_s[n + z[e], _ds(tb * 32, 32, 32), :],
                                               bo_s[n + z[rb], 0:128, e * 128:(e + 1) * 128]), keep(z_s[e], 64), e)
                    pc.finish()
                    start_if(prev < NG // 4, out_cp(jnp.minimum(prev, NG // 4 - 1) * 4 * GT, 4 * GT, 1 - e))

        loop(4, 0, 4, phase_out)
        last = out_tasks(free, x_s.at[S - 4 * GT:S, :], 1)
        for g in range(4):
            _run(last[2 * g:2 * g + 2])
            out_cp(S - (4 - g) * GT, GT, 1).start()
        pltpu.make_async_copy(x_s.at[pl.ds(0, S), :], out_h, so.at[0]).wait()

    def fn(A_x, A_wqkv, A_wo, B_x, B_w_gate, B_w_up, B_w_down):
        any_spec = pl.BlockSpec(memory_space=pl.ANY)
        out = pl.pallas_call(
            kern,
            in_specs=[any_spec] * 6,
            out_specs=any_spec,
            out_shape=jax.ShapeDtypeStruct((S, D), bf16),
            scratch_shapes=[
                pltpu.VMEM((S + 4 * GT, D), bf16),
                pltpu.VMEM((7, 4, D // 4, CW), bf16),
                pltpu.VMEM((1, D + 16, D), bf16),
                pltpu.VMEM((8, D // 4 + 16, CW), bf16),
                pltpu.VMEM((8, D // 4 + 16, CW), bf16),
                pltpu.VMEM((2, CW + 16, D), bf16),
                pltpu.VMEM((NP + 1, S // 8 + 8, 256), u32),
                pltpu.VMEM((NP + 1, S // 8 + 8, 256), u32),
                [pltpu.VMEM((NP + 1, 40, 256), u32)] * 3,
                pltpu.VMEM((NP + 1, 72, 256), u32),
                pltpu.VMEM((NP + 1, 72, 256), u32),
                pltpu.VMEM((NP + 1, 72, 256), u32),
                pltpu.VMEM((NP + 1, 136, 256), u32),
                pltpu.VMEM((24, S + PAD, 128), f32),
                pltpu.VMEM((2 * NZ + 4, S // 4 + 8, 128), f32),
                [pltpu.VMEM((NZ + 4, 136, 128), f32)] * 4,
                pltpu.VMEM((18, 144, 128), f32),
                [pltpu.VMEM((4 * W + 2, 16, 128), f32)] * 5,
                pltpu.VMEM((34, 16, 128), f32),
                [pltpu.VMEM((20, 8, 128), u32)] * 4,
                pltpu.SemaphoreType.DMA((8,)),
                pltpu.SemaphoreType.DMA((8,)),
                pltpu.SemaphoreType.DMA((6,)),
                pltpu.SemaphoreType.DMA((1,)),
                pltpu.SMEM((4,), i32),
            ],
            compiler_params=pltpu.CompilerParams(vmem_limit_bytes=127 << 20, flags=flags, disable_bounds_checks=nsc),
        )(A_x.reshape(S, D), A_wqkv.reshape(4, D // 4, 3 * D), A_wo,
          B_w_gate.reshape(4, D // 4, F), B_w_up.reshape(4, D // 4, F), B_w_down)
        return out.reshape(1, S, D)

    return fn


@jax.jit
def pallas_recurrent_scan__sliding_local_dilated__geglu_ffn__prompt_kernel(
    A_x, A_wqkv, A_wo, B_x, B_w_gate, B_w_up, B_w_down
):
    return make()(A_x, A_wqkv, A_wo, B_x, B_w_gate, B_w_up, B_w_down)
```

```python
import functools
import math

import jax
import jax.numpy as jnp
from jax import lax
import jax.experimental.pallas as pl
import jax.experimental.pallas.tpu as pltpu

S, D, F = 2048, 1024, 3584
DH, W, DIL = 32, 8, 2
PAD = 16
NP = 49
NZ = 28
GT = 64
NG = S // GT
CW = 512
NC = F // CW
NA = -(-NG // NC)
LOG2E = math.log2(math.e)
C0 = math.sqrt(2.0 / math.pi)
XS = (C0 * 0.044715) ** (1.0 / 3.0)
f32, bf16, u32, i32 = jnp.float32, jnp.bfloat16, jnp.uint32, jnp.int32
P = functools.partial


def _pack(v):
    return pltpu.bitcast(v.astype(bf16), u32)


def _unpack(v):
    return pltpu.bitcast(v, bf16)


def _ds(start, size, align):
    if isinstance(start, int):
        return pl.ds(start, size)
    return pl.ds(pl.multiple_of(start, align), size)


def _tile(v, j):
    return v[:, j * 128:(j + 1) * 128]


def _stacked(ref, n, rows):
    return jnp.concatenate([ref[n, 0:rows, k:k + 128] for k in (0, 128)], axis=0)


def _lane_bit(shape, bit):
    return (lax.broadcasted_iota(i32, shape, 1) & bit) == 0


def _sum(vs):
    return functools.reduce(lambda a, b: a + b, vs)


class _Pace:
    def __init__(self, zero=None, lag=256):
        self.zero, self.lag = zero, lag
        self.always = None if zero is None else zero == 0
        self.tok, self.time, self.tiles, self.due, self.queues = None, 0, 0, [], []

    def add(self, tasks, cycles):
        if tasks:
            steps = (None for fn, _ in tasks for _ in fn())
            self.queues.append([steps, sum(n for _, n in tasks), cycles, 0, 0])

    def finish(self):
        for q in self.queues:
            for _ in q[0]:
                pass
        self.queues = []

    def dot(self, lhs, rhs):
        rows, nk = 2 * lhs.shape[0], lhs.shape[1] // 128
        t0 = self.tiles // 4 * rows
        part = range(rows * (self.tiles % 4) // 4, rows * (self.tiles % 4 + nk) // 4)
        self.tiles += nk
        if self.due and self.due[0][0] < t0 + part.stop:
            col = [lhs[r:r + 8, 0:128] for r in range(0, rows // 2, 8)]
            toks = {}
            while self.due and self.due[0][0] < t0 + part.stop:
                t, tok = self.due.pop(0)
                toks.setdefault(max(t - t0, 0) // 16, []).append(pltpu.bitcast(tok, u32))
            for i, ts in toks.items():
                col[i] = jnp.where(self.always, col[i], functools.reduce(lambda a, b: a | b, ts))
            lhs = jnp.concatenate(
                [jnp.concatenate(col, axis=0)] + [_tile(lhs, j) for j in range(1, nk)], axis=1)
        y = jnp.dot(_unpack(lhs), _unpack(rhs), preferred_element_type=f32)
        for r in part[::8]:
            self.tok, self.time = functools.cache(lambda r=r: y[r:r + 8]), t0 + r
            for q in self.queues:
                q[3] += 8
                while q[4] < min(q[1], q[1] * q[3] // q[2]):
                    q[4] += 1
                    next(q[0], None)
        return y

    def const(self, c, rows):
        if self.zero is None or self.tok is None:
            return c
        return jnp.concatenate([jnp.where(self.always, c, self.tok())] * (rows // 8), axis=0)

    def gate(self, v):
        if self.zero is None or self.tok is None:
            return v
        return jnp.where(self.always, v, jnp.concatenate([self.tok()] * (v.shape[0] // 8), axis=0))

    def release(self, ref):
        if self.zero is not None and self.tok is not None:
            if ref.dtype == bf16:
                ref[self.zero, ref.shape[1] - 16:, 0:128] = pltpu.bitcast(self.tok(), bf16)
            else:
                ref[ref.shape[0] - 1 + self.zero, 0:8, 0:128] = pltpu.bitcast(self.tok(), ref.dtype)
        return ref

    def done(self, v, extra=0):
        if self.zero is not None:
            self.due.append((self.time + self.lag + extra, v[-8:]))
            self.due.sort(key=lambda d: d[0])
        return v

    def stored(self, ref, extra=0):
        if self.zero is not None:
            self.done(ref[ref.shape[0] - 1 + self.zero, ref.shape[1] - 8:, 0:128], extra)


def _run(tasks):
    for fn, _ in tasks:
        for _ in fn():
            pass


def _skewed(units):
    order = sorted((u + s, u, s) for u, st in enumerate(units) for s in range(len(st)))
    return [t for _, u, s in order for t in units[u][s]]


def _mix(*lists):
    keyed = []
    for i, ts in enumerate(lists):
        total, at = sum(n for _, n in ts), 0
        for t in ts:
            keyed.append(((at + t[1] / 2) / total, i, t))
            at += t[1]
    return [t for _, _, t in sorted(keyed, key=lambda k: k[:2])]


LHS, RHS = (6, 3, 0, 2, 1, 4, 5), (6, 0, 5, 4, 2, 1, 3)


def _basis(scaled, x11, x12, x21, x22):
    h = x21 if scaled else x21 * 0.5
    p = x11 + h
    return [x11 + x22, p, h + x22, (p + x22 + x12) * 0.5 if scaled else (p + x22) * 0.5 + x12]


def _unbasis(half, scaled, z0, z1, z2, z3):
    h = z0 * half
    e = z3 + h
    if scaled:
        return [e + z2, z2 + h + z1, h, e + z1]
    return [e + z2, (z2 + h + z1) * 0.5, z0, e + z1]


def _operands(side, block, pc, src, ref, rows, col, scaled=False):
    def quad(a, b):
        pc.release(src)
        return _basis(scaled, *[block(2 * a + n // 2, 2 * b + n % 2) for n in range(4)])

    def put(k, x):
        t, p, q, r = x
        for n, v in zip(side, (t, p, q, r, t - p, q - t, r - t)):
            ref[pl.ds(7 * side[k] + n, 1), rows, pl.ds(col, 128)] = _pack(v[None])
        pc.stored(ref)

    def steps():
        h = quad(1, 0) if scaled else [v * 0.5 for v in quad(1, 0)]
        yield
        x11 = quad(0, 0)
        put(1, [a + b for a, b in zip(x11, h)])
        yield
        put(5, [b - a for a, b in zip(x11, h)])
        yield
        x22 = quad(1, 1)
        t = [a + b for a, b in zip(x11, x22)]
        put(0, t)
        yield
        put(2, [a + b for a, b in zip(x22, h)])
        yield
        put(4, [a - b for a, b in zip(x22, h)])
        yield
        r = [(a + b + c) * 0.5 if scaled else (a + b) * 0.5 + c for a, b, c in zip(t, h, quad(0, 1))]
        put(3, r)
        yield
        put(6, [a - b for a, b in zip(r, t)])
        yield

    return steps, 8


def _weight_operands(pc, src, load, ref, rows, col, flip=0):
    load = functools.cache(load)
    return _operands(RHS, lambda i, j: _tile(load(i, (j ^ flip) // 2), (j ^ flip) % 2),
                     pc, src, ref, rows, col)


def _products(prod, emit, odd=0):
    for o in range(7):
        m = lambda i: prod(7 * o + i)
        early = (o + odd) % 2
        t = m(6) if early else None
        a = m(0)
        t = t - a if early else a
        emit(o, a + m(1))
        a = m(2)
        t = t - a if early else t + a
        emit(7 + o, a + m(3))
        a = m(4)
        t = t + a if early else a - t
        emit(14 + o, m(5) - a)
        emit(21 + o, t if early else t + m(6))


def _result(pc, ref, rows, base=0, scaled=False):
    x = []
    for k in range(4):
        if k % 2 == 0:
            pc.release(ref)
        m = [ref[base + 7 * k + o, rows, :] for o in range(7)]
        x.append(_unbasis(0.5, scaled, m[0] + m[1], m[2] + m[3], m[5] - m[4], m[4] + m[6] - m[0] - m[2]))
        if k % 2:
            yield
    half = pc.const(0.5, 8)
    x = [_unbasis(half, scaled, *col) for col in zip(*x)]
    yield
    return [[x[2 * (i // 2) + j // 2][2 * (i % 2) + j % 2] for j in range(4)] for i in range(4)]


def _swap(mine, other, lvl, upper, plain=False):
    keep = (_lane_bit(mine.shape, 4 << lvl) ^ (upper == 1)) | plain
    return jnp.where(keep, mine, pltpu.roll(other, (4 << lvl) + upper * (128 - (8 << lvl)), 1))


def _attention_tasks(pc, a0, qkv_s, att_s, r_s, o_s):
    base = pl.multiple_of(a0 * GT, GT)
    win = qkv_s.at[:, pl.ds(base, NA * GT + PAD), :]

    def block(b):
        a_s = att_s[b % len(att_s)]

        def shifted(j):
            v = {r: win[j, pl.ds(b * 16 + PAD + r, 8), :] for r in range(8, -DIL * W, -DIL)}
            return [jnp.concatenate([v[-DIL * w], v[8 - DIL * w]], axis=0) for w in range(W)]

        def scores():
            st = [None] * W
            for j in range(8):
                q = pc.gate(win[j, pl.ds(b * 16 + PAD, 16), :])
                for w, k in enumerate(shifted(8 + j)):
                    st[w] = q * k if j == 0 else st[w] + q * k
                pc.done(st[W - 1])
                yield
            for w in range(W):
                a_s[w] = st[w] + pltpu.roll(st[w], 127, 1)
            pc.stored(a_s, 128)

        def reduce():
            pc.release(a_s)
            for w in range(W):
                t = a_s[w]
                a_s[W + w] = t + pltpu.roll(t, 126, 1)
            pc.stored(a_s, 128)
            yield

        def softmax():
            pc.release(a_s)
            logits = []
            for w in range(W):
                t = a_s[W + w] * (DH ** -0.5 * LOG2E / XS ** 2)
                if b == 0 and w:
                    row = lax.broadcasted_iota(i32, (16, 128), 0) + base
                    t = jnp.where(row >= DIL * w, t, -1e9 * LOG2E)
                logits.append(t)
            m = functools.reduce(jnp.maximum, logits)
            yield
            m = pc.gate(m)
            e = [jnp.exp2(t - m) for t in logits]
            inv = (1.0 / XS) / _sum(e)
            yield
            inv = pc.gate(inv)
            for w in range(W):
                t = e[w] * inv
                a_s[2 * W + w] = jnp.where(_lane_bit((16, 128), 1), t, pltpu.roll(t, 1, 1))
            pc.stored(a_s, 128)
            yield

        def spread():
            pc.release(a_s)
            for w in range(W):
                t = a_s[2 * W + w]
                a_s[3 * W + w] = jnp.where(_lane_bit((16, 128), 2), t, pltpu.roll(t, 2, 1))
            pc.stored(a_s, 128)
            yield

        def values():
            for j in range(8):
                if j % 2 == 0:
                    pc.release(a_s)
                    p = [a_s[3 * W + w] for w in range(W)]
                v = shifted(16 + j)
                r_s[b % 4 * 8 + j] = pc.done(_sum([p[w] * (v[w] if w else pc.gate(v[w])) for w in range(W)]))
                yield

        tail = [_operands(LHS, lambda i, j, e=e: r_s[i * 8 + 2 * j + e], pc, r_s, o_s,
                          _ds((a0 + b // 4) * 8, 8, 8), e * 128) for e in range(2) if b % 4 == 3]
        return [[(scores, 8)], [(reduce, 1)], [(softmax, 3)], [(spread, 1)], [(values, 8)] + tail]

    return _skewed([block(b) for b in range(NA * 4)])


def _kernel(x_h, wqkv_h, wo_h, wg_h, wu_h, wd_h, out_h,
            x_s, wqkv_s, wo_s, wg_s, wu_s, wd_s,
            xa_s, o_s, ha_s,
            ba_s, bb_s, bd_s, bo_s,
            qkv_s, y_s, z_s, h_s, att_s, r_s, sw_s, sx, sq, zero_s):
    free = _Pace()

    def x_cp(t):
        r = _ds(t * 4 * GT, 4 * GT, 4 * GT)
        return pltpu.make_async_copy(x_h.at[r, :], x_s.at[r, :], sx.at[t])

    def x0_cp(t):
        r = _ds(t * 32 + GT, 32, 32)
        return pltpu.make_async_copy(x_h.at[r, :], x_s.at[r, :], sq.at[t])

    def q_cps(t):
        r = _ds(t * 32, 32, 32)
        return [pltpu.make_async_copy(wqkv_h.at[:, r, pl.ds(p * CW, CW)], wqkv_s.at[p, :, r, :], sq.at[t])
                for p in range(2)]

    def qkv_cp(p):
        src = wqkv_h.at[:, :, pl.ds(p * CW, CW)] if p < 6 else wg_h.at[:, :, pl.ds(0, CW)]
        return pltpu.make_async_copy(src, wqkv_s.at[p], sq.at[p])

    def up_cp(si, c):
        dst = (wg_s, wu_s)[si].at[pl.ds((c & 1) * 4, 4), pl.ds(0, D // 4)]
        return pltpu.make_async_copy((wg_h, wu_h)[si].at[:, :, _ds(c * CW, CW, CW)], dst, sx.at[2 * si + (c & 1)])

    def down_cp(c):
        return pltpu.make_async_copy(
            wd_h.at[_ds(c * CW, CW, CW), :], wd_s.at[c & 1, pl.ds(0, CW)], sx.at[4 + (c & 1)])

    def out_cp(row, rows, e):
        r = _ds(row, rows, GT)
        return pltpu.make_async_copy(x_s.at[r, pl.ds(e * CW, CW)], out_h.at[r, pl.ds(e * CW, CW)], sx.at[7])

    wo_cp = pltpu.make_async_copy(wo_h, wo_s.at[0, pl.ds(0, D)], sq.at[7])

    def start_if(cond, *cps):
        for cp in cps:
            pl.when(cond)(lambda: cp.start())

    def wait_if(cond, *cps):
        for cp in cps:
            pl.when(cond)(lambda: cp.wait())

    def zeros():
        return [zero_s[i] & 1 for i in range(4)]

    def center_task(pc, t, b):
        def steps():
            v = x_s[_ds(t * 256 + b * 16, 16, 16), :].astype(f32)
            v = pc.done(_sum([pc.gate(_tile(v, 0))] + [_tile(v, j) for j in range(1, 8)]))
            att_s[0][b] = jnp.broadcast_to(jnp.sum(v, axis=1, keepdims=True) * (1.0 / D), (16, 128))
            yield

        return steps, 1

    def scale_task(pc, t, b, z=0):
        def steps():
            v, m = x_s[_ds((t + z) * 256 + b * 16, 16, 16), :].astype(f32), pc.gate(att_s[0][b + z])
            v = [_tile(v, j) - m for j in range(8)]
            v = jnp.sum(pc.done(_sum([a * a for a in v])), axis=1, keepdims=True) * (1.0 / D)
            att_s[1][b] = jnp.broadcast_to(lax.rsqrt(v + 1e-5) * XS, (16, 128))
            yield
            yield

        return steps, 2

    def norm_task(pc, t, g, e, z=0):
        def block(i, j):
            v = x_s[_ds((t + z) * 256 + g * GT + i * 16, 16, 16), _ds((2 * j + e) * 128, 128, 128)]
            return (v.astype(f32) - att_s[0][4 * g + i]) * att_s[1][4 * g + i + z]

        return _operands(LHS, block, pc, att_s[0], xa_s, _ds(t * 32 + g * 8, 8, 8), _ds(e * 128, 128, 128).start)

    def qkv_tasks(pc, job, ref, units, plain=False):
        def unit(u, t_s):
            st = {}

            def swap(lvl):
                for i in range(4):
                    if lvl == 2:
                        a, b = [_pack(wqkv_s[s, i, _ds(u * 16, 16, 16), :])
                                for s in (job, jnp.where(plain, job, job ^ 1))]
                        st[i] = [_swap(_tile(a, c), _tile(b, c), 2, job & 1, plain) for c in range(4)]
                    else:
                        st[i] = [_swap(st[i][c], st[i][c ^ (1 << lvl)], lvl, c >> lvl & 1, plain)
                                 for c in range(4)]
                    if lvl == 0:
                        for c in range(4):
                            t_s[4 * i + c] = st[i][c]
                yield

            return [[(P(swap, lvl), 1)] for lvl in (2, 1, 0)] + [[
                _operands(RHS, lambda i, j: _unpack(t_s[4 * i + (j ^ 3)]).astype(f32), pc, t_s, ref,
                          _ds((u & 7) * 8, 8, 8), _ds((u >> 3) * 128, 128, 128).start)]]

        return _skewed([unit(u, sw_s[n % 4]) for n, u in enumerate(units)])

    def put_tasks(pc, src, job, g, ng, flip=0):
        def put(r):
            res = yield from _result(pc, src, pl.ds(r, 8))
            for j in range(4):
                for i in range(4):
                    rows = _ds((g + r // 16) * GT + i * 16 + r % 16 + PAD, 8, 8)
                    qkv_s[4 * job + j, rows, :] = res[i][j ^ flip]
            pc.done(res[0][3])

        return [(P(put, r), 3) for r in range(0, ng * 16, 8)]

    def keep(ref, rows):
        def emit(n, v):
            ref[n, 0:rows, :] = v

        return emit

    head_cp = pltpu.make_async_copy(x_h.at[0:GT, :], x_s.at[0:GT, :], sx.at[0])
    head_cp.start()
    for t in range(8):
        for cp in ([x0_cp(t)] if t < 6 else []) + q_cps(t):
            cp.start()
    x_cp(1).start()
    for i in range(4):
        zero_s[i] = 0
    for ref in [xa_s, o_s, ba_s, bb_s, bd_s, bo_s] + ha_s + att_s:
        ref[ref.shape[0] - 1, ref.shape[1] - 8:, 0:128] = jnp.zeros((8, 128), ref.dtype)

    z_s[1][0:NZ, 0:64, :] = jnp.zeros((NZ, 64, 128), f32)
    turn = (lax.broadcasted_iota(i32, (128, 128), 0) - lax.broadcasted_iota(i32, (128, 128), 1)) & 127
    for c in range(8):
        bb_s[c, 0:64, 0:128] = jnp.zeros((64, 128), u32)
        bb_s[c:c + 1, 0:64, 128:256] = _pack(jnp.where(turn == 4 * c, 1.0, 0.0)[None])

    def startup(it, _):
        wait_if(it < 6, x0_cp(jnp.minimum(it, 5)))
        wait_if(it < 8, *q_cps(jnp.minimum(it, 7)))
        u = [jnp.clip(it - s, 0, 7) for s in range(2)]
        blocks = [jnp.minimum(it, 5) * 2 + 4 + b for b in range(2)]
        for p, ref in enumerate((bd_s, bo_s)):
            v = [free.dot(bb_s[c, 0:64, 0:128], bb_s[c, 0:64, 128:256]) for c in range(4 * p, 4 * p + 4)]
            _run([_operands(RHS, lambda i, j, r=r: v[j][r * 64 + i * 16:r * 64 + i * 16 + 16], free, None, ref,
                            _ds((u[1] & 3) * 16 + r * 8, 8, 8), pl.multiple_of((u[1] >> 2) * 128, 128))
                  for r in range(2)])
        _run([norm_task(free, 0, u[1] >> 1, u[1] & 1)] + [center_task(free, 0, b) for b in blocks])
        for i in range(8):
            v = [_pack(wqkv_s[p, i % 4, _ds(u[0] * 32 + i // 4 * 16, 16, 16), :]) for p in range(2)]
            v = [pltpu.roll(_tile(v[c // 4], c % 4), 4 * c, 1) if c else _tile(v[0], 0) for c in range(8)]
            v = [v[-c] for c in range(8)]
            for b in (1, 2, 4):
                v = [jnp.where(_lane_bit((8, 128), 4 * b), v[c], v[c - b]) for c in range(8)]
            for c in range(8):
                bb_s[c, i * 8:(i + 1) * 8, 0:128] = v[c]
            if i == 3:
                _run([scale_task(free, 0, b, zero_s[0]) for b in blocks])
        z_s[1][0:NZ, _ds(u[0] * 8 + 64, 8, 8), :] = jnp.zeros((NZ, 8, 128), f32)
        x_s[_ds(S + u[0] * 32, 32, 32), CW:] = jnp.zeros((32, CW), bf16)
        start_if(it == 7, x_cp(2), qkv_cp(2), qkv_cp(3), x_cp(3))

    head_cp.wait()
    _run([task(free, 0, b) for task in (center_task, scale_task) for b in range(4)])
    lax.fori_loop(0, 9, startup, None)

    def phase_q(t, _):
        wait_if(t < 7, x_cp(jnp.minimum(t + 1, 7)))
        wait_if(t == 2, qkv_cp(2), qkv_cp(3))
        pc = _Pace(zero_s[0], 192)
        z = zeros()
        nxt = jnp.minimum(t + 1, 7)
        prep = qkv_tasks(pc, jnp.where(t < 2, 0, 2), ba_s, [jnp.clip(3 * t - 6, 0, 13) + i for i in range(3)])

        def first(n):
            ha_s[0][n, 0:32, :] = v = xa_s[n, _ds(t * 32, 32, 32), :]
            return v

        pc.add(_mix(put_tasks(pc, z_s[1], 1, jnp.maximum(t - 1, 0) * 4, 4), prep[:-1],
                    [center_task(pc, nxt, b) for b in range(16)]
                    + [scale_task(pc, nxt, b, z[0]) for b in range(16)]), NP * 32)
        _products(lambda n: pc.dot(first(n), _stacked(bd_s, n, 64)), keep(z_s[0], 64))
        pc.finish()
        pc.add(_mix(put_tasks(pc, z_s[0], 0, t * 4, 4), prep[-1:],
                    [norm_task(pc, nxt, g, e, z[1]) for g in range(4) for e in range(2)]), NP * 32)
        _products(lambda n: pc.dot(ha_s[0][n + z[0], 0:32, :], _stacked(bo_s, n, 64)), keep(z_s[1], 64), 1)
        pc.finish()
        start_if(t == 1, *[x_cp(i) for i in range(4, 8)])
        start_if(t == 4, wo_cp)

    lax.fori_loop(0, 8, phase_q, None)
    for cp in (qkv_cp(4), qkv_cp(5), qkv_cp(6), up_cp(1, 0), down_cp(0), up_cp(0, 1),
               up_cp(1, 1), down_cp(1), up_cp(0, 2)):
        cp.start()
    _run(put_tasks(free, z_s[1], 1, NG - 4, 4))
    wo_cp.wait()

    def phase_kv(job, _):
        wait_if(job == 3, qkv_cp(4), qkv_cp(5))
        wait_if(job == 5, qkv_cp(6))
        pc = _Pace(zero_s[0], 288)
        z = zeros()
        prep = qkv_tasks(pc, job + 1, bb_s, range(16), job == 5)

        def out_operands(u, e, j0):
            def load(i, h):
                lo = lax.broadcasted_iota(i32, (8, 256), 0) < 4
                v = [wo_s[0, _ds((u & 1) * 512 + (u >> 1) * 32 + k * 128 + i * 8, 8, 8),
                          pl.ds(e * CW + h * 256, 256)].astype(f32) for k in range(4)]
                return jnp.concatenate([
                    jnp.where(lo, pltpu.roll(a, 4, 0), b) if j0 else jnp.where(lo, a, pltpu.roll(b, 4, 0))
                    for a, b in (v[:2], v[2:])], axis=0)

            return _weight_operands(pc, wo_s, load, bo_s, _ds(j0 * 64 + u * 8, 8, 8), e * 128, 3)

        bo = [out_operands(2 * job - 4 + u, e, j0) for u in range(2) for e in range(2) for j0 in range(2)]

        def clear_y(n):
            for r in range(0, S // 4, 64):
                y_s[14 * (job - 2) + n, r:r + 64, :] = pc.const(0.0, 64)
                yield

        cuts, cuto, cutz = (0, 24, 45, 64, 64), (0, 3, 4, 5, 8), (0, 4, 8, 12, 14)
        for rb in range(4):
            def prod(n):
                y = pc.dot(xa_s[n, rb * 64:(rb + 1) * 64, :], _stacked(ba_s, n + z[rb] if rb < 3 else n, 64))
                if rb == 3:
                    ba_s[n, 0:64, :] = pc.release(bb_s)[n, 0:64, :]
                return y

            puts = put_tasks(pc, z_s[1 - rb % 2], job if rb else jnp.maximum(job - 1, 2), (rb - 1) % 4 * 8, 8, 3)
            pc.add(_mix(puts, prep[cuts[rb]:cuts[rb + 1]], bo[cuto[rb]:cuto[rb + 1]]),
                   NP * 64 - (256 if rb == 3 else 0))
            pc.add([(P(clear_y, n), 8) for n in range(cutz[rb], cutz[rb + 1])], NP * 64)
            _products(prod, keep(z_s[rb % 2], 128), rb)
            pc.finish()

    lax.fori_loop(2, 6, phase_kv, None)
    _run(put_tasks(free, z_s[1], 5, NG - 8, 8, 3))
    for j in range(8, 24):
        qkv_s[j, 0:PAD, :] = jnp.broadcast_to(qkv_s[j, PAD:PAD + 1, :], (PAD, 128))

    def phase_ffn(c, _):
        nxt = jnp.minimum(c + 1, NC - 1)
        up_cp(1, c).wait()
        down_cp(c).wait()
        wait_if(c + 1 < NC, up_cp(0, nxt))
        pc = _Pace(zero_s[0], 224)
        z = zeros()

        def up(rb, si):
            _products(lambda n: pc.dot(xa_s[n, rb * 64:(rb + 1) * 64, :],
                                       _stacked((ba_s, bb_s)[si], n + z[rb] if rb + si else n, 64)),
                      keep(z_s[rb % 2 * 2 + si], 128), pc.tiles // 2)

        def down(rb):
            for e in range(2):
                def emit(n, v):
                    y_s[e * NZ + n, rb * 128:(rb + 1) * 128, :] += v

                _products(lambda n: pc.dot(_stacked(ha_s[rb % 3], n + z[e + rb // 3 * 2], 32),
                                           bd_s[n + z[rb], 0:64, e * 128:(e + 1) * 128]), emit, e)

        def act(rb, r):
            g = yield from _result(pc, z_s[rb % 2 * 2], pl.ds(r, 8))
            u = yield from _result(pc, z_s[rb % 2 * 2 + 1], pl.ds(r, 8), scaled=True)
            for n in range(16):
                i, j = n // 4, n % 4
                if j == 0:
                    c0 = pc.const(C0 / XS, 8)
                t = g[i][j ^ 3]
                p = t * u[i][j]
                h_s[n, r:r + 8, :] = v = p * jnp.tanh(t * (t * t + c0)) + p
                if j == 3:
                    pc.done(v)
                    yield

        def up_operands(w_s, slot, ref, flip):
            return [_weight_operands(
                pc, w_s, lambda i, h, r=k + r: w_s[4 * slot + i, pl.ds(r, 16), pl.ds(h * 256, 256)].astype(f32),
                ref, pl.ds(r // 2, 8), k, flip) for k in (0, 128) for r in range(0, 128, 16)]

        bu, bn = up_operands(wu_s, c & 1, bb_s, 0), up_operands(wg_s, nxt & 1, ba_s, 3)
        bd = [_weight_operands(
            pc, wd_s,
            lambda i, h, e=e, r=r: wd_s[c & 1, pl.ds(i * 128 + r, 16), pl.ds(e * CW + h * 256, 256)].astype(f32),
            bd_s, pl.ds(r // 2, 8), e * 128) for e in range(2) for r in range(0, 128, 16)]
        acts = lambda rb: [(P(act, rb, r), 10) for r in range(0, 128, 8)]
        sums = lambda rb: [_operands(LHS, lambda i, j, e=e: h_s[4 * i + j, e * 16:(e + 1) * 16, :], pc, h_s,
                                     ha_s[rb % 3], pl.ds(e % 4 * 8, 8), e // 4 * 128, True) for e in range(8)]
        att = _attention_tasks(pc, jnp.minimum(c * NA, NG - NA), qkv_s, att_s, r_s, o_s)
        plan = [(P(up, 0, 0), bu, 448), (P(up, 0, 1), bd[:15], 0),
                (P(up, 1, 0), acts(0), 0), (P(up, 1, 1), _mix(sums(0), bd[15:]), 320),
                (P(down, 0), acts(1), 0), (P(up, 2, 0), sums(1), 0), (P(up, 2, 1), [], 0),
                (P(up, 3, 0), acts(2), 0), (P(up, 3, 1), sums(2) + bn[:10], 0),
                (P(down, 1), acts(3), 0), (P(down, 2), sums(3), 192), (P(down, 3), bn[10:], 320)]
        aw = (2, 4, 4, 10, 2, 12, 15, 4, 3, 3, 7, 6)
        for i, (products, tasks, slack) in enumerate(plan):
            lo, hi = [len(att) * sum(aw[:k]) // sum(aw) for k in (i, i + 1)]
            pc.add(_mix(tasks, att[lo:hi]), NP * 64 - slack)
            products()
            pc.finish()
        start_if(c + 2 < NC, up_cp(1, jnp.minimum(c + 2, NC - 1)), down_cp(jnp.minimum(c + 2, NC - 1)))
        start_if(c + 3 < NC, up_cp(0, jnp.minimum(c + 3, NC - 1)))

    lax.fori_loop(0, NC, phase_ffn, None)

    def out_tasks(pc, dst, e):
        def out(r):
            s = yield from _result(pc, z_s[e], pl.ds(r, 8))
            for i in range(4):
                rows = pl.ds(r // 16 * GT + i * 16 + r % 16, 8)
                if i % 2 == 0:
                    pc.release(z_s[2 + e])
                v = jnp.concatenate([s[i][j ^ 3] * z_s[2 + e][4 * i + j, r:r + 8, :] for j in range(4)], axis=1)
                v = dst[rows, e * CW:(e + 1) * CW].astype(f32) + v
                dst[rows, e * CW:(e + 1) * CW] = v.astype(bf16)
                pc.done(_tile(v, 0))
                if i % 2:
                    yield

        return [(P(out, r), 5) for r in range(0, 64, 8)]

    def phase_out(t, _):
        pc = _Pace(zero_s[0], 192)
        z = zeros()
        y0 = pl.multiple_of(t * 128, 128)
        for rb in range(2):
            tb = 2 * t + rb
            for e in range(2):
                def gate(r):
                    y = yield from _result(pc, y_s, pl.ds(y0 + rb * 64 + r, 8), e * NZ)
                    for n in range(16):
                        if n % 8 == 0:
                            scale = pc.const(0.25 / XS ** 2, 8)
                        h = y[n // 4][n % 4] * scale
                        z_s[2 + e][n, r:r + 8, :] = h = h * jnp.tanh(h) + h
                        if n % 8 == 7:
                            pc.done(h)
                            yield

                prev = tb if e else jnp.where(tb > 0, tb - 1, NG // 4)
                outs = out_tasks(pc, x_s.at[_ds(prev * 4 * GT, 4 * GT, 4 * GT), :], 1 - e)
                pc.add(_mix(outs, [(P(gate, r), 5) for r in range(0, 64, 8)]), NP * 32)
                _products(lambda n: pc.dot(o_s[n + z[e], _ds(tb * 32, 32, 32), :],
                                           bo_s[n + z[rb], 0:128, e * 128:(e + 1) * 128]), keep(z_s[e], 64), e)
                pc.finish()
                start_if(prev < NG // 4, out_cp(jnp.minimum(prev, NG // 4 - 1) * 4 * GT, 4 * GT, 1 - e))

    lax.fori_loop(0, 4, phase_out, None)
    last = out_tasks(free, x_s.at[S - 4 * GT:S, :], 1)
    for g in range(4):
        _run(last[2 * g:2 * g + 2])
        out_cp(S - (4 - g) * GT, GT, 1).start()
    pltpu.make_async_copy(x_s.at[pl.ds(0, S), :], out_h, sx.at[7]).wait()


@jax.jit
def pallas_recurrent_scan__sliding_local_dilated__geglu_ffn__prompt_kernel(
    A_x: jax.Array,
    A_wqkv: jax.Array,
    A_wo: jax.Array,
    B_x: jax.Array,
    B_w_gate: jax.Array,
    B_w_up: jax.Array,
    B_w_down: jax.Array,
):
    del B_x
    any_spec = pl.BlockSpec(memory_space=pl.ANY)
    out = pl.pallas_call(
        _kernel,
        in_specs=[any_spec] * 6,
        out_specs=any_spec,
        out_shape=jax.ShapeDtypeStruct((S, D), bf16),
        scratch_shapes=[
            pltpu.VMEM((S + 4 * GT, D), bf16),
            pltpu.VMEM((7, 4, D // 4, CW), bf16),
            pltpu.VMEM((1, D + 16, D), bf16),
            pltpu.VMEM((8, D // 4 + 16, CW), bf16),
            pltpu.VMEM((8, D // 4 + 16, CW), bf16),
            pltpu.VMEM((2, CW + 16, D), bf16),
            pltpu.VMEM((NP + 1, S // 8 + 8, 256), u32),
            pltpu.VMEM((NP + 1, S // 8 + 8, 256), u32),
            [pltpu.VMEM((NP + 1, 40, 256), u32)] * 3,
            pltpu.VMEM((NP + 1, 72, 256), u32),
            pltpu.VMEM((NP + 1, 72, 256), u32),
            pltpu.VMEM((NP + 1, 72, 256), u32),
            pltpu.VMEM((NP + 1, 136, 256), u32),
            pltpu.VMEM((24, S + PAD, 128), f32),
            pltpu.VMEM((2 * NZ + 4, S // 4 + 8, 128), f32),
            [pltpu.VMEM((NZ + 4, 136, 128), f32)] * 4,
            pltpu.VMEM((18, 144, 128), f32),
            [pltpu.VMEM((4 * W + 2, 16, 128), f32)] * 5,
            pltpu.VMEM((34, 16, 128), f32),
            [pltpu.VMEM((20, 8, 128), u32)] * 4,
            pltpu.SemaphoreType.DMA((8,)),
            pltpu.SemaphoreType.DMA((8,)),
            pltpu.SMEM((4,), i32),
        ],
        compiler_params=pltpu.CompilerParams(vmem_limit_bytes=127 << 20),
    )(A_x.reshape(S, D), A_wqkv.reshape(4, D // 4, 3 * D), A_wo,
      B_w_gate.reshape(4, D // 4, F), B_w_up.reshape(4, D // 4, F), B_w_down)
    return out.reshape(1, S, D)
```
